```python
import jax
import jax.numpy as jnp

def _softmax(x, axis=-1):
    return jax.nn.softmax(x, axis=axis)

def _gelu(x):
    return jax.nn.gelu(x, approximate=True)

def _silu(x):
    return jax.nn.silu(x)

def _sigmoid(x):
    return jax.nn.sigmoid(x)

def _layernorm(x, axis=-1, eps=1e-05):
    m = jnp.mean(x, axis=axis, keepdims=True)
    v = jnp.var(x, axis=axis, keepdims=True)
    return (x - m) / jnp.sqrt(v + eps)

def _scatter_add(tgt, idx, src, axis=0):
    return tgt.at[idx].add(src)

def _segment_sum(src, seg, n):
    return jax.ops.segment_sum(src, seg, n)

class _Rng:

    def __init__(self, key):
        self._k = key

    def _next(self):
        self._k, sub = jax.random.split(self._k)
        return sub

    def normal(self, shape):
        return jax.random.normal(self._next(), shape, dtype=jnp.bfloat16)

    def randint(self, lo, hi, shape):
        return jax.random.randint(self._next(), shape, lo, hi, dtype=jnp.int32)

    def uniform(self, shape, lo=0.0, hi=1.0):
        return jax.random.uniform(self._next(), shape, jnp.bfloat16, lo, hi)

    def permutation(self, n):
        return jax.random.permutation(self._next(), n)
kernel_name = 'adaLN_cond__ssm_conv_h3__glu_gated_bilinear__prompt'

def setup_inputs():
    _rng = _Rng(jax.random.key(int.from_bytes(__import__("os").urandom(4), "little")))
    _w = lambda a: (lambda t: t.astype(jnp.bfloat16) if jnp.issubdtype(t.dtype, jnp.floating) else t)(jnp.asarray(a))

    def _A_setup():
        B, S, D = (1, 2048, 640)
        ks = 4
        return {'q': _w((lambda *s: _rng.normal(s) * 0.05)(B, S, D)), 'k': _w((lambda *s: _rng.normal(s) * 0.05)(B, S, D)), 'v': _w((lambda *s: _rng.normal(s) * 0.05)(B, S, D)), 'shift_k': _w((lambda *s: _rng.normal(s) * 0.05)(D, ks) * 0.5), 'ssm_k': _w((lambda *s: _rng.normal(s) * 0.05)(D, S) * (1.0 / S ** 0.5)), 'ssm_D': _w((lambda *s: _rng.normal(s) * 0.05)(D))}
    _A_in = _A_setup()

    def _B_setup():
        B, S, D, F = (1, 2048, 640, 1536)
        return {'x': _w((lambda *s: _rng.normal(s) * 0.05)(B, S, D)), 'w_gate': _w((lambda *s: _rng.normal(s) * 0.05)(D, F) * D ** (-0.5)), 'w_up': _w((lambda *s: _rng.normal(s) * 0.05)(D, F) * D ** (-0.5)), 'w_down': _w((lambda *s: _rng.normal(s) * 0.05)(F, D) * F ** (-0.5))}
    _B_in = _B_setup()
    return {'A_q': _A_in['q'], 'A_k': _A_in['k'], 'A_v': _A_in['v'], 'A_shift_k': _A_in['shift_k'], 'A_ssm_k': _A_in['ssm_k'], 'A_ssm_D': _A_in['ssm_D'], 'B_x': _B_in['x'], 'B_w_gate': _B_in['w_gate'], 'B_w_up': _B_in['w_up'], 'B_w_down': _B_in['w_down'], 'c': _w((lambda *s: _rng.normal(s) * 0.05)(1, 640)), 'w_mod': _w((lambda *s: _rng.normal(s) * 0.05)(640, 6 * 640) * 640 ** (-0.5))}

def reference(A_q, A_k, A_v, A_shift_k, A_ssm_k, A_ssm_D, B_x, B_w_gate, B_w_up, B_w_down, c, w_mod):

    def _A_ref(q, k, v, shift_k, ssm_k, ssm_D):
        B, S, D = q.shape
        ks = shift_k.shape[-1]
        k_pad = jnp.pad(k, ((0, 0), (ks - 1, 0), (0, 0)))
        k_shift = jnp.zeros_like(k)
        for t in range(ks):
            k_shift = k_shift + k_pad[:, t:t + S, :] * shift_k[:, ks - 1 - t][None, None, :]
        kv = k_shift * v
        L = 2 * S
        kv_pad = jnp.pad(kv, ((0, 0), (0, S), (0, 0)))
        kf_pad = jnp.pad(ssm_k, ((0, 0), (0, S)))
        kv_f = (lambda x, axes=(-2, -1): jnp.fft.rfft2(x.astype(jnp.float32), axes=axes))(kv_pad[:, None, :, :], axes=(1, 2))
        kf_f = (lambda x, axes=(-2, -1): jnp.fft.rfft2(x.astype(jnp.float32), axes=axes))(kf_pad[:, None, :], axes=(1, 2))
        kf_f = (lambda x, *d: x.transpose(*d))(kf_f, 1, 2, 0)
        y_f = kv_f * kf_f[None, :, :, :]
        y = (lambda x, s, axes=(-2, -1): jnp.fft.irfft2(x, s=s, axes=axes).astype(jnp.bfloat16))(y_f, (1, L), axes=(1, 2))[:, 0, :S, :]
        y = y + kv * ssm_D[None, None, :]
        return q * y

    def _B_ref(x, w_gate, w_up, w_down):
        g = jnp.einsum('bsd,df->bsf', x, w_gate)
        u = jnp.einsum('bsd,df->bsf', x, w_up)
        h = g * u
        return jnp.einsum('bsf,fd->bsd', h, w_down)
    x = A_q
    mod = (_silu(c) @ w_mod).reshape(c.shape[0], 6, 1, -1)
    sa, ca, ga, sb, cb, gb = (mod[:, 0].copy(), mod[:, 1].copy(), mod[:, 2].copy(), mod[:, 3].copy(), mod[:, 4].copy(), mod[:, 5].copy())
    h = _layernorm(x, axis=-1) * (1 + ca) + sa
    x = x + ga * _A_ref(h, A_k, A_v, A_shift_k, A_ssm_k, A_ssm_D)
    h = _layernorm(x, axis=-1) * (1 + cb) + sb
    x = x + gb * _B_ref(h, B_w_gate, B_w_up, B_w_down)
    return x
```

```python
import numpy as np
import jax
import jax.numpy as jnp
from jax import lax
import jax.experimental.pallas as pl
import jax.experimental.pallas.tpu as pltpu

S, D, FF = 2048, 640, 1536
C = 128
NB = S // C
M = 256
NC = S // M
LT = D // 128
NT = FF // 128
EPS = 1e-5
F32 = jnp.float32
BF16 = jnp.bfloat16


def _dft_consts():
    r = np.arange(C)
    theta = np.pi * (4 * r + 1) / (2 * C)
    c = np.arange(C)
    ang = theta[:, None] * c[None, :]
    cs = np.stack([np.cos(ang), -np.sin(ang)], axis=0)
    fm = cs.reshape(2, 2, 8, 8, C).transpose(2, 1, 0, 3, 4).reshape(2 * C, C)
    a = np.concatenate([np.arange(0, C, 2), np.arange(1, C, 2)])
    ang2 = a[:, None] * theta[None, :64]
    g = np.zeros((C, 8, 2, 8))
    g[:, :, 0] = np.cos(ang2).reshape(C, 8, 8) / C
    g[:, :, 1] = -np.sin(ang2).reshape(C, 8, 8) / C
    g = g.reshape(C, C)
    return np.concatenate([fm, g], axis=0).astype(np.float32)


E_SLOTS = tuple(range(3, 35, 2))
AB_SLOTS = (1, 1, 2, 2, 3)
C_SLOTS = tuple(sorted(list(range(6, 39)) + [9, 11, 13, 15, 17, 19, 21]))
D_SLOTS = (39,) * 5
E1_SLOTS = (18, 19, 20, 21, 22, 23, 26, 27, 28, 29, 32, 33, 34, 35, 36, 37)
C1_SLOTS = tuple(sorted(3 * [18, 19, 20, 21, 22, 23, 26, 27, 28, 29] + 2 * [32, 33, 34, 35, 36]))
NSEM = 48


def _mo(x, m):
    return x if isinstance(x, int) else pl.multiple_of(x, m)


def _ls(t):
    return slice(t * 128, (t + 1) * 128)


def _kernel(q_h, k_h, v_h, sh_h, sk_h, sd_h, wg_h, wu_h, wd_h, c_h, wm_h, cst_h,
            o_h,
            q_v, k_v, v_v, sk_v, wg_v, wu_v, wd0, wd1, wd2, wm_v, cst_v,
            o_v, kbuf, xf, kf, qbuf, ybuf, x1buf, h2buf, modv, shb, sh_v, sd_v, c_v, pad_v,
            sem_in, sem_out):
    nsem = [0]

    def cp(src, dst):
        n = nsem[0]
        nsem[0] += 1
        return pltpu.make_async_copy(src, dst, sem_in.at[n])

    def conv_in(c0, c1):
        cols = pl.ds(c0 * M, (c1 - c0) * M)
        return [cp(sk_h.at[:, cols], sk_v.at[:, cols]), cp(k_h.at[c0:c1], k_v.at[c0:c1]),
                cp(v_h.at[c0:c1], v_v.at[c0:c1])]

    def q_in(c0, c1):
        return [cp(q_h.at[c0:c1], q_v.at[c0:c1])]

    def gu_in(n0, n1):
        cols = pl.ds(n0 * 128, (n1 - n0) * 128)
        return [cp(wg_h.at[:, cols], wg_v.at[0:D, cols]), cp(wu_h.at[:, cols], wu_v.at[0:D, cols])]

    def wd_in(n0, n1):
        cols = pl.ds(n0 * 128, (n1 - n0) * 128)
        return [cp(wd_h.at[kc * 512:(kc + 1) * 512, cols], w.at[0:512, cols])
                for kc, w in enumerate((wd0, wd1, wd2))]

    dma = dict(
        small=[cp(cst_h, cst_v), cp(sh_h, sh_v), cp(sd_h, sd_v), cp(c_h, c_v)],
        c0=conv_in(0, 1),
        c1=conv_in(1, 2),
        wma=[cp(wm_h.at[:, 0:5 * D], wm_v.at[:, 0:5 * D])] + q_in(0, 1),
        w1=gu_in(0, 4),
        w2=gu_in(4, 8),
        c2=conv_in(2, 3) + q_in(1, 2),
        w3=gu_in(8, 12),
        wd1=[cp(wm_h.at[:, 5 * D:6 * D], wm_v.at[:, 5 * D:6 * D])] + wd_in(0, 2),
        wd2=wd_in(2, 5),
        c3=conv_in(3, 4) + q_in(2, 3),
        rest=conv_in(4, 8) + q_in(3, 8),
    )
    assert nsem[0] <= NSEM

    def wait(name):
        with jax.named_scope("w_" + name):
            for c_ in dma[name]:
                c_.wait()

    def out_copy(i):
        return pltpu.make_async_copy(o_v.at[i], o_h.at[i], sem_out.at[i])

    for grp in dma.values():
        for c_ in grp:
            c_.start()

    for t in range(LT):
        kbuf[t, 24:32, :] = jnp.zeros((8, 128), F32)
    xf[0] = jnp.zeros((LT, 16, 24, 128), F32)
    qbuf[0] = jnp.zeros((LT, 8, 32, 128), F32)
    pad_v[...] = jnp.zeros(pad_v.shape, F32)
    wait('small')
    sh = sh_v[...].astype(F32)
    for j in range(4):
        shb[j] = jnp.broadcast_to(sh[j:j + 1, :], (8, D))

    def stage_a(c, t):
        r0 = _mo(c * M, M)
        ls = _ls(t)
        kk = k_v[c, :, ls].astype(F32)
        kbuf[t, pl.ds(r0 + 32, M), :] = kk
        acc = kk.reshape(32, 8, 128) * shb[0, :, ls][None]
        for j in range(1, 4):
            acc = acc + kbuf[t, pl.ds(r0 + 32 - j, M), :].reshape(32, 8, 128) * shb[j, :, ls][None]
        kv = acc.reshape(M, 128) * v_v[c, :, ls].astype(F32)
        for b in range(2):
            r = jnp.dot(cst_v[0:2 * C, :], kv[b * C:(b + 1) * C].astype(BF16),
                        preferred_element_type=F32).reshape(16, 16, 128)
            xf[2 * c + 1 + b, t, :, 0:16, :] = r
            xf[2 * c + 1 + b, t, :, 16:24, :] = r[:, 0:8, :] + r[:, 8:16, :]

    def stage_b(c, t):
        for b in range(2):
            kb = sk_v[_ls(t), pl.ds(_mo(c * M + b * C, C), C)]
            r = lax.dot_general(cst_v[0:2 * C, :], kb, (((1,), (1,)), ((), ())),
                                preferred_element_type=F32).reshape(16, 16, 128)
            cc = r[:, 0:8, :]
            d = r[:, 8:16, :]
            if isinstance(c, int) and c == 0 and b == 0:
                cc = cc + sd_v[...].astype(F32).reshape(1, 1, D)[:, :, _ls(t)]
            kf[2 * c + b, t, :, 0:8, :] = d - cc
            kf[2 * c + b, t, :, 8:16, :] = cc + d
            kf[2 * c + b, t, :, 16:24, :] = cc

    def lag_idx(c, cmin, cmax):
        nlag = 2 * cmax + 2
        jok = 2 * cmin + 1
        kidx = [j if j <= jok else jnp.minimum(j, 2 * c + 1) for j in range(nlag)]
        xidx = [2 * c + 2 - j if j <= jok + 1 else jnp.maximum(2 * c + 2 - j, 0) for j in range(nlag)]
        return kidx, xidx

    def _reim_eo(acc):
        re = acc[:, 16:24] - acc[:, 8:16]
        im = acc[:, 16:24] + acc[:, 0:8]
        return re[0] + re[1], im[0] + im[1], re[0] - re[1], im[0] - im[1]

    def cone(c, idx, t, u):
        kidx, xidx = idx
        nlag = len(kidx)
        us = slice(2 * u, 2 * u + 2)
        x = None
        acc0 = acc1 = None
        for j in reversed(range(nlag)):
            k = kf[kidx[j], t, us]
            if x is not None:
                p = k * x
                acc0 = p if acc0 is None else acc0 + p
            x = xf[xidx[j], t, us]
            p = k * x
            acc1 = p if acc1 is None else acc1 + p
        q0 = _reim_eo(acc0)
        q1 = _reim_eo(acc1)
        qbuf[c + 1, t, u] = jnp.concatenate(q1, axis=0)
        prev = qbuf[c, t, u]
        qp = (prev[0:8], prev[8:16], prev[16:24], prev[24:32])
        res = []
        for cur, pv in ((q0, qp), (q1, q0)):
            res.append(jnp.concatenate([cur[0] - pv[1], cur[1] + pv[0]], axis=0))
            res.append(jnp.concatenate([cur[2] - pv[3], cur[3] + pv[2]], axis=0))
        return res

    def stage_d(c, t, eo):
        for b in range(2):
            for par in range(2):
                w = jnp.concatenate([e[2 * b + par] for e in eo], axis=0).astype(BF16)
                g = cst_v[2 * C + 64 * par:2 * C + 64 * (par + 1), :]
                y = jnp.dot(g, w, preferred_element_type=F32)
                ybuf[c, t, pl.ds(b * C + par, 64, stride=2), :] = y

    def _ln(x):
        m = jnp.sum(x, axis=-1, keepdims=True) * (1.0 / D)
        xc = x - m
        var = jnp.sum(xc * xc, axis=-1, keepdims=True) * (1.0 / D)
        return xc * lax.rsqrt(var + EPS)

    def stage_e(c, g):
        rows = slice(16 * g, 16 * g + 16)
        x = q_v[c, rows, :].astype(F32).reshape(2, 8, D)
        y = jnp.concatenate([ybuf[c, t, rows, :] for t in range(LT)], axis=1).reshape(2, 8, D)
        x1 = x + (_ln(x) * modv[0][None] + modv[1][None]) * y
        h2 = _ln(x1) * modv[2][None] + modv[3][None]
        x1buf[c, rows, :] = x1.reshape(16, D)
        h2buf[c, rows, :] = h2.reshape(16, D)
        return h2.reshape(16, D)[:, 0:128]

    def mod_lhs():
        cf = c_v[...].astype(F32)
        sc = cf * (1.0 / (1.0 + jnp.exp(-cf)))
        return jnp.broadcast_to(sc, (16, D)).astype(BF16)

    def compute_mod_a():
        mod = jnp.dot(mod_lhs(), wm_v[:, 0:5 * D], preferred_element_type=F32)[0:8]
        sa, ca, ga, sb, cb = [mod[:, n * D:(n + 1) * D] for n in range(5)]
        modv[0] = ga * (1.0 + ca)
        modv[1] = ga * sa
        modv[2] = 1.0 + cb
        modv[3] = sb

    def compute_mod_b():
        modv[4] = jnp.dot(mod_lhs(), wm_v[:, 5 * D:6 * D], preferred_element_type=F32)[0:8]

    def conv_all(c):
        for t in range(LT):
            stage_b(c, t)
            stage_a(c, t)
        idx = lag_idx(c, c, c)
        for t in range(LT):
            stage_d(c, t, [cone(c, idx, t, u) for u in range(8)])

    def step(s, smin, smax, do_conv=True, do_e=True, first=False):
        if do_conv:
            idx = lag_idx(s + 1, smin + 1, smax + 1)
        par = s % 2
        items = [[] for _ in range(40)]
        ab_slots, c_slots, e_slots = AB_SLOTS, C_SLOTS, E_SLOTS
        if first:
            ab_slots, c_slots, e_slots = (16,) * 5, C1_SLOTS, E1_SLOTS
            items[8].append(("w", "w2"))
            items[16].append(("w", "c2"))
            items[24].append(("w", "wd1"))
            items[30].append(("w", "wd2"))
        if do_conv:
            for t in range(LT):
                items[D_SLOTS[t]].append(("d", t))
            for t in range(LT):
                items[ab_slots[t]].append(("ab", t))
            for p in range(40):
                assert ab_slots[p // 8] <= c_slots[p] < D_SLOTS[p // 8]
                items[c_slots[p]].append(("c", p))
        if first:
            items[16].append(("w", "w3"))
        if do_e:
            for g in range(16):
                items[e_slots[g]].append(("e", g))
        eo = {}

        def run_items(m, ref, nrows, dstride, col):
            npin = 0
            for kind, p in items[m]:
                if kind == "w":
                    wait(p)
                    if p == "wd1":
                        compute_mod_b()
                elif kind == "ab":
                    stage_b(s + 1, p)
                    stage_a(s + 1, p)
                elif kind == "d":
                    stage_d(s + 1, p, [eo[8 * p + u] for u in range(8)])
                else:
                    if kind == "c":
                        eo[p] = cone(s + 1, idx, p // 8, p % 8)
                        val = eo[p][2]
                    else:
                        val = stage_e(s, p)
                    assert npin < 4
                    ref[pl.ds(_mo(nrows + 64 * par + 16 * npin, 16), 16), _ls(col)] = val.astype(BF16)
                    npin += 1

        h = h2buf[s - 1].astype(BF16)
        hh = []
        for n in range(NT):
            run_items(2 * n, wg_v, D, 16, n)
            g = jnp.dot(h, wg_v[0:D, _ls(n)], preferred_element_type=F32)
            run_items(2 * n + 1, wu_v, D, 16, n)
            u = jnp.dot(h, wu_v[0:D, _ls(n)], preferred_element_type=F32)
            hh.append(g * u)
        hh = [jnp.concatenate(hh[4 * kc:4 * kc + 4], axis=1).astype(BF16) for kc in range(3)]
        for n in range(LT):
            o = None
            for kc, w in enumerate((wd0, wd1, wd2)):
                run_items(24 + 3 * n + kc, w, 512, 64, n)
                p = jnp.dot(hh[kc], w[0:512, _ls(n)], preferred_element_type=F32)
                o = p if o is None else o + p
            res = x1buf[s - 1, :, _ls(n)].reshape(32, 8, 128) + o.reshape(32, 8, 128) * modv[4, :, _ls(n)][None]
            o_v[s - 1, :, _ls(n)] = res.reshape(M, 128).astype(BF16)
        out_copy(s - 1).start()
        run_items(39, None, 0, 0, 0)

    one = jnp.minimum(pl.program_id(0), 0) + 1

    def dyn_step(s, **kw):
        def body(t, carry):
            with jax.named_scope("step%d" % s):
                step(t + s, s, s, **kw)
            return carry
        lax.fori_loop(0, one, body, 0)

    wait("c0")
    with jax.named_scope("conv0"):
        conv_all(0)
    wait("c1")
    with jax.named_scope("conv1"):
        conv_all(1)
    wait("wma")
    with jax.named_scope("mod_e0"):
        compute_mod_a()
        for g in range(16):
            stage_e(0, g)
    wait("w1")
    dyn_step(1, first=True)
    wait("c3")

    def body(s, carry):
        @pl.when(s == 3)
        def _():
            wait("rest")
        with jax.named_scope("step"):
            step(s, 2, 6)
        return carry
    lax.fori_loop(2, 7, body, 0)
    dyn_step(7, do_conv=False)
    dyn_step(8, do_conv=False, do_e=False)

    with jax.named_scope("wait_out"):
        for i in range(NC):
            out_copy(i).wait()


@jax.jit
def pallas_adaLN_cond__ssm_conv_h3__glu_gated_bilinear__prompt_kernel(A_q, A_k, A_v, A_shift_k, A_ssm_k, A_ssm_D, B_x, B_w_gate, B_w_up, B_w_down, c, w_mod):
    cst = jnp.asarray(_dft_consts(), dtype=BF16)
    any_spec = pl.BlockSpec(memory_space=pl.ANY)
    out = pl.pallas_call(
        _kernel,
        grid=(1,),
        in_specs=[any_spec] * 12,
        out_specs=any_spec,
        out_shape=jax.ShapeDtypeStruct((NC, M, D), BF16),
        scratch_shapes=[
            pltpu.VMEM((NC, M, D), BF16), pltpu.VMEM((NC, M, D), BF16), pltpu.VMEM((NC, M, D), BF16),
            pltpu.VMEM((D, S), BF16),
            pltpu.VMEM((D + 128, FF), BF16), pltpu.VMEM((D + 128, FF), BF16),
            pltpu.VMEM((512 + 128, D), BF16), pltpu.VMEM((512 + 128, D), BF16), pltpu.VMEM((512 + 128, D), BF16),
            pltpu.VMEM((D, 6 * D), BF16),
            pltpu.VMEM((3 * C, C), BF16),
            pltpu.VMEM((NC, M, D), BF16),
            pltpu.VMEM((LT, 32 + S, 128), F32),
            pltpu.VMEM((NB + 1, LT, 16, 24, 128), F32),
            pltpu.VMEM((NB, LT, 16, 24, 128), F32),
            pltpu.VMEM((NC + 1, LT, 8, 32, 128), F32),
            pltpu.VMEM((NC, LT, M, 128), F32),
            pltpu.VMEM((NC, M, D), F32),
            pltpu.VMEM((NC, M, D), F32),
            pltpu.VMEM((8, 8, D), F32),
            pltpu.VMEM((4, 8, D), F32),
            pltpu.VMEM((4, D), BF16), pltpu.VMEM((D,), BF16), pltpu.VMEM((1, D), BF16),
            pltpu.VMEM((14, 1, 128), F32),
            pltpu.SemaphoreType.DMA((NSEM,)),
            pltpu.SemaphoreType.DMA((NC,)),
        ],
        compiler_params=pltpu.CompilerParams(vmem_limit_bytes=120 * 1024 * 1024),
        name="fused_h3_glu",
    )(A_q.reshape(NC, M, D), A_k.reshape(NC, M, D), A_v.reshape(NC, M, D), A_shift_k.T, A_ssm_k, A_ssm_D,
      B_w_gate, B_w_up, B_w_down, c, w_mod, cst)
    return out.reshape(1, S, D)
```

```python
import numpy as np
import jax
import jax.numpy as jnp
from jax import lax
import jax.experimental.pallas as pl
import jax.experimental.pallas.tpu as pltpu

S, D, FF = 2048, 640, 1536
C = 128
NB = S // C
M = 256
NC = S // M
LT = D // 128
NT = FF // 128
EPS = 1e-5
F32 = jnp.float32
BF16 = jnp.bfloat16
U32 = jnp.uint32


def _dft_consts():
    r = np.arange(C)
    theta = np.pi * (4 * r + 1) / (2 * C)
    c = np.arange(C)
    ang = theta[:, None] * c[None, :]
    cs = np.stack([np.cos(ang), -np.sin(ang)], axis=0)
    fm = cs.reshape(2, 2, 8, 8, C).transpose(2, 1, 0, 3, 4).reshape(2 * C, C)
    a = np.concatenate([np.arange(0, C, 2), np.arange(1, C, 2)])
    ang2 = a[:, None] * theta[None, :64]
    g = np.zeros((C, 8, 2, 8))
    g[:, :, 0] = np.cos(ang2).reshape(C, 8, 8) / C
    g[:, :, 1] = -np.sin(ang2).reshape(C, 8, 8) / C
    g = g.reshape(C, C)
    return np.concatenate([fm, g], axis=0).astype(np.float32)


E_SLOTS = (92, 96, 97, 97, 98, 99, 100, 102, 103, 104, 106, 107, 108, 110, 111, 111)
AB_SLOTS = (0, 0, 0, 0, 0)
C_SLOTS = tuple(range(40, 80))
D_SLOT = 80
E1_SLOTS = (28, 29, 33, 34, 35, 36, 37, 38)
NSEM = 11
USE_EA = True
E_TIE = (None, 82, 86, 90, 94, 96, 96, 97, 98, 99, 101, 102, 103, 105, 106, 107)
TIE_N = 1
EA_SLOTS = tuple(range(2, 34, 2))
SPLIT = False
E_PIN = True


def _mo(x, m):
    return x if isinstance(x, int) else pl.multiple_of(x, m)


def _ls(t):
    return slice(t * 128, (t + 1) * 128)


def _kernel(q_h, k_h, v_h, sh_h, sk_h, sd_h, wg_h, wu_h, wd_h, c_h, wm_h, cst_h,
            o_h,
            q_v, k_v, v_v, sk_v, wg_v, wu_v, wd0, wd1, wd2, wm_v, cst_v,
            o_v, kbuf, xf, kf, qbuf, ybuf, x1buf, h2buf, lhsb, wgu, wdn, dlb, dl5, wbuf, modv, shb, zm, sh_v, sd_v, c_v, pad_v,
            sem_in, sem_out):
    def cp(src, dst):
        return (src, dst)

    def conv_in(c0, c1):
        cols = pl.ds(c0 * M, (c1 - c0) * M)
        return [cp(sk_h.at[:, cols], sk_v.at[:, cols]), cp(k_h.at[c0:c1], k_v.at[c0:c1]),
                cp(v_h.at[c0:c1], v_v.at[c0:c1])]

    def q_in(c0, c1):
        return [cp(q_h.at[c0:c1], q_v.at[c0:c1])]

    def gu_in(n0, n1):
        cols = pl.ds(n0 * 128, (n1 - n0) * 128)
        return [cp(wg_h.at[:, cols], wg_v.at[0:D, cols]), cp(wu_h.at[:, cols], wu_v.at[0:D, cols])]

    def wd_in(n0, n1):
        cols = pl.ds(n0 * 128, (n1 - n0) * 128)
        return [cp(wd_h.at[kc * 512:(kc + 1) * 512, cols], w.at[0:512, cols])
                for kc, w in enumerate((wd0, wd1, wd2))]

    dma = dict(
        small=[cp(cst_h, cst_v), cp(sh_h, sh_v), cp(sd_h, sd_v), cp(c_h, c_v)],
        c0=conv_in(0, 1),
        wma=[cp(wm_h.at[:, 0:5 * D], wm_v.at[:, 0:5 * D])] + q_in(0, 1),
        w1=gu_in(0, 4),
        w2=gu_in(4, 8),
        c1=conv_in(1, 2),
        w3=gu_in(8, 12),
        wd1=q_in(1, 2) + [cp(wm_h.at[:, 5 * D:6 * D], wm_v.at[:, 5 * D:6 * D])] + wd_in(0, 2),
        wd2=wd_in(2, 5),
        c2=conv_in(2, 3) + q_in(2, 3),
        rest=conv_in(3, 8) + q_in(3, 8),
    )
    assert len(dma) == NSEM
    dma = {name: [pltpu.make_async_copy(a, b, sem_in.at[n]) for a, b in grp]
           for n, (name, grp) in enumerate(dma.items())}

    def wait(name):
        with jax.named_scope("w_" + name):
            for c_ in dma[name]:
                c_.wait()

    def out_copy(i):
        return pltpu.make_async_copy(o_v.at[i], o_h.at[i], sem_out)

    for grp in dma.values():
        for c_ in grp:
            c_.start()

    for t in range(LT):
        kbuf[t, 24:32, :] = jnp.zeros((8, 128), F32)
    xf[0] = jnp.zeros((LT, 16, 24, 128), F32)
    qbuf[0] = jnp.zeros((LT, 8, 32, 128), F32)
    pad_v[...] = jnp.zeros(pad_v.shape, F32)
    zm[...] = jnp.zeros((8, 128), jnp.int32)
    wait('small')
    sh = sh_v[...].astype(F32)
    for j in range(4):
        shb[j] = jnp.broadcast_to(sh[j:j + 1, :], (8, D))

    def stage_a(c, t):
        r0 = _mo(c * M, M)
        ls = _ls(t)
        kk = k_v[c, :, ls].astype(F32)
        kbuf[t, pl.ds(r0 + 32, M), :] = kk
        acc = kk.reshape(32, 8, 128) * shb[0, :, ls][None]
        for j in range(1, 4):
            acc = acc + kbuf[t, pl.ds(r0 + 32 - j, M), :].reshape(32, 8, 128) * shb[j, :, ls][None]
        kv = acc.reshape(M, 128) * v_v[c, :, ls].astype(F32)
        for b in range(2):
            r = jnp.dot(cst_v[0:2 * C, :], kv[b * C:(b + 1) * C].astype(BF16),
                        preferred_element_type=F32).reshape(16, 16, 128)
            xf[2 * c + 1 + b, t, :, 0:16, :] = r
            xf[2 * c + 1 + b, t, :, 16:24, :] = r[:, 0:8, :] + r[:, 8:16, :]

    def stage_b(c, t):
        for b in range(2):
            kb = sk_v[_ls(t), pl.ds(_mo(c * M + b * C, C), C)]
            r = lax.dot_general(cst_v[0:2 * C, :], kb, (((1,), (1,)), ((), ())),
                                preferred_element_type=F32).reshape(16, 16, 128)
            cc = r[:, 0:8, :]
            d = r[:, 8:16, :]
            if isinstance(c, int) and c == 0 and b == 0:
                cc = cc + sd_v[...].astype(F32).reshape(1, 1, D)[:, :, _ls(t)]
            kf[2 * c + b, t, :, 0:8, :] = d - cc
            kf[2 * c + b, t, :, 8:16, :] = cc + d
            kf[2 * c + b, t, :, 16:24, :] = cc

    def lag_idx(c, cmin, cmax):
        nlag = 2 * cmax + 2
        jok = 2 * cmin + 1
        kidx = [j if j <= jok else jnp.minimum(j, 2 * c + 1) for j in range(nlag)]
        xidx = [2 * c + 2 - j if j <= jok + 1 else jnp.maximum(2 * c + 2 - j, 0) for j in range(nlag)]
        return kidx, xidx

    def _reim_eo(acc):
        re = acc[:, 16:24] - acc[:, 8:16]
        im = acc[:, 16:24] + acc[:, 0:8]
        return re[0] + re[1], im[0] + im[1], re[0] - re[1], im[0] - im[1]

    def cone(c, idx, t, u):
        kidx, xidx = idx
        nlag = len(kidx)
        us = slice(2 * u, 2 * u + 2)
        x = None
        acc0 = acc1 = None
        for j in reversed(range(nlag)):
            k = kf[kidx[j], t, us]
            if x is not None:
                p = k * x
                acc0 = p if acc0 is None else acc0 + p
            x = xf[xidx[j], t, us]
            p = k * x
            acc1 = p if acc1 is None else acc1 + p
        q0 = _reim_eo(acc0)
        q1 = _reim_eo(acc1)
        qv = qbuf.at[pl.ds(c, 2)]
        qv[1, t, u] = jnp.concatenate(q1, axis=0)
        prev = qv[0, t, u]
        qp = (prev[0:8], prev[8:16], prev[16:24], prev[24:32])
        res = []
        for cur, pv in ((q0, qp), (q1, q0)):
            res.append(jnp.concatenate([cur[0] - pv[1], cur[1] + pv[0]], axis=0))
            res.append(jnp.concatenate([cur[2] - pv[3], cur[3] + pv[2]], axis=0))
        return res

    def stage_d(c, t, wfn):
        for b in range(2):
            for par in range(2):
                g = cst_v[2 * C + 64 * par:2 * C + 64 * (par + 1), :]
                y = jnp.dot(g, wfn(2 * b + par), preferred_element_type=F32)
                ybuf[t, pl.ds(b * C + par, 64, stride=2), :] = y

    def wfn_vals(eo):
        return lambda n: jnp.concatenate([e[n] for e in eo], axis=0).astype(BF16)

    def pack(x):
        return pltpu.bitcast(x.astype(BF16), U32)

    def asums(a11, a12, a21, a22):
        return [a11 + a22, a21 + a22, a11, a22, a11 + a12, a21 - a11, a12 - a22]

    def bsums(b11, b12, b21, b22):
        return [b11 + b22, b11, b12 - b22, b21 - b11, b22, b11 + b12, b21 + b22]

    def _ln(x):
        m = jnp.sum(x, axis=-1, keepdims=True) * (1.0 / D)
        xc = x - m
        var = jnp.sum(xc * xc, axis=-1, keepdims=True) * (1.0 / D)
        return xc * lax.rsqrt(var + EPS)

    def e1_rows(c, r0):
        rows = slice(r0, r0 + 16)
        x = q_v[c, rows, :].astype(F32).reshape(2, 8, D)
        w = (_ln(x) * modv[0][None] + modv[1][None]).reshape(16, D)
        wbuf[rows, :] = w
        return w[:, 0:128]

    def e_rows(c, r0, have_w=False, tie=None):
        rows = slice(r0, r0 + 16)
        x = q_v[c, rows, :].astype(F32).reshape(2, 8, D)
        if tie is not None:
            never = (zm[...] != 0)[None]
            x = jnp.concatenate([jnp.where(never, tie.reshape(2, 8, 128), x[:, :, _ls(t)]) if t < TIE_N
                                 else x[:, :, _ls(t)] for t in range(LT)], axis=2)
        y = jnp.concatenate([ybuf[t, rows, :] for t in range(LT)], axis=1).reshape(2, 8, D)
        if have_w:
            w = wbuf[rows, :].reshape(2, 8, D)
        else:
            w = _ln(x) * modv[0][None] + modv[1][None]
        x1 = x + w * y
        h2 = _ln(x1) * modv[2][None] + modv[3][None]
        x1buf.at[pl.ds(c, 2)][1, rows, :] = x1.reshape(16, D)
        return h2.reshape(16, D)

    def stage_e(c, g, dst, top=None, tie=None):
        bot = e_rows(c, C + 16 * g, top is not None and USE_EA, tie)
        if top is None:
            top = e_rows(c, 16 * g)
        rows = slice(64 + 8 * g, 64 + 8 * g + 8)
        for kt in range(2):
            ss = asums(top[:, _ls(kt)], top[:, _ls(2 + kt)], bot[:, _ls(kt)], bot[:, _ls(2 + kt)])
            for i in range(7):
                dst[rows, _ls(2 * i + kt)] = pack(ss[i])
        dst[rows, _ls(14)] = pack(top[:, _ls(4)])
        dst[rows, _ls(15)] = pack(bot[:, _ls(4)])
        return ss[0]

    def lhs_view(s):
        return lhsb.at[pl.ds(pl.multiple_of((s - 1) * 64, 64), 128)]

    def prep_gu(mat, p):
        w = (wg_v, wu_v)[mat]
        base = (2 * p + mat) * 8
        for rc in range(8):
            r = slice(32 * rc, 32 * rc + 32)
            r2 = slice(256 + 32 * rc, 256 + 32 * rc + 32)
            cols = slice(256 * p, 256 * p + 256)
            hi = w[r, cols].astype(F32)
            lo = w[r2, cols].astype(F32)
            bs = bsums(hi[:, 0:128], hi[:, 128:256], lo[:, 0:128], lo[:, 128:256])
            for i in range(7):
                wgu[16 * rc:16 * rc + 16, _ls(base + i)] = pack(bs[i])
        for cc in range(2):
            wgu[64 * cc:64 * cc + 64, _ls(base + 7)] = pltpu.bitcast(w[512:640, _ls(2 * p + cc)], U32)

    def prep_dn(pp):
        for p in range(6):
            w = (wd0, wd1, wd2)[p // 2]
            r0 = 256 * (p % 2)
            if pp == 2:
                for r in range(2):
                    wdn[64 * p:64 * p + 64, _ls(14 + r)] = pltpu.bitcast(
                        w[r0 + 128 * r:r0 + 128 * r + 128, _ls(4)], U32)
                continue
            cols = slice(256 * pp, 256 * pp + 256)
            for rc in range(4):
                hi = w[r0 + 32 * rc:r0 + 32 * rc + 32, cols].astype(F32)
                lo = w[r0 + 128 + 32 * rc:r0 + 128 + 32 * rc + 32, cols].astype(F32)
                bs = bsums(hi[:, 0:128], hi[:, 128:256], lo[:, 0:128], lo[:, 128:256])
                for i in range(7):
                    wdn[64 * p + 16 * rc:64 * p + 16 * rc + 16, _ls(pp * 7 + i)] = pack(bs[i])

    def mod_lhs():
        cf = c_v[...].astype(F32)
        sc = cf * (1.0 / (1.0 + jnp.exp(-cf)))
        return jnp.broadcast_to(sc, (16, D)).astype(BF16)

    def compute_mod_a():
        mod = jnp.dot(mod_lhs(), wm_v[:, 0:5 * D], preferred_element_type=F32)[0:8]
        sa, ca, ga, sb, cb = [mod[:, n * D:(n + 1) * D] for n in range(5)]
        modv[0] = ga * (1.0 + ca)
        modv[1] = ga * sa
        modv[2] = 1.0 + cb
        modv[3] = sb

    def compute_mod_b():
        modv[4] = jnp.dot(mod_lhs(), wm_v[:, 5 * D:6 * D], preferred_element_type=F32)[0:8]

    def conv_all(c):
        for t in range(LT):
            stage_b(c, t)
            stage_a(c, t)
        idx = lag_idx(c, c, c)
        for t in range(LT):
            stage_d(c, t, wfn_vals([cone(c, idx, t, u) for u in range(8)]))

    def first_step(s):
        idx = lag_idx(s, 1, 1)
        par = s % 2
        items = [[] for _ in range(40)]
        items[8].append(("w", "w2"))
        items[16].append(("w", "c1"))
        for t in range(LT):
            items[24].append(("d", t))
            items[16].append(("ab", t))
        items[16].append(("w", "w3"))
        items[24].append(("w", "wd1"))
        items[30].append(("w", "wd2"))
        for p in range(6):
            items[8 * (p // 2)].append(("pgu", p))
        items[24].append(("pdn", 0))
        items[30].append(("pdn", 1))
        items[30].append(("pdn", 2))
        for p in range(40):
            items[19 + p // 8].append(("c", p))
        for g in range(8):
            items[E1_SLOTS[g]].append(("e", g))
        eo = {}

        def run_items(m, ref, nrows, col):
            npin = 0
            for kind, p in items[m]:
                if kind == "w":
                    wait(p)
                    if p == "wd1":
                        compute_mod_b()
                elif kind == "pgu":
                    prep_gu(0, p)
                    prep_gu(1, p)
                elif kind == "pdn":
                    prep_dn(p)
                elif kind == "ab":
                    stage_b(s, p)
                    stage_a(s, p)
                elif kind == "d":
                    stage_d(s, p, wfn_vals([eo[8 * p + u] for u in range(8)]))
                else:
                    if kind == "c":
                        eo[p] = cone(s, idx, p // 8, p % 8)
                        val = eo[p][2]
                    else:
                        val = stage_e(s, p, lhs_view(s))
                    assert npin < 8
                    ref[pl.ds(_mo(nrows + 128 * par + 16 * npin, 16), 16), _ls(col)] = val.astype(BF16)
                    npin += 1

        h = h2buf[...].astype(BF16)
        hh = []
        for n in range(NT):
            run_items(2 * n, wg_v, D, n)
            g = jnp.dot(h, wg_v[0:D, _ls(n)], preferred_element_type=F32)
            run_items(2 * n + 1, wu_v, D, n)
            u = jnp.dot(h, wu_v[0:D, _ls(n)], preferred_element_type=F32)
            hh.append(g * u)
        hh = [jnp.concatenate(hh[4 * kc:4 * kc + 4], axis=1).astype(BF16) for kc in range(3)]
        for n in range(LT):
            o = None
            for kc, w in enumerate((wd0, wd1, wd2)):
                run_items(24 + 3 * n + kc, w, 512, n)
                p = jnp.dot(hh[kc], w[0:512, _ls(n)], preferred_element_type=F32)
                o = p if o is None else o + p
            res = x1buf.at[pl.ds(s, 2)][0, :, _ls(n)].reshape(32, 8, 128) + o.reshape(32, 8, 128) * modv[4, :, _ls(n)][None]
            o_v[s - 1, :, _ls(n)] = res.reshape(M, 128).astype(BF16)
        out_copy(s - 1).start()

    def step(s, smin, smax, do_conv=True):
        if do_conv:
            idx = lag_idx(s, smin, smax)
        off = 32 * (s % 2)
        lv = lhs_view(s)
        zw = s % 2
        zr = (s + 2) % 2
        dl_w = dlb.at[pl.ds(pl.multiple_of(zw * 64, 64), 64)]
        dl_r = dlb.at[pl.ds(pl.multiple_of(zr * 64, 64), 64)]

        def hold(x):
            return lambda: x
        items = [[] for _ in range(113)]
        if do_conv:
            for t in range(LT):
                items[AB_SLOTS[t]].append(("ab", t))
            for p in range(40):
                items[C_SLOTS[p]].append(("c", p))
            items[D_SLOT].append(("d", 0))
            for g in range(16):
                items[E_SLOTS[g]].append(("e", g))
                if USE_EA:
                    items[EA_SLOTS[g]].append(("ea", g))
        tops = {}
        hist = {}

        def tie_of(p):
            if E_TIE is None or E_TIE[p] is None:
                return None
            return hist[E_TIE[p]][112:128]
        where = {}
        slot = [0]

        def pin_rows(nrows, n):
            return pl.ds(_mo(nrows + off + 8 * n, 8), 8)

        def run_d():
            for t in range(LT):
                def wfn(n):
                    parts = []
                    for u in range(8):
                        ref, nrows, col = where[8 * t + u]
                        parts.append(ref[pin_rows(nrows, n), _ls(col)])
                    return pltpu.bitcast(jnp.concatenate(parts, axis=0), BF16)
                stage_d(s, t, wfn)

        def hook(ref, nrows, col):
            m = slot[0]
            slot[0] += 1
            npin = 0
            for kind, p in items[m]:
                if kind == "ab":
                    stage_b(s, p)
                    stage_a(s, p)
                    continue
                if kind == "d":
                    run_d()
                    if SPLIT:
                        out_copy(s - 2).wait()
                    continue
                if kind == "c":
                    assert npin == 0
                    res = cone(s, idx, p // 8, p % 8)
                    for n in range(4):
                        ref[pin_rows(nrows, n), _ls(col)] = pack(res[n])
                    where[p] = (ref, nrows, col)
                else:
                    if kind == "ea":
                        val = e1_rows(s, 16 * p)
                    elif p % 2 == 0:
                        tops[p // 2] = e_rows(s, 8 * p, USE_EA, tie_of(p))
                        val = tops[p // 2][:, _ls(4)]
                    else:
                        val = stage_e(s, p // 2, lv, tops[p // 2], tie_of(p))
                    if E_PIN:
                        assert npin < 4
                        ref[pin_rows(nrows, npin), _ls(col)] = pack(val)
                npin += 1

        def dot(a, w):
            r = jnp.dot(a, pltpu.bitcast(w, BF16), preferred_element_type=F32)
            hist.setdefault(slot[0] - 1, r)
            return r

        def strassen(lhs, ref, nrows, base, left):
            def m(i):
                hook(ref, nrows, base + i - 1)
                return dot(lhs(i - 1), ref[0:nrows, _ls(base + i - 1)])
            m2 = m(2)
            m4 = m(4)
            c21 = m2 + m4
            if left is not None:
                c21 = hold(c21)
            m2 = hold(m2)
            m4 = hold(m4)
            m3 = m(3)
            m5 = m(5)
            c12 = m3 + m5
            if left is not None:
                c12 = hold(c12)
            c11 = hold(m4() - m5)
            c22 = hold(m3 - m2())
            m1 = m(1)
            m7 = m(7)
            c11 = c11() + m1 + m7
            if left is not None:
                c11 = hold(c11)
            c22 = hold(c22() + m1)
            c22 = c22() + m(6)
            if left is not None:
                hook(ref, nrows, base + 7)
                c22 = c22 + left(1, 1)
                c11 = c11() + left(0, 0)
                c12 = c12() + left(0, 1)
                c21 = c21() + left(1, 0)
            return c11, c12, c21, c22

        def lhs1(i):
            return pltpu.bitcast(lv[0:64, 256 * i:256 * i + 256], BF16)

        for p in range(6):
            res = []
            for mat in range(2):
                base = (2 * p + mat) * 8
                res.append(strassen(
                    lhs1, wgu, 128, base,
                    lambda r, c: dot(pltpu.bitcast(lv[0:64, _ls(14 + r)], BF16),
                                     wgu[64 * c:64 * c + 64, _ls(base + 7)])))
                if mat == 0:
                    res[0] = [hold(x) for x in res[0]]
            hq = [res[0][i]() * res[1][i] for i in range(4)]
            for i, x in enumerate(asums(*hq) + [hq[1], hq[2]]):
                if p < 5:
                    dl_w[:, _ls(6 * i + p)] = pack(x)
                else:
                    dl5[:, _ls(i)] = pack(x)
        dla = [dl_r[:, 768 * i:768 * i + 640] for i in range(9)]
        dlz = [dl5[:, _ls(i)] for i in range(9)]
        dl = [pltpu.bitcast(jnp.concatenate([dla[i], dlz[i]], axis=1), BF16) for i in range(9)]

        def emit(r, n, o):
            rows = slice(r * C, (r + 1) * C)
            res = x1buf.at[pl.ds(s, 2)][0, rows, _ls(n)].reshape(16, 8, 128) + o.reshape(16, 8, 128) * modv[4, :, _ls(n)][None]
            o_v[s - 1, rows, _ls(n)] = res.reshape(C, 128).astype(BF16)

        hook(wdn, 384, 14)
        ta = dot(pltpu.bitcast(dla[2], BF16), wdn[0:320, _ls(14)])
        tb = dot(pltpu.bitcast(dla[8], BF16), wdn[0:320, _ls(14)])
        ta = ta + dot(pltpu.bitcast(dlz[2], BF16), wdn[320:384, _ls(14)])
        tb = tb + dot(pltpu.bitcast(dlz[8], BF16), wdn[320:384, _ls(14)])
        hook(wdn, 384, 15)
        emit(0, 4, ta + dot(dl[7], wdn[0:384, _ls(15)]))
        emit(1, 4, tb + dot(dl[3], wdn[0:384, _ls(15)]))
        for pp in range(2):
            cs = strassen(lambda i: dl[i], wdn, 384, 7 * pp, None)
            for i in range(4):
                emit(i // 2, 2 * pp + i % 2, cs[i])
        out_copy(s - 1).start()

    one = jnp.minimum(pl.program_id(0), 0) + 1

    def dyn_step(s, **kw):
        def body(t, carry):
            with jax.named_scope("step%d" % s):
                if s == 1:
                    first_step(t + s)
                else:
                    step(t + s, s, s, **kw)
            return carry
        lax.fori_loop(0, one, body, 0)

    wait("c0")
    with jax.named_scope("conv0"):
        conv_all(0)
    wait("wma")
    with jax.named_scope("mod_e0"):
        compute_mod_a()
        for g in range(16):
            h2buf[16 * g:16 * g + 16, :] = e_rows(0, 16 * g)
    wait("w1")
    dyn_step(1)
    wait("c2")

    def body(s, carry):
        @pl.when(s == 3)
        def _():
            wait("rest")
        with jax.named_scope("step"):
            step(s, 2, 7)
        return carry
    lax.fori_loop(2, 8, body, 0)
    dyn_step(8, do_conv=False)

    with jax.named_scope("wait_out"):
        for i in range(NC - 2 if SPLIT else 0, NC):
            out_copy(i).wait()


@jax.jit
def pallas_adaLN_cond__ssm_conv_h3__glu_gated_bilinear__prompt_kernel(A_q, A_k, A_v, A_shift_k, A_ssm_k, A_ssm_D, B_x, B_w_gate, B_w_up, B_w_down, c, w_mod):
    cst = jnp.asarray(_dft_consts(), dtype=BF16)
    any_spec = pl.BlockSpec(memory_space=pl.ANY)
    out = pl.pallas_call(
        _kernel,
        grid=(1,),
        in_specs=[any_spec] * 12,
        out_specs=any_spec,
        out_shape=jax.ShapeDtypeStruct((NC, M, D), BF16),
        scratch_shapes=[
            pltpu.VMEM((NC, M, D), BF16), pltpu.VMEM((NC, M, D), BF16), pltpu.VMEM((NC, M, D), BF16),
            pltpu.VMEM((D, S), BF16),
            pltpu.VMEM((D + 256, FF), BF16), pltpu.VMEM((D + 256, FF), BF16),
            pltpu.VMEM((512 + 256, D), BF16), pltpu.VMEM((512 + 256, D), BF16), pltpu.VMEM((512 + 256, D), BF16),
            pltpu.VMEM((D, 6 * D), BF16),
            pltpu.VMEM((3 * C, C), BF16),
            pltpu.VMEM((NC, M, D), BF16),
            pltpu.VMEM((LT, 32 + S, 128), F32),
            pltpu.VMEM((NB + 1, LT, 16, 24, 128), F32),
            pltpu.VMEM((NB, LT, 16, 24, 128), F32),
            pltpu.VMEM((NC + 1, LT, 8, 32, 128), F32),
            pltpu.VMEM((LT, M, 128), F32),
            pltpu.VMEM((NC + 2, M, D), F32),
            pltpu.VMEM((M, D), F32),
            pltpu.VMEM(((NC + 1) * 64, 16 * 128), U32),
            pltpu.VMEM((128 + 64, 96 * 128), U32),
            pltpu.VMEM((384 + 64, 16 * 128), U32),
            pltpu.VMEM((2 * 64, 9 * 768), U32),
            pltpu.VMEM((64, 9 * 128), U32),
            pltpu.VMEM((M, D), F32),
            pltpu.VMEM((8, 8, D), F32),
            pltpu.VMEM((4, 8, D), F32),
            pltpu.VMEM((8, 128), jnp.int32),
            pltpu.VMEM((4, D), BF16), pltpu.VMEM((D,), BF16), pltpu.VMEM((1, D), BF16),
            pltpu.VMEM((6, 1, 128), F32),
            pltpu.SemaphoreType.DMA((NSEM,)),
            pltpu.SemaphoreType.DMA(()),
        ],
        compiler_params=pltpu.CompilerParams(vmem_limit_bytes=120 * 1024 * 1024),
        name="fused_h3_glu",
    )(A_q.reshape(NC, M, D), A_k.reshape(NC, M, D), A_v.reshape(NC, M, D), A_shift_k.T, A_ssm_k, A_ssm_D,
      B_w_gate, B_w_up, B_w_down, c, w_mod, cst)
    return out.reshape(1, S, D)
```

```python
import numpy as np
import jax
import jax.numpy as jnp
from jax import lax
import jax.experimental.pallas as pl
import jax.experimental.pallas.tpu as pltpu

S, D, FF = 2048, 640, 1536
C = 128
NB = S // C
M = 256
NC = S // M
LT = D // 128
EPS = 1e-5
F32 = jnp.float32
BF16 = jnp.bfloat16
U32 = jnp.uint32


def _dft_consts():
    r = np.arange(C)
    theta = np.pi * (4 * r + 1) / (2 * C)
    c = np.arange(C)
    ang = theta[:, None] * c[None, :]
    cs = np.stack([np.cos(ang), -np.sin(ang)], axis=0)
    fm = cs.reshape(2, 2, 8, 8, C).transpose(2, 1, 0, 3, 4).reshape(2 * C, C)
    a = np.concatenate([np.arange(0, C, 2), np.arange(1, C, 2)])
    ang2 = a[:, None] * theta[None, :64]
    g = np.zeros((C, 8, 2, 8))
    g[:, :, 0] = np.cos(ang2).reshape(C, 8, 8) / C
    g[:, :, 1] = -np.sin(ang2).reshape(C, 8, 8) / C
    g = g.reshape(C, C)
    return np.concatenate([fm, g], axis=0).astype(np.float32)


E_SLOTS = (92, 96, 97, 97, 98, 99, 100, 102, 103, 104, 106, 107, 108, 110, 111, 111)
E_TIE = (None, 82, 86, 90, 94, 96, 96, 97, 98, 99, 101, 102, 103, 105, 106, 107)
EA_SLOTS = tuple(range(2, 34, 2))
C_SLOTS = tuple(range(40, 80))
D_SLOT = 80
WC_SLOTS = tuple(range(54, 94))
W_WAITS = {0: ("p0",), 16: ("p1",), 32: ("p2",), 48: ("p3",), 96: ("wd",)}
W_AB = 40
W_D = 96
W_MOD = 97
WE_SLOTS = (98, 98, 99, 100, 101, 102, 103, 104, 105, 106, 107, 108, 109, 110, 111, 111)


def _mo(x, m):
    return x if isinstance(x, int) else pl.multiple_of(x, m)


def _ls(t):
    return slice(t * 128, (t + 1) * 128)


def _pack(x):
    return pltpu.bitcast(x.astype(BF16), U32)


def _asums(a11, a12, a21, a22):
    return [a11 + a22, a21 + a22, a11, a22, a11 + a12, a21 - a11, a12 - a22]


def _ln(x):
    m = jnp.sum(x, axis=-1, keepdims=True) * (1.0 / D)
    xc = x - m
    var = jnp.sum(xc * xc, axis=-1, keepdims=True) * (1.0 / D)
    return xc * lax.rsqrt(var + EPS)


def _kernel(q_h, k_h, v_h, sh_h, sk_h, sd_h, wg_h, wu_h, wd_h, c_h, wm_h, cst_h,
            o_h,
            q_v, k_v, v_v, sk_v, wg_v, wu_v, wd_v, wm_v, cst_v,
            o_v, kbuf, xf, kf, qbuf, ybuf, x1buf, lhsb, wgu, wdn, dlb, dl5, wbuf, modv, shb, zm,
            sh_v, sd_v, c_v, pad_v,
            sem_in, sem_out):
    def conv_in(c0, c1):
        cols = pl.ds(c0 * M, (c1 - c0) * M)
        return [(sk_h.at[:, cols], sk_v.at[:, cols]), (k_h.at[c0:c1], k_v.at[c0:c1]),
                (v_h.at[c0:c1], v_v.at[c0:c1])]

    def q_in(c0, c1):
        return [(q_h.at[c0:c1], q_v.at[c0:c1])]

    def gu_in(p0, p1):
        cols = pl.ds(p0 * 256, (p1 - p0) * 256)
        return [(wg_h.at[:, cols], wg_v.at[:, cols]), (wu_h.at[:, cols], wu_v.at[:, cols])]

    def wm_in(n0, n1):
        cols = pl.ds(n0 * D, (n1 - n0) * D)
        return [(wm_h.at[:, cols], wm_v.at[:, cols])]

    dma = dict(
        small=[(cst_h, cst_v), (sh_h, sh_v), (sd_h, sd_v), (c_h, c_v)],
        c0=conv_in(0, 1),
        c1=conv_in(1, 2),
        wm1=q_in(0, 2) + wm_in(0, 3),
        wm2=wm_in(3, 5),
        p0=gu_in(0, 1),
        p1=gu_in(1, 2),
        p2=gu_in(2, 3) + conv_in(2, 3),
        p3=gu_in(3, 6),
        wd=q_in(2, 3) + wm_in(5, 6) + [(wd_h, wd_v)],
        c3=conv_in(3, 4) + q_in(3, 4),
        rest=conv_in(4, 8) + q_in(4, 8),
    )
    dma = {name: [pltpu.make_async_copy(a, b, sem_in.at[n]) for a, b in grp]
           for n, (name, grp) in enumerate(dma.items())}

    def wait(name):
        with jax.named_scope("w_" + name):
            for cp in dma[name]:
                cp.wait()

    def out_copy(i, rows=slice(None), cols=slice(None)):
        return pltpu.make_async_copy(o_v.at[i, rows, cols], o_h.at[i, rows, cols], sem_out)

    last_parts = [(slice(None), _ls(4)), (slice(None), slice(0, 256)), (slice(C, M), _ls(2)),
                  (slice(0, C), _ls(3)), (slice(0, C), _ls(2)), (slice(C, M), _ls(3))]

    for grp in dma.values():
        for cp in grp:
            cp.start()

    for t in range(LT):
        kbuf[t, 24:32, :] = jnp.zeros((8, 128), F32)
    xf[0] = jnp.zeros((LT, 16, 24, 128), F32)
    qbuf[0] = jnp.zeros((LT, 8, 32, 128), F32)
    pad_v[...] = jnp.zeros(pad_v.shape, F32)
    zm[...] = jnp.zeros((8, 128), jnp.int32)
    wait("small")
    sh = sh_v[...].astype(F32)
    for j in range(4):
        shb[j] = jnp.broadcast_to(sh[j:j + 1, :], (8, D))

    def stage_a(c, t):
        r0 = _mo(c * M, M)
        ls = _ls(t)
        kk = k_v[c, :, ls].astype(F32)
        kbuf[t, pl.ds(r0 + 32, M), :] = kk
        acc = kk.reshape(32, 8, 128) * shb[0, :, ls][None]
        for j in range(1, 4):
            acc = acc + kbuf[t, pl.ds(r0 + 32 - j, M), :].reshape(32, 8, 128) * shb[j, :, ls][None]
        kv = acc.reshape(M, 128) * v_v[c, :, ls].astype(F32)
        for b in range(2):
            r = jnp.dot(cst_v[0:2 * C, :], kv[b * C:(b + 1) * C].astype(BF16),
                        preferred_element_type=F32).reshape(16, 16, 128)
            xf[2 * c + 1 + b, t, :, 0:16, :] = r
            xf[2 * c + 1 + b, t, :, 16:24, :] = r[:, 0:8, :] + r[:, 8:16, :]

    def stage_b(c, t):
        for b in range(2):
            kb = sk_v[_ls(t), pl.ds(_mo(c * M + b * C, C), C)]
            r = lax.dot_general(cst_v[0:2 * C, :], kb, (((1,), (1,)), ((), ())),
                                preferred_element_type=F32).reshape(16, 16, 128)
            cc = r[:, 0:8, :]
            d = r[:, 8:16, :]
            if isinstance(c, int) and c == 0 and b == 0:
                cc = cc + sd_v[...].astype(F32).reshape(1, 1, D)[:, :, _ls(t)]
            kf[2 * c + b, t, :, 0:8, :] = d - cc
            kf[2 * c + b, t, :, 8:16, :] = cc + d
            kf[2 * c + b, t, :, 16:24, :] = cc

    def lag_idx(c, cmin, cmax):
        nlag = 2 * cmax + 2
        jok = 2 * cmin + 1
        kidx = [j if j <= jok else jnp.minimum(j, 2 * c + 1) for j in range(nlag)]
        xidx = [2 * c + 2 - j if j <= jok + 1 else jnp.maximum(2 * c + 2 - j, 0) for j in range(nlag)]
        return kidx, xidx

    def reim_eo(acc):
        re = acc[:, 16:24] - acc[:, 8:16]
        im = acc[:, 16:24] + acc[:, 0:8]
        return re[0] + re[1], im[0] + im[1], re[0] - re[1], im[0] - im[1]

    def cone(c, idx, t, u):
        kidx, xidx = idx
        us = slice(2 * u, 2 * u + 2)
        x = None
        acc0 = acc1 = None
        for j in reversed(range(len(kidx))):
            k = kf[kidx[j], t, us]
            if x is not None:
                p = k * x
                acc0 = p if acc0 is None else acc0 + p
            x = xf[xidx[j], t, us]
            p = k * x
            acc1 = p if acc1 is None else acc1 + p
        q0 = reim_eo(acc0)
        q1 = reim_eo(acc1)
        qv = qbuf.at[pl.ds(c, 2)]
        qv[1, t, u] = jnp.concatenate(q1, axis=0)
        prev = qv[0, t, u]
        qp = (prev[0:8], prev[8:16], prev[16:24], prev[24:32])
        res = []
        for cur, pv in ((q0, qp), (q1, q0)):
            res.append(jnp.concatenate([cur[0] - pv[1], cur[1] + pv[0]], axis=0))
            res.append(jnp.concatenate([cur[2] - pv[3], cur[3] + pv[2]], axis=0))
        return res

    def stage_d(yi, t, wfn):
        for b in range(2):
            for par in range(2):
                g = cst_v[2 * C + 64 * par:2 * C + 64 * (par + 1), :]
                y = jnp.dot(g, wfn(2 * b + par), preferred_element_type=F32)
                ybuf[yi, t, pl.ds(b * C + par, 64, stride=2), :] = y

    def conv_all(c):
        for t in range(LT):
            stage_b(c, t)
            stage_a(c, t)
        idx = lag_idx(c, c, c)
        for t in range(LT):
            eo = [cone(c, idx, t, u) for u in range(8)]
            stage_d(c, t, lambda n: jnp.concatenate([e[n] for e in eo], axis=0).astype(BF16))

    def load_q(c, r0, tie):
        x = q_v[c, r0:r0 + 16, :].astype(F32).reshape(2, 8, D)
        if tie is not None:
            never = (zm[...] != 0)[None]
            x = jnp.concatenate([jnp.where(never, tie.reshape(2, 8, 128), x[:, :, 0:128]), x[:, :, 128:]], axis=2)
        return x

    def gate_coef(x):
        return _ln(x) * modv[0][None] + modv[1][None]

    def ea_rows(c, r0):
        w = gate_coef(load_q(c, r0, None)).reshape(16, D)
        wbuf[r0:r0 + 16, :] = w
        return w[:, 0:128]

    def norm2_rows(c, r0, yi, x1dst, have_w, tie=None):
        rows = slice(r0, r0 + 16)
        x = load_q(c, r0, tie)
        y = jnp.concatenate([ybuf[yi, t, rows, :] for t in range(LT)], axis=1).reshape(2, 8, D)
        w = wbuf[rows, :].reshape(2, 8, D) if have_w else gate_coef(x)
        x1 = x + w * y
        x1dst[rows, :] = x1.reshape(16, D)
        return _ln(x1)

    def mod2(n2):
        return (n2 * modv[2][None] + modv[3][None]).reshape(16, D)

    def store_lhs(dst, r8, top, bot):
        rows = slice(r8, r8 + 8)
        for kt in range(2):
            ss = _asums(top[:, _ls(kt)], top[:, _ls(2 + kt)], bot[:, _ls(kt)], bot[:, _ls(2 + kt)])
            for i in range(7):
                dst[rows, _ls(2 * i + kt)] = _pack(ss[i])
        dst[rows, _ls(14)] = _pack(top[:, _ls(4)])
        dst[rows, _ls(15)] = _pack(bot[:, _ls(4)])
        return ss[0]

    def mod_part(n0, n1):
        cf = c_v[...].astype(F32)
        sc = cf * (1.0 / (1.0 + jnp.exp(-cf)))
        lhs = jnp.broadcast_to(sc, (16, D)).astype(BF16)
        mod = jnp.dot(lhs, wm_v[:, n0 * D:n1 * D], preferred_element_type=F32)[0:8]
        return [mod[:, n * D:(n + 1) * D] for n in range(n1 - n0)]

    bspec = [((0, 0), 1, (1, 1)), ((0, 0), 0, None), ((0, 1), -1, (1, 1)), ((1, 0), -1, (0, 0)),
             ((1, 1), 0, None), ((0, 0), 1, (0, 1)), ((1, 0), 1, (1, 1))]

    def bsum(quad, i):
        qa, sign, qb = bspec[i]
        if sign == 0:
            return pltpu.bitcast(quad(*qa), U32)
        a = quad(*qa).astype(F32)
        b = quad(*qb).astype(F32)
        return _pack(a + b if sign > 0 else a - b)

    def prep_gu(col):
        p, mat, i = col // 16, (col // 8) % 2, col % 8
        w = (wg_v, wu_v)[mat]
        if i == 7:
            for cc in range(2):
                wgu[64 * cc:64 * cc + 64, _ls(col)] = pltpu.bitcast(w[512:640, _ls(2 * p + cc)], U32)
        else:
            wgu[0:128, _ls(col)] = bsum(lambda r, c: w[256 * r:256 * r + 256, _ls(2 * p + c)], i)

    def prep_dn(col):
        for p in range(6):
            if col >= 14:
                val = pltpu.bitcast(wd_v[_ls(2 * p + col - 14), _ls(4)], U32)
            else:
                val = bsum(lambda r, c: wd_v[_ls(2 * p + r), _ls(2 * (col // 7) + c)], col % 7)
            wdn[64 * p:64 * p + 64, _ls(col)] = val

    def step(s, smin, smax, do_conv=True, warm=False):
        nch = 2 if warm else 1
        R = 64 * nch
        if do_conv:
            idx = lag_idx(s, smin, smax)
        off = (64 if warm else 32) * (s % 2)
        lv = lhsb.at[pl.ds(pl.multiple_of((s - nch) * 64, 64), R + 64)]
        x1v = x1buf.at[pl.ds(s - nch, nch + 1)]
        if warm:
            dl_w = dl_r = dlb
        else:
            dl_w = dlb.at[pl.ds(pl.multiple_of((s % 2) * 64, 64), 64)]
            dl_r = dlb.at[pl.ds(pl.multiple_of(((s + 2) % 2) * 64, 64), 64)]

        items = [[] for _ in range(112)]
        if warm:
            items[W_D].append(("d", 0))
            for m, names in W_WAITS.items():
                for name in names:
                    items[m].append(("w", name))
            items[W_AB].append(("ab", 0))
            items[W_MOD].append(("mod", 0))
            c_slots, ea_slots, e_slots, e_tie = WC_SLOTS, None, WE_SLOTS, None
        elif do_conv:
            items[0].append(("ab", 0))
            items[D_SLOT].append(("d", 0))
            c_slots, ea_slots, e_slots, e_tie = C_SLOTS, EA_SLOTS, E_SLOTS, E_TIE
        if do_conv:
            for p in range(40):
                items[c_slots[p]].append(("c", p))
            for g in range(16):
                items[e_slots[g]].append(("e", g))
                if ea_slots is not None:
                    items[ea_slots[g]].append(("ea", g))
        tops, hist, where = {}, {}, {}
        slot = [0]

        def tie_of(p):
            if e_tie is None or e_tie[p] is None:
                return None
            return hist[e_tie[p]][112:128]

        def pin_rows(nrows, n):
            return pl.ds(_mo(nrows + off + 8 * n, 8), 8)

        def hook(ref, nrows, col):
            m = slot[0]
            slot[0] += 1
            npin = 0
            todo = [x for x in items[m] if x[0] in ("d", "w", "ab", "mod")]
            if warm:
                todo.append(("prep", col))
            todo += [x for x in items[m] if x[0] not in ("d", "w", "ab", "mod")]
            for kind, p in todo:
                if kind == "w":
                    wait(p)
                elif kind == "prep":
                    (prep_gu if m < 96 else prep_dn)(p)
                elif kind == "mod":
                    modv[4] = mod_part(5, 6)[0]
                elif kind == "ab":
                    for t in range(LT):
                        stage_b(s, t)
                        stage_a(s, t)
                elif kind == "d":
                    for t in range(LT):
                        def wfn(n):
                            parts = []
                            for u in range(8):
                                rf, nr, cl, n0 = where[8 * t + u]
                                parts.append(rf[pin_rows(nr, n0 + n), _ls(cl)])
                            return pltpu.bitcast(jnp.concatenate(parts, axis=0), BF16)
                        stage_d(0, t, wfn)
                elif kind == "c":
                    res = cone(s, idx, p // 8, p % 8)
                    for n in range(4):
                        ref[pin_rows(nrows, npin + n), _ls(col)] = _pack(res[n])
                    where[p] = (ref, nrows, col, npin)
                    npin += 4
                else:
                    if kind == "ea":
                        val = ea_rows(s, 16 * p)
                    else:
                        g = p // 2
                        h2 = mod2(norm2_rows(s, 16 * g + C * (p % 2), 0, x1v.at[nch], ea_slots is not None, tie_of(p)))
                        if p % 2 == 0:
                            tops[g] = h2
                            val = h2[:, _ls(4)]
                        else:
                            val = store_lhs(lv, R + 8 * g, tops[g], h2)
                    ref[pin_rows(nrows, npin), _ls(col)] = _pack(val)
                    npin += 1
                assert npin <= 4 * nch

        def dot(a, w):
            r = jnp.dot(pltpu.bitcast(a, BF16), pltpu.bitcast(w, BF16), preferred_element_type=F32)
            hist.setdefault(slot[0] - 1, r)
            return r

        def strassen(lhs, ref, nrows, base, left):
            def m(i):
                hook(ref, nrows, base + i - 1)
                return dot(lhs(i - 1), ref[0:nrows, _ls(base + i - 1)])
            m2 = m(2)
            m4 = m(4)
            c21 = m2 + m4
            m3 = m(3)
            m5 = m(5)
            c12 = m3 + m5
            c11 = m4 - m5
            c22 = m3 - m2
            m1 = m(1)
            m7 = m(7)
            c11 = c11 + m1 + m7
            c22 = c22 + m1
            c22 = c22 + m(6)
            if left is not None:
                hook(ref, nrows, base + 7)
                c22 = c22 + left(1, 1)
                c11 = c11 + left(0, 0)
                c12 = c12 + left(0, 1)
                c21 = c21 + left(1, 0)
            return c11, c12, c21, c22

        for p in range(6):
            res = []
            for mat in range(2):
                base = (2 * p + mat) * 8
                res.append(strassen(
                    lambda i: lv[0:R, 256 * i:256 * i + 256], wgu, 128, base,
                    lambda r, c: dot(lv[0:R, _ls(14 + r)], wgu[64 * c:64 * c + 64, _ls(base + 7)])))
            hq = [res[0][i] * res[1][i] for i in range(4)]
            for i, x in enumerate(_asums(*hq) + [hq[1], hq[2]]):
                if p < 5:
                    dl_w[:, _ls(5 * i + p)] = _pack(x)
                else:
                    dl5[0:R, _ls(i)] = _pack(x)

        def dla(i):
            return dl_r[:, 640 * i:640 * i + 640]

        def dlz(i):
            return dl5[0:R, _ls(i)]

        def dl(i):
            return jnp.concatenate([dla(i), dlz(i)], axis=1)

        def emit(r, n, o):
            rows = slice(r * C, (r + 1) * C)
            for ch in range(nch):
                res = (x1v[ch, rows, _ls(n)].reshape(16, 8, 128)
                       + o[ch * C:(ch + 1) * C].reshape(16, 8, 128) * modv[4, :, _ls(n)][None])
                o_v[s - nch + ch, rows, _ls(n)] = res.reshape(C, 128).astype(BF16)

        hook(wdn, 384, 14)
        ta = dot(dla(2), wdn[0:320, _ls(14)])
        tb = dot(dla(8), wdn[0:320, _ls(14)])
        ta = ta + dot(dlz(2), wdn[320:384, _ls(14)])
        tb = tb + dot(dlz(8), wdn[320:384, _ls(14)])
        hook(wdn, 384, 15)
        emit(0, 4, ta + dot(dl(7), wdn[0:384, _ls(15)]))
        emit(1, 4, tb + dot(dl(3), wdn[0:384, _ls(15)]))
        if not do_conv:
            out_copy(s - 1, *last_parts[0]).start()
        for pp in range(2):
            cs = strassen(dl, wdn, 384, 7 * pp, None)
            for n, i in enumerate((2, 1, 0, 3)):
                emit(i // 2, 2 * pp + i % 2, cs[i])
                if not do_conv and pp == 1:
                    out_copy(s - 1, *last_parts[2 + n]).start()
            if not do_conv and pp == 0:
                out_copy(s - 1, *last_parts[1]).start()
        if do_conv:
            for ch in range(nch):
                out_copy(s - nch + ch).start()

    one = jnp.minimum(pl.program_id(0), 0) + 1

    def dyn_step(s, **kw):
        def body(t, carry):
            with jax.named_scope("step%d" % s):
                step(t + s, s, s, **kw)
            return carry
        lax.fori_loop(0, one, body, 0)

    wait("c0")
    with jax.named_scope("conv0"):
        conv_all(0)
    wait("c1")
    with jax.named_scope("conv1"):
        conv_all(1)
    wait("wm1")
    with jax.named_scope("mod1"):
        sa, ca, ga = mod_part(0, 3)
        modv[0] = ga * (1.0 + ca)
        modv[1] = ga * sa
        for c in range(2):
            for g in range(16):
                wbuf[c * M + 16 * g:c * M + 16 * g + 16, :] = norm2_rows(
                    c, 16 * g, c, x1buf.at[c], False).reshape(16, D)
    wait("wm2")
    with jax.named_scope("mod2"):
        sb, cb = mod_part(3, 5)
        modv[2] = 1.0 + cb
        modv[3] = sb
        for c in range(2):
            for g in range(8):
                top, bot = [mod2(wbuf[r:r + 16, :].reshape(2, 8, D))
                            for r in (c * M + 16 * g, c * M + C + 16 * g)]
                store_lhs(lhsb, 64 * c + 8 * g, top, bot)
    dyn_step(2, warm=True)
    wait("c3")

    def body(s, carry):
        @pl.when(s == 4)
        def _():
            wait("rest")
        with jax.named_scope("step"):
            step(s, 3, 7)
        return carry
    lax.fori_loop(3, 8, body, 0)
    dyn_step(8, do_conv=False)

    with jax.named_scope("wait_out"):
        for i in range(NC - 1):
            out_copy(i).wait()
        for part in last_parts:
            out_copy(NC - 1, *part).wait()


@jax.jit
def pallas_adaLN_cond__ssm_conv_h3__glu_gated_bilinear__prompt_kernel(A_q, A_k, A_v, A_shift_k, A_ssm_k, A_ssm_D, B_x, B_w_gate, B_w_up, B_w_down, c, w_mod):
    cst = jnp.asarray(_dft_consts(), dtype=BF16)
    any_spec = pl.BlockSpec(memory_space=pl.ANY)
    out = pl.pallas_call(
        _kernel,
        grid=(1,),
        in_specs=[any_spec] * 12,
        out_specs=any_spec,
        out_shape=jax.ShapeDtypeStruct((NC, M, D), BF16),
        scratch_shapes=[
            pltpu.VMEM((NC, M, D), BF16), pltpu.VMEM((NC, M, D), BF16), pltpu.VMEM((NC, M, D), BF16),
            pltpu.VMEM((D, S), BF16),
            pltpu.VMEM((D, FF), BF16), pltpu.VMEM((D, FF), BF16), pltpu.VMEM((FF, D), BF16),
            pltpu.VMEM((D, 6 * D), BF16),
            pltpu.VMEM((3 * C, C), BF16),
            pltpu.VMEM((NC, M, D), BF16),
            pltpu.VMEM((LT, 32 + S, 128), F32),
            pltpu.VMEM((NB + 1, LT, 16, 24, 128), F32),
            pltpu.VMEM((NB, LT, 16, 24, 128), F32),
            pltpu.VMEM((NC + 1, LT, 8, 32, 128), F32),
            pltpu.VMEM((2, LT, M, 128), F32),
            pltpu.VMEM((NC + 1, M, D), F32),
            pltpu.VMEM(((NC + 1) * 64, 16 * 128), U32),
            pltpu.VMEM((128 + 64, 96 * 128), U32),
            pltpu.VMEM((384 + 64, 16 * 128), U32),
            pltpu.VMEM((2 * 64, 9 * 640), U32),
            pltpu.VMEM((2 * 64, 9 * 128), U32),
            pltpu.VMEM((2 * M, D), F32),
            pltpu.VMEM((8, 8, D), F32),
            pltpu.VMEM((4, 8, D), F32),
            pltpu.VMEM((8, 128), jnp.int32),
            pltpu.VMEM((4, D), BF16), pltpu.VMEM((D,), BF16), pltpu.VMEM((1, D), BF16),
            pltpu.VMEM((6, 1, 128), F32),
            pltpu.SemaphoreType.DMA((12,)),
            pltpu.SemaphoreType.DMA(()),
        ],
        compiler_params=pltpu.CompilerParams(vmem_limit_bytes=120 * 1024 * 1024),
        name="fused_h3_glu",
    )(A_q.reshape(NC, M, D), A_k.reshape(NC, M, D), A_v.reshape(NC, M, D), A_shift_k.T, A_ssm_k, A_ssm_D,
      B_w_gate, B_w_up, B_w_down, c, w_mod, cst)
    return out.reshape(1, S, D)
```

```python
import numpy as np
import jax
import jax.numpy as jnp
from jax import lax
import jax.experimental.pallas as pl
import jax.experimental.pallas.tpu as pltpu

S, D, FF = 2048, 640, 1536
C = 128
NB = S // C
M = 256
NC = S // M
LT = D // 128
EPS = 1e-5
F32 = jnp.float32
BF16 = jnp.bfloat16
U32 = jnp.uint32


def _dft_consts():
    r = np.arange(C)
    theta = np.pi * (4 * r + 1) / (2 * C)
    c = np.arange(C)
    ang = theta[:, None] * c[None, :]
    cs = np.stack([np.cos(ang), -np.sin(ang)], axis=0)
    fm = cs.reshape(2, 2, 8, 8, C).transpose(2, 1, 0, 3, 4).reshape(2 * C, C)
    a = np.concatenate([np.arange(0, C, 2), np.arange(1, C, 2)])
    ang2 = a[:, None] * theta[None, :64]
    g = np.zeros((C, 8, 2, 8))
    g[:, :, 0] = np.cos(ang2).reshape(C, 8, 8) / C
    g[:, :, 1] = -np.sin(ang2).reshape(C, 8, 8) / C
    g = g.reshape(C, C)
    return np.concatenate([fm, g], axis=0).astype(np.float32)


C_SLOTS = tuple(range(40, 80))
D_SLOT = 80
E_SLOTS = tuple(x for x in (86, 90, 94, 97, 97, 98, 99, 101, 102, 104, 105, 106, 108, 109, 111, 111) for _ in range(2))
WK_SLOTS = (68, 70, 72, 74, 76, 77, 78, 79)
WWK_SLOTS = (99, 100, 101, 102, 103, 104, 105, 106)
X_FAST = False
X_WKS = 4
WC_SLOTS = tuple(sorted(2 * list(range(60, 80))))
W_WAITS = {0: ("p0",), 16: ("p1",), 48: ("p3",), 80: ("p5",), 96: ("wd",)}
W_AB = 48
W_CMIN = 1
W_D = 80
W_MOD = 97
W_BFIRST = False
WE_SLOTS = tuple(x for x in (86, 90, 94, 98, 98, 99, 100, 102, 103, 104, 106, 107, 108, 110, 111, 111) for _ in range(2))


def _mo(x, m):
    return x if isinstance(x, int) else pl.multiple_of(x, m)


def _ls(t):
    return slice(t * 128, (t + 1) * 128)


def _pack(x):
    return pltpu.bitcast(x.astype(BF16), U32)


def _asums(a11, a12, a21, a22):
    return [a11 + a22, a21 + a22, a11, a22, a11 + a12, a21 - a11, a12 - a22]


def _ln(x, fast=False):
    m = jnp.sum(x, axis=-1, keepdims=True) * (1.0 / D)
    if fast:
        ms = jnp.sum(x * x, axis=-1, keepdims=True) * (1.0 / D)
        return (x - m) * lax.rsqrt(jnp.maximum(ms - m * m, 0.0) + EPS)
    xc = x - m
    var = jnp.sum(xc * xc, axis=-1, keepdims=True) * (1.0 / D)
    return xc * lax.rsqrt(var + EPS)


def _kernel(q_h, k_h, v_h, sh_h, sk_h, sd_h, wg_h, wu_h, wd_h, c_h, wm_h, cst_h,
            o_h,
            q_v, k_v, v_v, sk_v, wg_v, wu_v, wd_v, wm_v, cst_v,
            o_v, kbuf, xf, kf, qbuf, ybuf, x1buf, lhsb, wgu, wdn, dlb, dl5, wbuf, modv, shb,
            sh_v, sd_v, c_v, pad_v,
            sem_in, sem_out):
    def k_in(c0, c1):
        return [(k_h.at[c0:c1], k_v.at[c0:c1])]

    def conv_in(c0, c1, with_k=True):
        cols = pl.ds(c0 * M, (c1 - c0) * M)
        return ([(sk_h.at[:, cols], sk_v.at[:, cols])] + (k_in(c0, c1) if with_k else [])
                + [(v_h.at[c0:c1], v_v.at[c0:c1])])

    def q_in(c0, c1):
        return [(q_h.at[c0:c1], q_v.at[c0:c1])]

    def gu_in(p0, p1):
        cols = pl.ds(p0 * 256, (p1 - p0) * 256)
        return [(wg_h.at[:, cols], wg_v.at[:, cols]), (wu_h.at[:, cols], wu_v.at[:, cols])]

    def wm_in(n0, n1):
        cols = pl.ds(n0 * D, (n1 - n0) * D)
        return [(wm_h.at[:, cols], wm_v.at[:, cols])]

    dma = dict(
        small=[(cst_h, cst_v), (sh_h, sh_v), (sd_h, sd_v), (c_h, c_v)],
        c0=conv_in(0, 1),
        c1=conv_in(1, 2),
        c2=conv_in(2, 3),
        wm1=q_in(0, 2) + wm_in(0, 3),
        wm2=wm_in(3, 5),
        p0=gu_in(0, 1),
        p1=gu_in(1, 3),
        p3=conv_in(3, 4) + gu_in(3, 5),
        p5=gu_in(5, 6) + q_in(2, 4),
        wd=wm_in(5, 6) + [(wd_h, wd_v)] + k_in(4, 6),
        r1=conv_in(4, 6, False) + k_in(6, 8),
        r2=q_in(4, 8) + conv_in(6, 8, False),
    )
    dma = {name: [pltpu.make_async_copy(a, b, sem_in.at[n]) for a, b in grp]
           for n, (name, grp) in enumerate(dma.items())}

    def wait(name):
        with jax.named_scope("w_" + name):
            for cp in dma[name]:
                cp.wait()

    def out_copy(i, rows=None, cols=None):
        if rows is None:
            return pltpu.make_async_copy(o_v.at[pl.ds(i, 2)], o_h.at[pl.ds(i, 2)], sem_out)
        return pltpu.make_async_copy(o_v.at[i, rows, cols], o_h.at[i, rows, cols], sem_out)

    last_parts = [(slice(None), _ls(4)), (slice(None), slice(0, 256)), (slice(C, M), _ls(2)),
                  (slice(0, C), _ls(3)), (slice(0, C), _ls(2)), (slice(C, M), _ls(3))]

    for grp in dma.values():
        for cp in grp:
            cp.start()

    for t in range(LT):
        kbuf[t, 24:32, :] = jnp.zeros((8, 128), F32)
    xf[0] = jnp.zeros((LT, 16, 24, 128), F32)
    qbuf[0] = jnp.zeros((LT, 8, 32, 128), F32)
    pad_v[...] = jnp.zeros(pad_v.shape, F32)
    wait("small")
    sh = sh_v[...].astype(F32)
    modv[5] = jnp.broadcast_to(sd_v[...].astype(F32).reshape(1, D), (8, D))
    modv[6] = jnp.zeros((8, D), F32)
    for j in range(4):
        shb[j] = jnp.broadcast_to(sh[j:j + 1, :], (8, D))

    def widen_next_k(s, part, gate):
        kbuf[0, pl.ds(pl.multiple_of(8 * (s % 2048), 8), 8), :] = gate
        r0 = _mo(s * M, M)
        n = 2 * M // (len(WK_SLOTS) * X_WKS)
        ch, r = divmod(part * n, M)
        kk = k_v[jnp.minimum(s + 2 + ch, NC - 1), r:r + n, :].astype(F32)
        for t in range(LT):
            kbuf[t, pl.ds(r0 + 32 + 2 * M + part * n, n), :] = kk[:, _ls(t)]

    def stage_a(c, t, widen=True):
        r0 = _mo(c * M, M)
        ls = _ls(t)
        if widen:
            kk = k_v[c, :, ls].astype(F32)
            kbuf[t, pl.ds(r0 + 32, M), :] = kk
        else:
            kk = kbuf[t, pl.ds(r0 + 32, M), :]
        acc = kk.reshape(32, 8, 128) * shb[0, :, ls][None]
        for j in range(1, 4):
            acc = acc + kbuf[t, pl.ds(r0 + 32 - j, M), :].reshape(32, 8, 128) * shb[j, :, ls][None]
        kv = acc.reshape(M, 128) * v_v[c, :, ls].astype(F32)
        for b in range(2):
            r = jnp.dot(cst_v[0:2 * C, :], kv[b * C:(b + 1) * C].astype(BF16),
                        preferred_element_type=F32).reshape(16, 16, 128)
            xf[2 * c + 1 + b, t, :, 0:16, :] = r
            xf[2 * c + 1 + b, t, :, 16:24, :] = r[:, 0:8, :] + r[:, 8:16, :]

    def stage_b(c, t, maybe_first=False):
        for b in range(2):
            kb = sk_v[_ls(t), pl.ds(_mo(c * M + b * C, C), C)]
            r = lax.dot_general(cst_v[0:2 * C, :], kb, (((1,), (1,)), ((), ())),
                                preferred_element_type=F32).reshape(16, 16, 128)
            cc = r[:, 0:8, :]
            d = r[:, 8:16, :]
            if maybe_first and b == 0:
                cc = cc + modv[5 + jnp.minimum(c, 1), :, _ls(t)][None]
            kf[2 * c + b, t, :, 0:8, :] = d - cc
            kf[2 * c + b, t, :, 8:16, :] = cc + d
            kf[2 * c + b, t, :, 16:24, :] = cc

    def lag_idx(c, cmin, cmax, nout):
        top = 2 * c + nout - 1
        nlag = 2 * cmax + nout
        jok = 2 * cmin + nout - 1
        kidx = [j if j <= jok else jnp.minimum(j, top) for j in range(nlag)]
        xidx = [top + 1 - j if j <= jok + 1 else jnp.maximum(top + 1 - j, 0) for j in range(nlag)]
        return kidx, xidx, nout

    def block_conv(idx, t, us):
        kidx, xidx, nout = idx
        xs = []
        acc = [None] * nout
        for j in reversed(range(len(kidx))):
            k = kf[kidx[j], t, us]
            xs = [xf[xidx[j], t, us]] + xs[:nout - 1]
            for o in reversed(range(len(xs))):
                p = k * xs[o]
                acc[o] = p if acc[o] is None else acc[o] + p
        return [(a[..., 16:24, :] - a[..., 8:16, :], a[..., 16:24, :] + a[..., 0:8, :]) for a in reversed(acc)]

    def cone(c, idx, t, u, pin=None):
        nout = idx[2]
        if nout == 2:
            ri = [((re[0], im[0]), (re[1], im[1])) for re, im in block_conv(idx, t, slice(2 * u, 2 * u + 2))]
        else:
            hs = []
            for h in range(2):
                hs.append(block_conv(idx, t, 2 * u + h))
                tot = [re + im for re, im in hs[h]]
                pin(h, (tot[0] + tot[1]) + (tot[2] + tot[3]))
            ri = list(zip(*hs))
        qs = [(h0[0] + h1[0], h0[1] + h1[1], h0[0] - h1[0], h0[1] - h1[1]) for h0, h1 in ri]
        qv = qbuf.at[pl.ds(c, nout // 2 + 1)]
        qv[nout // 2, t, u] = jnp.concatenate(qs[-1], axis=0)
        prev = qv[0, t, u]
        pv = (prev[0:8], prev[8:16], prev[16:24], prev[24:32])
        res = []
        for cur in qs:
            res.append(jnp.concatenate([cur[0] - pv[1], cur[1] + pv[0]], axis=0))
            res.append(jnp.concatenate([cur[2] - pv[3], cur[3] + pv[2]], axis=0))
            pv = cur
        return res

    def stage_d(yi, t, wfn):
        for b in range(2):
            for par in range(2):
                g = cst_v[2 * C + 64 * par:2 * C + 64 * (par + 1), :]
                y = jnp.dot(g, wfn(2 * b + par), preferred_element_type=F32)
                ybuf[yi, t, pl.ds(b * C + par, 64, stride=2), :] = y

    def ab_all(c):
        for t in range(LT):
            stage_b(c, t, True)
            stage_a(c, t)

    def cd_all(c, cmin, cmax):
        idx = lag_idx(c, cmin, cmax, 2)
        for t in range(LT):
            eo = [cone(c, idx, t, u) for u in range(8)]
            stage_d(c, t, lambda n: jnp.concatenate([e[n] for e in eo], axis=0).astype(BF16))

    def norm2_rows(c, r0, yi, x1dst):
        rows = slice(r0, r0 + 16)
        x = q_v[c, rows, :].astype(F32).reshape(2, 8, D)
        y = jnp.concatenate([ybuf[yi, t, rows, :] for t in range(LT)], axis=1).reshape(2, 8, D)
        x1 = x + (_ln(x, X_FAST) * modv[0][None] + modv[1][None]) * y
        x1dst[rows, :] = x1.reshape(16, D)
        return _ln(x1, X_FAST)

    def mod2(n2):
        return (n2 * modv[2][None] + modv[3][None]).reshape(16, D)

    def store_lhs(dst, r8, top, bot):
        rows = slice(r8, r8 + 8)
        for kt in range(2):
            ss = _asums(top[:, _ls(kt)], top[:, _ls(2 + kt)], bot[:, _ls(kt)], bot[:, _ls(2 + kt)])
            for i in range(7):
                dst[rows, _ls(2 * i + kt)] = _pack(ss[i])
        dst[rows, _ls(14)] = _pack(top[:, _ls(4)])
        dst[rows, _ls(15)] = _pack(bot[:, _ls(4)])
        return ss[0]

    def mod_part(n0, n1):
        cf = c_v[...].astype(F32)
        sc = cf * (1.0 / (1.0 + jnp.exp(-cf)))
        lhs = jnp.broadcast_to(sc, (16, D)).astype(BF16)
        mod = jnp.dot(lhs, wm_v[:, n0 * D:n1 * D], preferred_element_type=F32)[0:8]
        return [mod[:, n * D:(n + 1) * D] for n in range(n1 - n0)]

    bspec = [((0, 0), 1, (1, 1)), ((0, 0), 0, None), ((0, 1), -1, (1, 1)), ((1, 0), -1, (0, 0)),
             ((1, 1), 0, None), ((0, 0), 1, (0, 1)), ((1, 0), 1, (1, 1))]

    def bsum(quad, i):
        qa, sign, qb = bspec[i]
        if sign == 0:
            return pltpu.bitcast(quad(*qa), U32)
        a = quad(*qa).astype(F32)
        b = quad(*qb).astype(F32)
        return _pack(a + b if sign > 0 else a - b)

    def prep_gu(col):
        p, mat, i = col // 16, (col // 8) % 2, col % 8
        w = (wg_v, wu_v)[mat]
        if i == 7:
            for cc in range(2):
                wgu[64 * cc:64 * cc + 64, _ls(col)] = pltpu.bitcast(w[512:640, _ls(2 * p + cc)], U32)
        else:
            wgu[0:128, _ls(col)] = bsum(lambda r, c: w[256 * r:256 * r + 256, _ls(2 * p + c)], i)

    def prep_dn(col):
        for p in range(6):
            if col >= 14:
                val = pltpu.bitcast(wd_v[_ls(2 * p + col - 14), _ls(4)], U32)
            else:
                val = bsum(lambda r, c: wd_v[_ls(2 * p + r), _ls(2 * (col // 7) + c)], col % 7)
            wdn[64 * p:64 * p + 64, _ls(col)] = val

    def step(s, mode):
        warm, main, last = mode == "warm", mode == "main", mode == "last"
        nch = 1 if last else 2
        R = 64 * nch
        off = 128 * (s % 2)
        lv = lhsb.at[pl.ds(pl.multiple_of((s - 2) * 64, 64), 2 * R)]
        x1v = x1buf.at[pl.ds(s - 2, 2 * nch)]
        dl_w = dlb.at[pl.ds(pl.multiple_of((s % 2) * 32, 32), R)]
        dl_r = dlb.at[pl.ds(pl.multiple_of(((s + 2) % 2) * 32, 32), R)]

        items = [[] for _ in range(112)]
        if warm:
            c0, nout = s + 1, 2
            idx = lag_idx(c0, W_CMIN, 3, nout)
            items[W_D].append(("d", 0))
            for m, names in W_WAITS.items():
                for name in names:
                    items[m].append(("w", name))
            items[W_AB].append(("ab", 0))
            items[W_MOD].append(("mod", 0))
            c_slots, e_slots, yis = WC_SLOTS, WE_SLOTS, (2, 0)
        elif main:
            c0, nout = s, 4
            idx = lag_idx(c0, 4, 6, nout)
            items[0].append(("ab", 0))
            items[D_SLOT].append(("d", 0))
            c_slots, e_slots, yis = C_SLOTS, E_SLOTS, (0, 1)
        if not last:
            for n, m in enumerate(WWK_SLOTS if warm else WK_SLOTS):
                items[m].append(("wk", n))
            for p in range(40):
                items[c_slots[p]].append(("c", p))
            for g in range(32):
                items[e_slots[g]].append(("e", g))
        tops, hist, where = {}, {}, {}
        slot = [0]

        def pin_rows(nrows, n):
            return pl.ds(_mo(nrows + off + 8 * n, 8), 8)

        def hook(ref, nrows, col):
            m = slot[0]
            slot[0] += 1
            npin = 0
            todo = [x for x in items[m] if x[0] not in ("c", "e")]
            if warm:
                todo.append(("prep", col))
            todo += [x for x in items[m] if x[0] in ("c", "e")]
            for kind, p in todo:
                if kind == "w":
                    wait(p)
                elif kind == "prep":
                    (prep_gu if m < 96 else prep_dn)(p)
                elif kind == "mod":
                    modv[4] = mod_part(5, 6)[0]
                elif kind == "ab":
                    for ch in range(nout // 2):
                        for t in range(LT):
                            stage_b(c0 + ch, t)
                            if not (warm and W_BFIRST):
                                stage_a(c0 + ch, t, warm)
                    if warm and W_BFIRST:
                        for t in range(LT):
                            stage_a(c0, t, warm)
                elif kind == "wk":
                    for r in range(X_WKS):
                        r0 = 8 * (32 * r // X_WKS)
                        widen_next_k(s, X_WKS * p + r, hist[m - 1][r0:r0 + 8])
                elif kind == "d":
                    for ch in range(nout // 2):
                        for t in range(LT):
                            def wfn(n):
                                parts = []
                                for u in range(8):
                                    rf, nr, cl = where[8 * t + u]
                                    parts.append(rf[pin_rows(nr, 8 * ch + n), _ls(cl)])
                                return pltpu.bitcast(jnp.concatenate(parts, axis=0), BF16)
                            stage_d(ch, t, wfn)
                    if main:
                        out_copy(s - 4).wait()

                        @pl.when(s == 4)
                        def _():
                            wait("r2")
                elif kind == "c":
                    def pin(h, val):
                        ref[pin_rows(nrows, 15 - 3 * h), _ls(col)] = pltpu.bitcast(val, U32)
                    res = cone(c0, idx, p // 8, p % 8, pin)
                    n0 = (4 - npin) if warm else 0
                    for n in range(2 * nout):
                        ref[pin_rows(nrows, n0 + n % 4 + 8 * (n // 4)), _ls(col)] = _pack(res[n])
                    where[p] = (ref, nrows + 8 * n0, col)
                    npin += 2 * nout
                else:
                    ch, g, half = p // 16, (p % 16) // 2, p % 2
                    h2 = mod2(norm2_rows(s + ch, 16 * g + C * half, yis[ch], x1v.at[2 + ch]))
                    if half == 0:
                        tops[g] = h2
                        val = h2[:, _ls(4)]
                    else:
                        val = store_lhs(lv, R + 64 * ch + 8 * g, tops[g], h2)
                    ref[pin_rows(nrows, npin), _ls(col)] = _pack(val)
                    npin += 1
                assert npin <= 8

        def dot(a, w):
            r = jnp.dot(pltpu.bitcast(a, BF16), pltpu.bitcast(w, BF16), preferred_element_type=F32)
            hist.setdefault(slot[0] - 1, r)
            return r

        def strassen(lhs, ref, nrows, base, left):
            def m(i):
                hook(ref, nrows, base + i - 1)
                return dot(lhs(i - 1), ref[0:nrows, _ls(base + i - 1)])
            m2 = m(2)
            m4 = m(4)
            c21 = m2 + m4
            m3 = m(3)
            m5 = m(5)
            c12 = m3 + m5
            c11 = m4 - m5
            c22 = m3 - m2
            m1 = m(1)
            m7 = m(7)
            c11 = c11 + m1 + m7
            c22 = c22 + m1
            c22 = c22 + m(6)
            if left is not None:
                hook(ref, nrows, base + 7)
                c22 = c22 + left(1, 1)
                c11 = c11 + left(0, 0)
                c12 = c12 + left(0, 1)
                c21 = c21 + left(1, 0)
            return c11, c12, c21, c22

        for p in range(6):
            res = []
            for mat in range(2):
                base = (2 * p + mat) * 8
                res.append(strassen(
                    lambda i: lv[0:R, 256 * i:256 * i + 256], wgu, 128, base,
                    lambda r, c: dot(lv[0:R, _ls(14 + r)], wgu[64 * c:64 * c + 64, _ls(base + 7)])))
            hq = [res[0][i] * res[1][i] for i in range(4)]
            for i, x in enumerate(_asums(*hq) + [hq[1], hq[2]]):
                if p < 5:
                    dl_w[:, _ls(5 * i + p)] = _pack(x)
                else:
                    dl5[0:R, _ls(i)] = _pack(x)

        def dla(i):
            return dl_r[:, 640 * i:640 * i + 640]

        def dlz(i):
            return dl5[0:R, _ls(i)]

        def dl(i):
            return jnp.concatenate([dla(i), dlz(i)], axis=1)

        def emit(r, n, o):
            rows = slice(r * C, (r + 1) * C)
            for ch in range(nch):
                res = (x1v[ch, rows, _ls(n)].reshape(16, 8, 128)
                       + o[ch * C:(ch + 1) * C].reshape(16, 8, 128) * modv[4, :, _ls(n)][None])
                o_v[s - 2 + ch, rows, _ls(n)] = res.reshape(C, 128).astype(BF16)

        hook(wdn, 384, 14)
        ta = dot(dla(2), wdn[0:320, _ls(14)])
        tb = dot(dla(8), wdn[0:320, _ls(14)])
        ta = ta + dot(dlz(2), wdn[320:384, _ls(14)])
        tb = tb + dot(dlz(8), wdn[320:384, _ls(14)])
        hook(wdn, 384, 15)
        emit(0, 4, ta + dot(dl(7), wdn[0:384, _ls(15)]))
        emit(1, 4, tb + dot(dl(3), wdn[0:384, _ls(15)]))
        if last:
            out_copy(s - 2, *last_parts[0]).start()
        for pp in range(2):
            cs = strassen(dl, wdn, 384, 7 * pp, None)
            for n, i in enumerate((2, 1, 0, 3)):
                emit(i // 2, 2 * pp + i % 2, cs[i])
                if last and pp == 1:
                    out_copy(s - 2, *last_parts[2 + n]).start()
            if last and pp == 0:
                out_copy(s - 2, *last_parts[1]).start()
        if not last:
            out_copy(s - 2).start()

    one = jnp.minimum(pl.program_id(0), 0) + 1

    def dyn_step(s, mode):
        def body(t, carry):
            with jax.named_scope("step%d" % s):
                step(t + s, mode)
            return carry
        lax.fori_loop(0, one, body, 0)

    def conv012(c, carry):
        for n in range(3):
            @pl.when(c == n)
            def _():
                wait("c%d" % n)
        with jax.named_scope("ab"):
            ab_all(c)

        @pl.when(c == 0)
        def _():
            with jax.named_scope("cd0"):
                cd_all(c, 0, 0)

        @pl.when(c > 0)
        def _():
            with jax.named_scope("cd12"):
                cd_all(c, 1, 2)
        return carry
    lax.fori_loop(0, 3, conv012, 0)
    wait("wm1")
    with jax.named_scope("mod1"):
        sa, ca, ga = mod_part(0, 3)
        modv[0] = ga * (1.0 + ca)
        modv[1] = ga * sa

        def norm01(c, carry):
            for g in range(16):
                wbuf[c, 16 * g:16 * g + 16, :] = norm2_rows(c, 16 * g, c, x1buf.at[c]).reshape(16, D)
            return carry
        lax.fori_loop(0, 2, norm01, 0)
    wait("wm2")
    with jax.named_scope("mod2"):
        sb, cb = mod_part(3, 5)
        modv[2] = 1.0 + cb
        modv[3] = sb
        for c in range(2):
            for g in range(8):
                top, bot = [mod2(wbuf[c, r:r + 16, :].reshape(2, 8, D)) for r in (16 * g, C + 16 * g)]
                store_lhs(lhsb, 64 * c + 8 * g, top, bot)
    dyn_step(2, "warm")
    wait("r1")

    def body(i, s):
        with jax.named_scope("step"):
            step(s, "main")
        return s + 2
    lax.fori_loop(0, 2, body, 3 + one)

    def tail(s, carry):
        with jax.named_scope("tail"):
            step(s, "last")
        return carry
    lax.fori_loop(8, 10, tail, 0)

    with jax.named_scope("wait_out"):
        out_copy(4).wait()
        for c in (6, 7):
            for part in last_parts:
                out_copy(c, *part).wait()


@jax.jit
def pallas_adaLN_cond__ssm_conv_h3__glu_gated_bilinear__prompt_kernel(A_q, A_k, A_v, A_shift_k, A_ssm_k, A_ssm_D, B_x, B_w_gate, B_w_up, B_w_down, c, w_mod):
    cst = jnp.asarray(_dft_consts(), dtype=BF16)
    any_spec = pl.BlockSpec(memory_space=pl.ANY)
    out = pl.pallas_call(
        _kernel,
        grid=(1,),
        in_specs=[any_spec] * 12,
        out_specs=any_spec,
        out_shape=jax.ShapeDtypeStruct((NC, M, D), BF16),
        scratch_shapes=[
            pltpu.VMEM((NC, M, D), BF16), pltpu.VMEM((NC, M, D), BF16), pltpu.VMEM((NC, M, D), BF16),
            pltpu.VMEM((D, S), BF16),
            pltpu.VMEM((D, FF), BF16), pltpu.VMEM((D, FF), BF16), pltpu.VMEM((FF, D), BF16),
            pltpu.VMEM((D, 6 * D), BF16),
            pltpu.VMEM((3 * C, C), BF16),
            pltpu.VMEM((NC, M, D), BF16),
            pltpu.VMEM((LT, 32 + S + 2 * M, 128), F32),
            pltpu.VMEM((NB + 1, LT, 16, 24, 128), F32),
            pltpu.VMEM((NB, LT, 16, 24, 128), F32),
            pltpu.VMEM((NC + 1, LT, 8, 32, 128), F32),
            pltpu.VMEM((3, LT, M, 128), F32),
            pltpu.VMEM((NC + 2, M, D), F32),
            pltpu.VMEM(((NC + 2) * 64, 16 * 128), U32),
            pltpu.VMEM((128 + 128, 96 * 128), U32),
            pltpu.VMEM((384 + 64, 16 * 128), U32),
            pltpu.VMEM((128 + 32, 9 * 640), U32),
            pltpu.VMEM((2 * 64, 9 * 128), U32),
            pltpu.VMEM((2, M, D), F32),
            pltpu.VMEM((8, 8, D), F32),
            pltpu.VMEM((4, 8, D), F32),
            pltpu.VMEM((4, D), BF16), pltpu.VMEM((D,), BF16), pltpu.VMEM((1, D), BF16),
            pltpu.VMEM((14, 1, 128), F32),
            pltpu.SemaphoreType.DMA((13,)),
            pltpu.SemaphoreType.DMA(()),
        ],
        compiler_params=pltpu.CompilerParams(vmem_limit_bytes=120 * 1024 * 1024),
        name="fused_h3_glu",
    )(A_q.reshape(NC, M, D), A_k.reshape(NC, M, D), A_v.reshape(NC, M, D), A_shift_k.T, A_ssm_k, A_ssm_D,
      B_w_gate, B_w_up, B_w_down, c, w_mod, cst)
    return out.reshape(1, S, D)
```

```python
import numpy as np
import jax
import jax.numpy as jnp
from jax import lax
import jax.experimental.pallas as pl
import jax.experimental.pallas.tpu as pltpu

S, D, FF = 2048, 640, 1536
C = 128
NB = S // C
M = 256
NC = S // M
LT = D // 128
EPS = 1e-5
F32 = jnp.float32
BF16 = jnp.bfloat16
U32 = jnp.uint32


def _dft_consts():
    r = np.arange(C)
    theta = np.pi * (4 * r + 1) / (2 * C)
    c = np.arange(C)
    ang = theta[:, None] * c[None, :]
    cs = np.stack([np.cos(ang), -np.sin(ang)], axis=0)
    fm = cs.reshape(2, 2, 8, 8, C).transpose(2, 1, 0, 3, 4).reshape(2 * C, C)
    a = np.concatenate([np.arange(0, C, 2), np.arange(1, C, 2)])
    ang2 = a[:, None] * theta[None, :64]
    g = np.zeros((C, 8, 2, 8))
    g[:, :, 0] = np.cos(ang2).reshape(C, 8, 8) / C
    g[:, :, 1] = -np.sin(ang2).reshape(C, 8, 8) / C
    g = g.reshape(C, C)
    return np.concatenate([fm, g], axis=0).astype(np.float32)


C_SLOTS = tuple(range(40, 80))
D_SLOT = 80
E_SLOTS = tuple(x for x in (86, 90, 94, 97, 97, 98, 99, 101, 102, 104, 105, 106, 108, 109, 111, 111) for _ in range(2))
WK_SLOTS = (68, 70, 72, 74, 76, 77, 78, 79)
WWK_SLOTS = (99, 100, 101, 102, 103, 104, 105, 106)
X_FAST = False
X_NOCHK = True
X_WKS = 4
WC_SLOTS = tuple(sorted(2 * list(range(60, 80))))
W_WAITS = {0: ("p0",), 16: ("p1",), 48: ("p3",), 80: ("p5",), 96: ("wd",)}
W_AB = 48
W_CMIN = 1
W_D = 80
W_MOD = 97
W_WIDE = False
WE_SLOTS = tuple(x for x in (87, 93, 99, 101, 104, 106, 109, 111) for _ in range(4))


def _mo(x, m):
    return x if isinstance(x, int) else pl.multiple_of(x, m)


def _ls(t):
    return slice(t * 128, (t + 1) * 128)


def _pack(x):
    return pltpu.bitcast(x.astype(BF16), U32)


def _asums(a11, a12, a21, a22):
    return [a11 + a22, a21 + a22, a11, a22, a11 + a12, a21 - a11, a12 - a22]


def _ln(x, fast=False):
    m = jnp.sum(x, axis=-1, keepdims=True) * (1.0 / D)
    if fast:
        ms = jnp.sum(x * x, axis=-1, keepdims=True) * (1.0 / D)
        return (x - m) * lax.rsqrt(jnp.maximum(ms - m * m, 0.0) + EPS)
    xc = x - m
    var = jnp.sum(xc * xc, axis=-1, keepdims=True) * (1.0 / D)
    return xc * lax.rsqrt(var + EPS)


def _kernel(q_h, k_h, v_h, sh_h, sk_h, sd_h, wg_h, wu_h, wd_h, c_h, wm_h, cst_h,
            o_h,
            q_v, k_v, v_v, sk_v, wg_v, wu_v, wd_v, wm_v, cst_v,
            o_v, kbuf, xf, kf, qbuf, ybuf, x1buf, lhsb, wgu, wdn, dlb, dl5, wbuf, modv, shb,
            sh_v, sd_v, c_v, pad_v,
            sem_in, sem_out):
    def k_in(c0, c1):
        return [(k_h.at[c0:c1], k_v.at[c0:c1])]

    def conv_in(c0, c1, with_k=True):
        cols = pl.ds(c0 * M, (c1 - c0) * M)
        return ([(sk_h.at[:, cols], sk_v.at[:, cols])] + (k_in(c0, c1) if with_k else [])
                + [(v_h.at[c0:c1], v_v.at[c0:c1])])

    def q_in(c0, c1):
        return [(q_h.at[c0:c1], q_v.at[c0:c1])]

    def gu_in(p0, p1):
        cols = pl.ds(p0 * 256, (p1 - p0) * 256)
        return [(wg_h.at[:, cols], wg_v.at[:, cols]), (wu_h.at[:, cols], wu_v.at[:, cols])]

    def wm_in(n0, n1):
        cols = pl.ds(n0 * D, (n1 - n0) * D)
        return [(wm_h.at[:, cols], wm_v.at[:, cols])]

    dma = dict(
        small=[(cst_h, cst_v), (sh_h, sh_v), (sd_h, sd_v), (c_h, c_v)],
        c0=conv_in(0, 1),
        c1=conv_in(1, 2),
        c2=conv_in(2, 3),
        wm1=q_in(0, 2) + wm_in(0, 3),
        wm2=wm_in(3, 5),
        p0=gu_in(0, 1),
        p1=gu_in(1, 3),
        p3=conv_in(3, 4) + gu_in(3, 5),
        p5=gu_in(5, 6) + q_in(2, 4),
        wd=wm_in(5, 6) + [(wd_h, wd_v)] + k_in(4, 6),
        r1=conv_in(4, 6, False) + k_in(6, 8),
        r2=q_in(4, 8) + conv_in(6, 8, False),
    )
    dma = {name: [pltpu.make_async_copy(a, b, sem_in.at[n]) for a, b in grp]
           for n, (name, grp) in enumerate(dma.items())}

    def wait(name):
        with jax.named_scope("w_" + name):
            for cp in dma[name]:
                cp.wait()

    def out_copy(i, rows=None, cols=None):
        if rows is None:
            return pltpu.make_async_copy(o_v.at[pl.ds(i, 2)], o_h.at[pl.ds(i, 2)], sem_out)
        return pltpu.make_async_copy(o_v.at[i, rows, cols], o_h.at[i, rows, cols], sem_out)

    last_parts = [(slice(None), _ls(4)), (slice(None), slice(0, 256)), (slice(C, M), _ls(2)),
                  (slice(0, C), _ls(3)), (slice(0, C), _ls(2)), (slice(C, M), _ls(3))]

    for grp in dma.values():
        for cp in grp:
            cp.start()

    for t in range(LT):
        kbuf[t, 24:32, :] = jnp.zeros((8, 128), F32)
    xf[0] = jnp.zeros((LT, 16, 24, 128), F32)
    qbuf[0] = jnp.zeros((LT, 8, 32, 128), F32)
    pad_v[...] = jnp.zeros(pad_v.shape, F32)
    wait("small")
    sh = sh_v[...].astype(F32)
    modv[5] = jnp.broadcast_to(sd_v[...].astype(F32).reshape(1, D), (8, D))
    modv[6] = jnp.zeros((8, D), F32)
    for j in range(4):
        shb[j] = jnp.broadcast_to(sh[j:j + 1, :], (8, D))

    def widen_next_k(s, part, gate):
        kbuf[0, pl.ds(pl.multiple_of(8 * (s % 2048), 8), 8), :] = gate
        r0 = _mo(s * M, M)
        n = 2 * M // (len(WK_SLOTS) * X_WKS)
        ch, r = divmod(part * n, M)
        kk = k_v[jnp.minimum(s + 2 + ch, NC - 1), r:r + n, :].astype(F32)
        for t in range(LT):
            kbuf[t, pl.ds(r0 + 32 + 2 * M + part * n, n), :] = kk[:, _ls(t)]

    def stage_a(c, t, widen=True):
        r0 = _mo(c * M, M)
        ls = _ls(t)
        if widen:
            kk = k_v[c, :, ls].astype(F32)
            kbuf[t, pl.ds(r0 + 32, M), :] = kk
        else:
            kk = kbuf[t, pl.ds(r0 + 32, M), :]
        acc = kk.reshape(32, 8, 128) * shb[0, :, ls][None]
        for j in range(1, 4):
            acc = acc + kbuf[t, pl.ds(r0 + 32 - j, M), :].reshape(32, 8, 128) * shb[j, :, ls][None]
        kv = acc.reshape(M, 128) * v_v[c, :, ls].astype(F32)
        for b in range(2):
            r = jnp.dot(cst_v[0:2 * C, :], kv[b * C:(b + 1) * C].astype(BF16),
                        preferred_element_type=F32).reshape(16, 16, 128)
            xf[2 * c + 1 + b, t, :, 0:16, :] = r
            xf[2 * c + 1 + b, t, :, 16:24, :] = r[:, 0:8, :] + r[:, 8:16, :]

    def stage_b(c, t, maybe_first=False):
        for b in range(2):
            kb = sk_v[_ls(t), pl.ds(_mo(c * M + b * C, C), C)]
            r = lax.dot_general(cst_v[0:2 * C, :], kb, (((1,), (1,)), ((), ())),
                                preferred_element_type=F32).reshape(16, 16, 128)
            cc = r[:, 0:8, :]
            d = r[:, 8:16, :]
            if maybe_first and b == 0:
                cc = cc + modv[5 + jnp.minimum(c, 1), :, _ls(t)][None]
            kf[2 * c + b, t, :, 0:8, :] = d - cc
            kf[2 * c + b, t, :, 8:16, :] = cc + d
            kf[2 * c + b, t, :, 16:24, :] = cc

    def lag_idx(c, cmin, cmax, nout):
        top = 2 * c + nout - 1
        nlag = 2 * cmax + nout
        jok = 2 * cmin + nout - 1
        kidx = [j if j <= jok else jnp.minimum(j, top) for j in range(nlag)]
        xidx = [top + 1 - j if j <= jok + 1 else jnp.maximum(top + 1 - j, 0) for j in range(nlag)]
        return kidx, xidx, nout

    def block_conv(idx, t, us):
        kidx, xidx, nout = idx
        xs = []
        acc = [None] * nout
        for j in reversed(range(len(kidx))):
            k = kf[kidx[j], t, us]
            xs = [xf[xidx[j], t, us]] + xs[:nout - 1]
            for o in reversed(range(len(xs))):
                p = k * xs[o]
                acc[o] = p if acc[o] is None else acc[o] + p
        return [(a[..., 16:24, :] - a[..., 8:16, :], a[..., 16:24, :] + a[..., 0:8, :]) for a in reversed(acc)]

    def cone(c, idx, t, u, pin=None):
        nout = idx[2]
        if nout == 2:
            ri = [((re[0], im[0]), (re[1], im[1])) for re, im in block_conv(idx, t, slice(2 * u, 2 * u + 2))]
        else:
            hs = []
            for h in range(2):
                hs.append(block_conv(idx, t, 2 * u + h))
                tot = [re + im for re, im in hs[h]]
                pin(h, (tot[0] + tot[1]) + (tot[2] + tot[3]))
            ri = list(zip(*hs))
        qs = [(h0[0] + h1[0], h0[1] + h1[1], h0[0] - h1[0], h0[1] - h1[1]) for h0, h1 in ri]
        qv = qbuf.at[pl.ds(c, nout // 2 + 1)]
        qv[nout // 2, t, u] = jnp.concatenate(qs[-1], axis=0)
        prev = qv[0, t, u]
        pv = (prev[0:8], prev[8:16], prev[16:24], prev[24:32])
        res = []
        for cur in qs:
            res.append(jnp.concatenate([cur[0] - pv[1], cur[1] + pv[0]], axis=0))
            res.append(jnp.concatenate([cur[2] - pv[3], cur[3] + pv[2]], axis=0))
            pv = cur
        return res

    def stage_d(yi, t, wfn):
        for b in range(2):
            for par in range(2):
                g = cst_v[2 * C + 64 * par:2 * C + 64 * (par + 1), :]
                y = jnp.dot(g, wfn(2 * b + par), preferred_element_type=F32)
                ybuf[yi, t, pl.ds(b * C + par, 64, stride=2), :] = y

    def ab_all(c):
        for t in range(LT):
            stage_b(c, t, True)
            stage_a(c, t)

    def cd_all(c, cmin, cmax):
        idx = lag_idx(c, cmin, cmax, 2)
        for t in range(LT):
            eo = [cone(c, idx, t, u) for u in range(8)]
            stage_d(c, t, lambda n: jnp.concatenate([e[n] for e in eo], axis=0).astype(BF16))

    def norm2_rows(c, r0, yi, x1dst):
        rows = slice(r0, r0 + 16)
        x = q_v[c, rows, :].astype(F32).reshape(2, 8, D)
        y = jnp.concatenate([ybuf[yi, t, rows, :] for t in range(LT)], axis=1).reshape(2, 8, D)
        x1 = x + (_ln(x, X_FAST) * modv[0][None] + modv[1][None]) * y
        x1dst[rows, :] = x1.reshape(16, D)
        return _ln(x1, X_FAST)

    def mod2(n2):
        return (n2 * modv[2][None] + modv[3][None]).reshape(16, D)

    def store_lhs(dst, r8, top, bot):
        rows = slice(r8, r8 + 8)
        for kt in range(2):
            ss = _asums(top[:, _ls(kt)], top[:, _ls(2 + kt)], bot[:, _ls(kt)], bot[:, _ls(2 + kt)])
            for i in range(7):
                dst[rows, _ls(2 * i + kt)] = _pack(ss[i])
        dst[rows, _ls(14)] = _pack(top[:, _ls(4)])
        dst[rows, _ls(15)] = _pack(bot[:, _ls(4)])
        return ss[0]

    def mod_part(n0, n1):
        cf = c_v[...].astype(F32)
        sc = cf * (1.0 / (1.0 + jnp.exp(-cf)))
        lhs = jnp.broadcast_to(sc, (16, D)).astype(BF16)
        mod = jnp.dot(lhs, wm_v[:, n0 * D:n1 * D], preferred_element_type=F32)[0:8]
        return [mod[:, n * D:(n + 1) * D] for n in range(n1 - n0)]

    bspec = [((0, 0), 1, (1, 1)), ((0, 0), 0, None), ((0, 1), -1, (1, 1)), ((1, 0), -1, (0, 0)),
             ((1, 1), 0, None), ((0, 0), 1, (0, 1)), ((1, 0), 1, (1, 1))]

    def bsum(quad, i):
        qa, sign, qb = bspec[i]
        if sign == 0:
            return pltpu.bitcast(quad(*qa), U32)
        a = quad(*qa).astype(F32)
        b = quad(*qb).astype(F32)
        return _pack(a + b if sign > 0 else a - b)

    def prep_gu(col):
        p, mat, i = col // 16, (col // 8) % 2, col % 8
        w = (wg_v, wu_v)[mat]
        if i == 7:
            for cc in range(2):
                wgu[64 * cc:64 * cc + 64, _ls(col)] = pltpu.bitcast(w[512:640, _ls(2 * p + cc)], U32)
        else:
            wgu[0:128, _ls(col)] = bsum(lambda r, c: w[256 * r:256 * r + 256, _ls(2 * p + c)], i)

    def prep_dn(col):
        for p in range(6):
            if col >= 14:
                val = pltpu.bitcast(wd_v[_ls(2 * p + col - 14), _ls(4)], U32)
            else:
                val = bsum(lambda r, c: wd_v[_ls(2 * p + r), _ls(2 * (col // 7) + c)], col % 7)
            wdn[64 * p:64 * p + 64, _ls(col)] = val

    def step(s, mode):
        warm, main, last = mode == "warm", mode == "main", mode == "last"
        nch = 1 if last else 2
        R = 64 * nch
        off = 128 * (s % 2)
        lv = lhsb.at[pl.ds(pl.multiple_of((s - 2) * 64, 64), 2 * R)]
        x1v = x1buf.at[pl.ds(s - 2, 2 * nch)]
        dl_w = dlb.at[pl.ds(pl.multiple_of((s % 2) * 32, 32), R)]
        dl_r = dlb.at[pl.ds(pl.multiple_of(((s + 2) % 2) * 32, 32), R)]

        items = [[] for _ in range(112)]
        if warm:
            c0, nout = s + 1, 2
            idx = lag_idx(c0, W_CMIN, 3, nout)
            items[W_D].append(("d", 0))
            for m, names in W_WAITS.items():
                for name in names:
                    items[m].append(("w", name))
            items[W_AB].append(("ab", 0))
            items[W_MOD].append(("mod", 0))
            c_slots, e_slots, yis = WC_SLOTS, WE_SLOTS, (2, 0)
        elif main:
            c0, nout = s, 4
            idx = lag_idx(c0, 4, 6, nout)
            items[0].append(("ab", 0))
            items[D_SLOT].append(("d", 0))
            c_slots, e_slots, yis = C_SLOTS, E_SLOTS, (0, 1)
        if not last:
            for n, m in enumerate(WWK_SLOTS if warm else WK_SLOTS):
                items[m].append(("wk", n))
            for p in range(40):
                items[c_slots[p]].append(("c", p))
            for g in range(32):
                items[e_slots[g]].append(("e", g))
        tops, hist, where = {}, {}, {}
        slot = [0]

        def pin_rows(nrows, n):
            return pl.ds(_mo(nrows + off + 8 * n, 8), 8)

        def hook(ref, nrows, col):
            m = slot[0]
            slot[0] += 1
            npin = 0
            todo = [x for x in items[m] if x[0] not in ("c", "e")]
            if warm:
                todo.append(("prep", col))
            todo += [x for x in items[m] if x[0] in ("c", "e")]
            for kind, p in todo:
                if kind == "w":
                    wait(p)
                elif kind == "prep":
                    (prep_gu if m < 96 else prep_dn)(p)
                elif kind == "mod":
                    modv[4] = mod_part(5, 6)[0]
                elif kind == "ab":
                    if warm and W_WIDE:
                        rw = pl.multiple_of(8 * ((s + (32 + 3 * M) // 8 - 2) % 2048), 8)
                        kk = k_v[c0].astype(F32)
                        for t in range(LT):
                            kbuf[t, pl.ds(rw, M), :] = kk[:, _ls(t)]
                    for ch in range(nout // 2):
                        for t in range(LT):
                            stage_b(c0 + ch, t)
                            stage_a(c0 + ch, t, warm and not W_WIDE)
                elif kind == "wk":
                    for r in range(X_WKS):
                        r0 = 8 * (32 * r // X_WKS)
                        widen_next_k(s, X_WKS * p + r, hist[m - 1][r0:r0 + 8])
                elif kind == "d":
                    for ch in range(nout // 2):
                        for t in range(LT):
                            def wfn(n):
                                parts = []
                                for u in range(8):
                                    rf, nr, cl = where[8 * t + u]
                                    parts.append(rf[pin_rows(nr, 8 * ch + n), _ls(cl)])
                                return pltpu.bitcast(jnp.concatenate(parts, axis=0), BF16)
                            stage_d(ch, t, wfn)
                    if main:
                        out_copy(s - 4).wait()

                        @pl.when(s == 4)
                        def _():
                            wait("r2")
                elif kind == "c":
                    def pin(h, val):
                        ref[pin_rows(nrows, 15 - 3 * h), _ls(col)] = pltpu.bitcast(val, U32)
                    res = cone(c0, idx, p // 8, p % 8, pin)
                    n0 = (4 - npin) if warm else 0
                    for n in range(2 * nout):
                        ref[pin_rows(nrows, n0 + n % 4 + 8 * (n // 4)), _ls(col)] = _pack(res[n])
                    where[p] = (ref, nrows + 8 * n0, col)
                    npin += 2 * nout
                else:
                    ch, g, half = p // 16, (p % 16) // 2, p % 2
                    h2 = mod2(norm2_rows(s + ch, 16 * g + C * half, yis[ch], x1v.at[2 + ch]))
                    if half == 0:
                        tops[g] = h2
                        val = h2[:, _ls(4)]
                    else:
                        val = store_lhs(lv, R + 64 * ch + 8 * g, tops[g], h2)
                    ref[pin_rows(nrows, npin), _ls(col)] = _pack(val)
                    npin += 1
                assert npin <= 8

        def dot(a, w):
            r = jnp.dot(pltpu.bitcast(a, BF16), pltpu.bitcast(w, BF16), preferred_element_type=F32)
            hist.setdefault(slot[0] - 1, r)
            return r

        def strassen(lhs, ref, nrows, base, left):
            def m(i):
                hook(ref, nrows, base + i - 1)
                return dot(lhs(i - 1), ref[0:nrows, _ls(base + i - 1)])
            m2 = m(2)
            m4 = m(4)
            c21 = m2 + m4
            m3 = m(3)
            m5 = m(5)
            c12 = m3 + m5
            c11 = m4 - m5
            c22 = m3 - m2
            m1 = m(1)
            m7 = m(7)
            c11 = c11 + m1 + m7
            c22 = c22 + m1
            c22 = c22 + m(6)
            if left is not None:
                hook(ref, nrows, base + 7)
                c22 = c22 + left(1, 1)
                c11 = c11 + left(0, 0)
                c12 = c12 + left(0, 1)
                c21 = c21 + left(1, 0)
            return c11, c12, c21, c22

        for p in range(6):
            res = []
            for mat in range(2):
                base = (2 * p + mat) * 8
                res.append(strassen(
                    lambda i: lv[0:R, 256 * i:256 * i + 256], wgu, 128, base,
                    lambda r, c: dot(lv[0:R, _ls(14 + r)], wgu[64 * c:64 * c + 64, _ls(base + 7)])))
            hq = [res[0][i] * res[1][i] for i in range(4)]
            for i, x in enumerate(_asums(*hq) + [hq[1], hq[2]]):
                if p < 5:
                    dl_w[:, _ls(5 * i + p)] = _pack(x)
                else:
                    dl5[0:R, _ls(i)] = _pack(x)

        def dla(i):
            return dl_r[:, 640 * i:640 * i + 640]

        def dlz(i):
            return dl5[0:R, _ls(i)]

        def dl(i):
            return jnp.concatenate([dla(i), dlz(i)], axis=1)

        def emit(r, n, o):
            rows = slice(r * C, (r + 1) * C)
            for ch in range(nch):
                res = (x1v[ch, rows, _ls(n)].reshape(16, 8, 128)
                       + o[ch * C:(ch + 1) * C].reshape(16, 8, 128) * modv[4, :, _ls(n)][None])
                o_v[s - 2 + ch, rows, _ls(n)] = res.reshape(C, 128).astype(BF16)

        hook(wdn, 384, 14)
        ta = dot(dla(2), wdn[0:320, _ls(14)])
        tb = dot(dla(8), wdn[0:320, _ls(14)])
        ta = ta + dot(dlz(2), wdn[320:384, _ls(14)])
        tb = tb + dot(dlz(8), wdn[320:384, _ls(14)])
        hook(wdn, 384, 15)
        emit(0, 4, ta + dot(dl(7), wdn[0:384, _ls(15)]))
        emit(1, 4, tb + dot(dl(3), wdn[0:384, _ls(15)]))
        if last:
            out_copy(s - 2, *last_parts[0]).start()
        for pp in range(2):
            cs = strassen(dl, wdn, 384, 7 * pp, None)
            for n, i in enumerate((2, 1, 0, 3)):
                emit(i // 2, 2 * pp + i % 2, cs[i])
                if last and pp == 1:
                    out_copy(s - 2, *last_parts[2 + n]).start()
            if last and pp == 0:
                out_copy(s - 2, *last_parts[1]).start()
        if not last:
            out_copy(s - 2).start()

    def conv012(c, carry):
        for n in range(3):
            @pl.when(c == n)
            def _():
                wait("c%d" % n)
        with jax.named_scope("ab"):
            ab_all(c)

        @pl.when(c == 0)
        def _():
            with jax.named_scope("cd0"):
                cd_all(c, 0, 0)

        @pl.when(c > 0)
        def _():
            with jax.named_scope("cd12"):
                cd_all(c, 1, 2)
        return carry
    lax.fori_loop(0, 3, conv012, 0)
    wait("wm1")
    with jax.named_scope("mod1"):
        sa, ca, ga = mod_part(0, 3)
        modv[0] = ga * (1.0 + ca)
        modv[1] = ga * sa

        def norm01(c, carry):
            for g in range(16):
                wbuf[c, 16 * g:16 * g + 16, :] = norm2_rows(c, 16 * g, c, x1buf.at[c]).reshape(16, D)
            return carry
        lax.fori_loop(0, 2, norm01, 0)
    wait("wm2")
    with jax.named_scope("mod2"):
        sb, cb = mod_part(3, 5)
        modv[2] = 1.0 + cb
        modv[3] = sb
        for c in range(2):
            for g in range(8):
                top, bot = [mod2(wbuf[c, r:r + 16, :].reshape(2, 8, D)) for r in (16 * g, C + 16 * g)]
                store_lhs(lhsb, 64 * c + 8 * g, top, bot)
    def passes(i, s):
        @pl.when(i == 0)
        def _():
            with jax.named_scope("warm"):
                step(s, "warm")
            wait("r1")

        @pl.when(jnp.logical_and(i > 0, i < 3))
        def _():
            with jax.named_scope("main"):
                step(s, "main")

        @pl.when(i >= 3)
        def _():
            with jax.named_scope("tail"):
                step(s, "last")
        return s + jnp.where(i < 3, 2, 1)
    lax.fori_loop(0, 5, passes, 2)

    with jax.named_scope("wait_out"):
        out_copy(4).wait()
        for c in (6, 7):
            for part in last_parts:
                out_copy(c, *part).wait()


@jax.jit
def pallas_adaLN_cond__ssm_conv_h3__glu_gated_bilinear__prompt_kernel(A_q, A_k, A_v, A_shift_k, A_ssm_k, A_ssm_D, B_x, B_w_gate, B_w_up, B_w_down, c, w_mod):
    cst = jnp.asarray(_dft_consts(), dtype=BF16)
    any_spec = pl.BlockSpec(memory_space=pl.ANY)
    out = pl.pallas_call(
        _kernel,
        grid=(1,),
        in_specs=[any_spec] * 12,
        out_specs=any_spec,
        out_shape=jax.ShapeDtypeStruct((NC, M, D), BF16),
        scratch_shapes=[
            pltpu.VMEM((NC, M, D), BF16), pltpu.VMEM((NC, M, D), BF16), pltpu.VMEM((NC, M, D), BF16),
            pltpu.VMEM((D, S), BF16),
            pltpu.VMEM((D, FF), BF16), pltpu.VMEM((D, FF), BF16), pltpu.VMEM((FF, D), BF16),
            pltpu.VMEM((D, 6 * D), BF16),
            pltpu.VMEM((3 * C, C), BF16),
            pltpu.VMEM((NC, M, D), BF16),
            pltpu.VMEM((LT, 32 + S + 2 * M, 128), F32),
            pltpu.VMEM((NB + 1, LT, 16, 24, 128), F32),
            pltpu.VMEM((NB, LT, 16, 24, 128), F32),
            pltpu.VMEM((NC + 1, LT, 8, 32, 128), F32),
            pltpu.VMEM((3, LT, M, 128), F32),
            pltpu.VMEM((NC + 2, M, D), F32),
            pltpu.VMEM(((NC + 2) * 64, 16 * 128), U32),
            pltpu.VMEM((128 + 128, 96 * 128), U32),
            pltpu.VMEM((384 + 64, 16 * 128), U32),
            pltpu.VMEM((128 + 32, 9 * 640), U32),
            pltpu.VMEM((2 * 64, 9 * 128), U32),
            pltpu.VMEM((2, M, D), F32),
            pltpu.VMEM((8, 8, D), F32),
            pltpu.VMEM((4, 8, D), F32),
            pltpu.VMEM((4, D), BF16), pltpu.VMEM((D,), BF16), pltpu.VMEM((1, D), BF16),
            pltpu.VMEM((14, 1, 128), F32),
            pltpu.SemaphoreType.DMA((13,)),
            pltpu.SemaphoreType.DMA(()),
        ],
        compiler_params=pltpu.CompilerParams(vmem_limit_bytes=120 * 1024 * 1024,
                                             disable_bounds_checks=X_NOCHK, disable_semaphore_checks=X_NOCHK),
        name="fused_h3_glu",
    )(A_q.reshape(NC, M, D), A_k.reshape(NC, M, D), A_v.reshape(NC, M, D), A_shift_k.T, A_ssm_k, A_ssm_D,
      B_w_gate, B_w_up, B_w_down, c, w_mod, cst)
    return out.reshape(1, S, D)
```

```python
import numpy as np
import jax
import jax.numpy as jnp
from jax import lax
import jax.experimental.pallas as pl
import jax.experimental.pallas.tpu as pltpu

S, D, FF = 2048, 640, 1536
C = 128
NB = S // C
M = 256
NC = S // M
LT = D // 128
EPS = 1e-5
F32 = jnp.float32
BF16 = jnp.bfloat16
U32 = jnp.uint32


def _dft_consts():
    r = np.arange(C)
    theta = np.pi * (4 * r + 1) / (2 * C)
    c = np.arange(C)
    ang = theta[:, None] * c[None, :]
    cs = np.stack([np.cos(ang), -np.sin(ang)], axis=0)
    fm = cs.reshape(2, 2, 8, 8, C).transpose(2, 1, 0, 3, 4).reshape(2 * C, C)
    a = np.concatenate([np.arange(0, C, 2), np.arange(1, C, 2)])
    ang2 = a[:, None] * theta[None, :64]
    g = np.zeros((C, 8, 2, 8))
    g[:, :, 0] = np.cos(ang2).reshape(C, 8, 8) / C
    g[:, :, 1] = -np.sin(ang2).reshape(C, 8, 8) / C
    g = g.reshape(C, C)
    return np.concatenate([fm, g], axis=0).astype(np.float32)


C_SLOTS = tuple(range(40, 80))
D_SLOT = 80
E_SLOTS = tuple(x for x in (86, 90, 94, 97, 97, 98, 99, 101, 102, 104, 105, 106, 108, 109, 111, 111) for _ in range(2))
WK_SLOTS = (68, 70, 72, 74, 76, 77, 78, 79)
WWK_SLOTS = (99, 100, 101, 102, 103, 104, 105, 106)
X_FAST = False
X_NOCHK = True
X_WKS = 4
WC_SLOTS = tuple(sorted(2 * list(range(60, 80))))
W_WAITS = {0: ("p0",), 16: ("p1",), 48: ("p3",), 80: ("p5",), 96: ("wd",)}
W_AB = 48
W_CMIN = 1
W_D = 80
W_MOD = 97
W_WIDE = False
WE_SLOTS = tuple(x for x in (87, 93, 99, 101, 104, 106, 109, 111) for _ in range(4))


def _mo(x, m):
    return x if isinstance(x, int) else pl.multiple_of(x, m)


def _ls(t):
    return slice(t * 128, (t + 1) * 128)


def _pack(x):
    return pltpu.bitcast(x.astype(BF16), U32)


def _asums(a11, a12, a21, a22):
    return [a11 + a22, a21 + a22, a11, a22, a11 + a12, a21 - a11, a12 - a22]


def _ln(x, fast=False):
    m = jnp.sum(x, axis=-1, keepdims=True) * (1.0 / D)
    if fast:
        ms = jnp.sum(x * x, axis=-1, keepdims=True) * (1.0 / D)
        return (x - m) * lax.rsqrt(jnp.maximum(ms - m * m, 0.0) + EPS)
    xc = x - m
    var = jnp.sum(xc * xc, axis=-1, keepdims=True) * (1.0 / D)
    return xc * lax.rsqrt(var + EPS)


def _kernel(q_h, k_h, v_h, sh_h, sk_h, sd_h, wg_h, wu_h, wd_h, c_h, wm_h, cst_h,
            o_h,
            q_v, k_v, v_v, sk_v, wg_v, wu_v, wd_v, wm_v, cst_v,
            o_v, kbuf, xf, kf, qbuf, ybuf, x1buf, lhsb, wgu, wdn, dlb, dl5, wbuf, modv, shb,
            sh_v, sd_v, c_v, pad_v,
            sem_in, sem_out):
    def k_in(c0, c1):
        return [(k_h.at[c0:c1], k_v.at[c0:c1])]

    def conv_in(c0, c1, with_k=True):
        cols = pl.ds(c0 * M, (c1 - c0) * M)
        return ([(sk_h.at[:, cols], sk_v.at[:, cols])] + (k_in(c0, c1) if with_k else [])
                + [(v_h.at[c0:c1], v_v.at[c0:c1])])

    def q_in(c0, c1):
        return [(q_h.at[c0:c1], q_v.at[c0:c1])]

    def gu_in(p0, p1):
        cols = pl.ds(p0 * 256, (p1 - p0) * 256)
        return [(wg_h.at[:, cols], wg_v.at[:, cols]), (wu_h.at[:, cols], wu_v.at[:, cols])]

    def wm_in(n0, n1):
        cols = pl.ds(n0 * D, (n1 - n0) * D)
        return [(wm_h.at[:, cols], wm_v.at[:, cols])]

    dma = dict(
        small=[(cst_h, cst_v), (sh_h, sh_v), (sd_h, sd_v), (c_h, c_v)],
        c0=conv_in(0, 1),
        c1=conv_in(1, 2),
        c2=conv_in(2, 3),
        wm1=q_in(0, 2) + wm_in(0, 3),
        wm2=wm_in(3, 5),
        p0=gu_in(0, 1),
        p1=gu_in(1, 3),
        p3=conv_in(3, 4) + gu_in(3, 5),
        p5=gu_in(5, 6) + q_in(2, 4),
        wd=wm_in(5, 6) + [(wd_h, wd_v)] + k_in(4, 6),
        r1=conv_in(4, 6, False) + k_in(6, 8),
        r2=q_in(4, 8) + conv_in(6, 8, False),
    )
    dma = {name: [pltpu.make_async_copy(a, b, sem_in.at[n]) for a, b in grp]
           for n, (name, grp) in enumerate(dma.items())}

    def wait(name):
        with jax.named_scope("w_" + name):
            for cp in dma[name]:
                cp.wait()

    def out_copy(i, rows=None, cols=None):
        if rows is None:
            return pltpu.make_async_copy(o_v.at[pl.ds(i, 2)], o_h.at[pl.ds(i, 2)], sem_out)
        return pltpu.make_async_copy(o_v.at[i, rows, cols], o_h.at[i, rows, cols], sem_out)

    last_parts = [(slice(None), _ls(4)), (slice(None), slice(0, 256)), (slice(C, M), _ls(2)),
                  (slice(0, C), _ls(3)), (slice(0, C), _ls(2)), (slice(C, M), _ls(3))]

    for grp in dma.values():
        for cp in grp:
            cp.start()

    for t in range(LT):
        kbuf[t, 24:32, :] = jnp.zeros((8, 128), F32)
    xf[0] = jnp.zeros((LT, 16, 24, 128), F32)
    qbuf[0] = jnp.zeros((LT, 8, 32, 128), F32)
    pad_v[...] = jnp.zeros(pad_v.shape, F32)
    wait("small")
    sh = sh_v[...].astype(F32)
    modv[5] = jnp.broadcast_to(sd_v[...].astype(F32).reshape(1, D), (8, D))
    modv[6] = jnp.zeros((8, D), F32)
    for j in range(4):
        shb[j] = jnp.broadcast_to(sh[j:j + 1, :], (8, D))

    def widen_next_k(s, part, gate):
        kbuf[0, pl.ds(pl.multiple_of(8 * (s % 2048), 8), 8), :] = gate
        r0 = _mo(s * M, M)
        n = 2 * M // (len(WK_SLOTS) * X_WKS)
        ch, r = divmod(part * n, M)
        kk = k_v[jnp.minimum(s + 2 + ch, NC - 1), r:r + n, :].astype(F32)
        for t in range(LT):
            kbuf[t, pl.ds(r0 + 32 + 2 * M + part * n, n), :] = kk[:, _ls(t)]

    def stage_a(c, t, widen=True):
        r0 = _mo(c * M, M)
        ls = _ls(t)
        if widen:
            kk = k_v[c, :, ls].astype(F32)
            kbuf[t, pl.ds(r0 + 32, M), :] = kk
        else:
            kk = kbuf[t, pl.ds(r0 + 32, M), :]
        acc = kk.reshape(32, 8, 128) * shb[0, :, ls][None]
        for j in range(1, 4):
            acc = acc + kbuf[t, pl.ds(r0 + 32 - j, M), :].reshape(32, 8, 128) * shb[j, :, ls][None]
        kv = acc.reshape(M, 128) * v_v[c, :, ls].astype(F32)
        for b in range(2):
            r = jnp.dot(cst_v[0:2 * C, :], kv[b * C:(b + 1) * C].astype(BF16),
                        preferred_element_type=F32).reshape(16, 16, 128)
            xf[2 * c + 1 + b, t, :, 0:16, :] = r
            xf[2 * c + 1 + b, t, :, 16:24, :] = r[:, 0:8, :] + r[:, 8:16, :]

    def stage_b(c, t, maybe_first=False):
        for b in range(2):
            kb = sk_v[_ls(t), pl.ds(_mo(c * M + b * C, C), C)]
            r = lax.dot_general(cst_v[0:2 * C, :], kb, (((1,), (1,)), ((), ())),
                                preferred_element_type=F32).reshape(16, 16, 128)
            cc = r[:, 0:8, :]
            d = r[:, 8:16, :]
            if maybe_first and b == 0:
                cc = cc + modv[5 + jnp.minimum(c, 1), :, _ls(t)][None]
            kf[2 * c + b, t, :, 0:8, :] = d - cc
            kf[2 * c + b, t, :, 8:16, :] = cc + d
            kf[2 * c + b, t, :, 16:24, :] = cc

    def lag_idx(c, cmin, cmax, nout):
        top = 2 * c + nout - 1
        nlag = 2 * cmax + nout
        jok = 2 * cmin + nout - 1
        kidx = [j if j <= jok else jnp.minimum(j, top) for j in range(nlag)]
        xidx = [top + 1 - j if j <= jok + 1 else jnp.maximum(top + 1 - j, 0) for j in range(nlag)]
        return kidx, xidx, nout

    def block_conv(idx, t, us):
        kidx, xidx, nout = idx
        xs = []
        acc = [None] * nout
        for j in reversed(range(len(kidx))):
            k = kf[kidx[j], t, us]
            xs = [xf[xidx[j], t, us]] + xs[:nout - 1]
            for o in reversed(range(len(xs))):
                p = k * xs[o]
                acc[o] = p if acc[o] is None else acc[o] + p
        return [(a[..., 16:24, :] - a[..., 8:16, :], a[..., 16:24, :] + a[..., 0:8, :]) for a in reversed(acc)]

    def cone(c, idx, t, u, pin=None):
        nout = idx[2]
        if nout == 2:
            ri = [((re[0], im[0]), (re[1], im[1])) for re, im in block_conv(idx, t, slice(2 * u, 2 * u + 2))]
        else:
            hs = []
            for h in range(2):
                hs.append(block_conv(idx, t, 2 * u + h))
                tot = [re + im for re, im in hs[h]]
                pin(h, (tot[0] + tot[1]) + (tot[2] + tot[3]))
            ri = list(zip(*hs))
        qs = [(h0[0] + h1[0], h0[1] + h1[1], h0[0] - h1[0], h0[1] - h1[1]) for h0, h1 in ri]
        qv = qbuf.at[pl.ds(c, nout // 2 + 1)]
        qv[nout // 2, t, u] = jnp.concatenate(qs[-1], axis=0)
        prev = qv[0, t, u]
        pv = (prev[0:8], prev[8:16], prev[16:24], prev[24:32])
        res = []
        for cur in qs:
            res.append(jnp.concatenate([cur[0] - pv[1], cur[1] + pv[0]], axis=0))
            res.append(jnp.concatenate([cur[2] - pv[3], cur[3] + pv[2]], axis=0))
            pv = cur
        return res

    def stage_d(yi, t, wfn):
        for b in range(2):
            for par in range(2):
                g = cst_v[2 * C + 64 * par:2 * C + 64 * (par + 1), :]
                y = jnp.dot(g, wfn(2 * b + par), preferred_element_type=F32)
                ybuf[yi, t, pl.ds(b * C + par, 64, stride=2), :] = y

    def ab_all(c):
        for t in range(LT):
            stage_b(c, t, True)
            stage_a(c, t)

    def cd_all(c, cmin, cmax):
        idx = lag_idx(c, cmin, cmax, 2)
        for t in range(LT):
            eo = [cone(c, idx, t, u) for u in range(8)]
            stage_d(c, t, lambda n: jnp.concatenate([e[n] for e in eo], axis=0).astype(BF16))

    def norm2_rows(c, r0, yi, x1dst):
        rows = slice(r0, r0 + 16)
        x = q_v[c, rows, :].astype(F32).reshape(2, 8, D)
        y = jnp.concatenate([ybuf[yi, t, rows, :] for t in range(LT)], axis=1).reshape(2, 8, D)
        x1 = x + (_ln(x, X_FAST) * modv[0][None] + modv[1][None]) * y
        x1dst[rows, :] = x1.reshape(16, D)
        return _ln(x1, X_FAST)

    def mod2(n2):
        return (n2 * modv[2][None] + modv[3][None]).reshape(16, D)

    def store_lhs(dst, r8, top, bot):
        rows = slice(r8, r8 + 8)
        for kt in range(2):
            ss = _asums(top[:, _ls(kt)], top[:, _ls(2 + kt)], bot[:, _ls(kt)], bot[:, _ls(2 + kt)])
            for i in range(7):
                dst[rows, _ls(2 * i + kt)] = _pack(ss[i])
        dst[rows, _ls(14)] = _pack(top[:, _ls(4)])
        dst[rows, _ls(15)] = _pack(bot[:, _ls(4)])
        return ss[0]

    def mod_part(n0, n1):
        cf = c_v[...].astype(F32)
        sc = cf * (1.0 / (1.0 + jnp.exp(-cf)))
        lhs = jnp.broadcast_to(sc, (16, D)).astype(BF16)
        mod = jnp.dot(lhs, wm_v[:, n0 * D:n1 * D], preferred_element_type=F32)[0:8]
        return [mod[:, n * D:(n + 1) * D] for n in range(n1 - n0)]

    bspec = [((0, 0), (1, 1)), ((0, 0), None), ((0, 1), (1, 1)), ((1, 0), (0, 0)),
             ((1, 1), None), ((0, 0), (0, 1)), ((1, 0), (1, 1))]

    def bsum(quad, i):
        qa, qb = bspec[i]
        if qb is None:
            return pltpu.bitcast(quad(*qa), U32)
        return _pack(quad(*qa).astype(F32) - quad(*qb).astype(F32))

    def prep_gu(col):
        p, mat, i = col // 16, (col // 8) % 2, col % 8
        w = (wg_v, wu_v)[mat]
        if i == 7:
            for cc in range(2):
                wgu[64 * cc:64 * cc + 64, _ls(col)] = pltpu.bitcast(w[512:640, _ls(2 * p + cc)], U32)
        else:
            wgu[0:128, _ls(col)] = bsum(lambda r, c: w[256 * r:256 * r + 256, _ls(2 * p + c)], i)

    def prep_dn(col):
        for p in range(6):
            if col >= 14:
                val = pltpu.bitcast(wd_v[_ls(2 * p + col - 14), _ls(4)], U32)
            else:
                val = bsum(lambda r, c: wd_v[_ls(2 * p + r), _ls(2 * (col // 7) + c)], col % 7)
            wdn[64 * p:64 * p + 64, _ls(col)] = val

    def step(s, mode):
        warm, main, last = mode == "warm", mode == "main", mode == "last"
        nch = 1 if last else 2
        R = 64 * nch
        off = 128 * (s % 2)
        lv = lhsb.at[pl.ds(pl.multiple_of((s - 2) * 64, 64), 2 * R)]
        x1v = x1buf.at[pl.ds(s - 2, 2 * nch)]
        dl_w = dlb.at[pl.ds(pl.multiple_of((s % 2) * 32, 32), R)]
        dl_r = dlb.at[pl.ds(pl.multiple_of(((s + 2) % 2) * 32, 32), R)]

        items = [[] for _ in range(112)]
        if warm:
            c0, nout = s + 1, 2
            idx = lag_idx(c0, W_CMIN, 3, nout)
            items[W_D].append(("d", 0))
            for m, names in W_WAITS.items():
                for name in names:
                    items[m].append(("w", name))
            items[W_AB].append(("ab", 0))
            items[W_MOD].append(("mod", 0))
            c_slots, e_slots, yis = WC_SLOTS, WE_SLOTS, (2, 0)
        elif main:
            c0, nout = s, 4
            idx = lag_idx(c0, 4, 6, nout)
            items[0].append(("ab", 0))
            items[D_SLOT].append(("d", 0))
            c_slots, e_slots, yis = C_SLOTS, E_SLOTS, (0, 1)
        if not last:
            for n, m in enumerate(WWK_SLOTS if warm else WK_SLOTS):
                items[m].append(("wk", n))
            for p in range(40):
                items[c_slots[p]].append(("c", p))
            for g in range(32):
                items[e_slots[g]].append(("e", g))
        tops, hist, where = {}, {}, {}
        slot = [0]

        def pin_rows(nrows, n):
            return pl.ds(_mo(nrows + off + 8 * n, 8), 8)

        def hook(ref, nrows, col):
            m = slot[0]
            slot[0] += 1
            npin = 0
            todo = [x for x in items[m] if x[0] not in ("c", "e")]
            if warm:
                todo.append(("prep", col))
            todo += [x for x in items[m] if x[0] in ("c", "e")]
            for kind, p in todo:
                if kind == "w":
                    wait(p)
                elif kind == "prep":
                    (prep_gu if m < 96 else prep_dn)(p)
                elif kind == "mod":
                    modv[4] = mod_part(5, 6)[0]
                elif kind == "ab":
                    if warm and W_WIDE:
                        rw = pl.multiple_of(8 * ((s + (32 + 3 * M) // 8 - 2) % 2048), 8)
                        kk = k_v[c0].astype(F32)
                        for t in range(LT):
                            kbuf[t, pl.ds(rw, M), :] = kk[:, _ls(t)]
                    for ch in range(nout // 2):
                        for t in range(LT):
                            stage_b(c0 + ch, t)
                            stage_a(c0 + ch, t, warm and not W_WIDE)
                elif kind == "wk":
                    for r in range(X_WKS):
                        r0 = 8 * (32 * r // X_WKS)
                        widen_next_k(s, X_WKS * p + r, hist[m - 1][r0:r0 + 8])
                elif kind == "d":
                    for ch in range(nout // 2):
                        for t in range(LT):
                            def wfn(n):
                                parts = []
                                for u in range(8):
                                    rf, nr, cl = where[8 * t + u]
                                    parts.append(rf[pin_rows(nr, 8 * ch + n), _ls(cl)])
                                return pltpu.bitcast(jnp.concatenate(parts, axis=0), BF16)
                            stage_d(ch, t, wfn)
                    if main:
                        out_copy(s - 4).wait()

                        @pl.when(s == 4)
                        def _():
                            wait("r2")
                elif kind == "c":
                    def pin(h, val):
                        ref[pin_rows(nrows, 15 - 3 * h), _ls(col)] = pltpu.bitcast(val, U32)
                    res = cone(c0, idx, p // 8, p % 8, pin)
                    n0 = (4 - npin) if warm else 0
                    for n in range(2 * nout):
                        ref[pin_rows(nrows, n0 + n % 4 + 8 * (n // 4)), _ls(col)] = _pack(res[n])
                    where[p] = (ref, nrows + 8 * n0, col)
                    npin += 2 * nout
                else:
                    ch, g, half = p // 16, (p % 16) // 2, p % 2
                    h2 = mod2(norm2_rows(s + ch, 16 * g + C * half, yis[ch], x1v.at[2 + ch]))
                    if half == 0:
                        tops[g] = h2
                        val = h2[:, _ls(4)]
                    else:
                        val = store_lhs(lv, R + 64 * ch + 8 * g, tops[g], h2)
                    ref[pin_rows(nrows, npin), _ls(col)] = _pack(val)
                    npin += 1
                assert npin <= 8

        def dot(a, w):
            r = jnp.dot(pltpu.bitcast(a, BF16), pltpu.bitcast(w, BF16), preferred_element_type=F32)
            hist.setdefault(slot[0] - 1, r)
            return r

        def strassen(lhs, ref, nrows, base, left):
            def m(i):
                hook(ref, nrows, base + i - 1)
                return dot(lhs(i - 1), ref[0:nrows, _ls(base + i - 1)])
            m2 = m(2)
            m4 = m(4)
            c21 = m2 + m4
            m3 = m(3)
            m5 = m(5)
            c12 = m3 + m5
            c11 = m4 + m5
            c22 = m3 + m2
            m1 = m(1)
            m7 = m(7)
            c11 = c11 + m1 + m7
            c22 = c22 - m1
            c22 = c22 - m(6)
            if left is not None:
                hook(ref, nrows, base + 7)
                c22 = c22 + left(1, 1)
                c11 = c11 + left(0, 0)
                c12 = c12 + left(0, 1)
                c21 = c21 + left(1, 0)
            return c11, c12, c21, c22

        for p in range(6):
            res = []
            for mat in range(2):
                base = (2 * p + mat) * 8
                res.append(strassen(
                    lambda i: lv[0:R, 256 * i:256 * i + 256], wgu, 128, base,
                    lambda r, c: dot(lv[0:R, _ls(14 + r)], wgu[64 * c:64 * c + 64, _ls(base + 7)])))
            hq = [res[0][i] * res[1][i] for i in range(4)]
            for i, x in enumerate(_asums(*hq) + [hq[1], hq[2]]):
                if p < 5:
                    dl_w[:, _ls(5 * i + p)] = _pack(x)
                else:
                    dl5[0:R, _ls(i)] = _pack(x)

        def dla(i):
            return dl_r[:, 640 * i:640 * i + 640]

        def dlz(i):
            return dl5[0:R, _ls(i)]

        def dl(i):
            return jnp.concatenate([dla(i), dlz(i)], axis=1)

        def emit(r, n, o):
            rows = slice(r * C, (r + 1) * C)
            for ch in range(nch):
                res = (x1v[ch, rows, _ls(n)].reshape(16, 8, 128)
                       + o[ch * C:(ch + 1) * C].reshape(16, 8, 128) * modv[4, :, _ls(n)][None])
                o_v[s - 2 + ch, rows, _ls(n)] = res.reshape(C, 128).astype(BF16)

        hook(wdn, 384, 14)
        ta = dot(dla(2), wdn[0:320, _ls(14)])
        tb = dot(dla(8), wdn[0:320, _ls(14)])
        ta = ta + dot(dlz(2), wdn[320:384, _ls(14)])
        tb = tb + dot(dlz(8), wdn[320:384, _ls(14)])
        hook(wdn, 384, 15)
        emit(0, 4, ta + dot(dl(7), wdn[0:384, _ls(15)]))
        emit(1, 4, tb + dot(dl(3), wdn[0:384, _ls(15)]))
        if last:
            out_copy(s - 2, *last_parts[0]).start()
        for pp in range(2):
            cs = strassen(dl, wdn, 384, 7 * pp, None)
            for n, i in enumerate((2, 1, 0, 3)):
                emit(i // 2, 2 * pp + i % 2, cs[i])
                if last and pp == 1:
                    out_copy(s - 2, *last_parts[2 + n]).start()
            if last and pp == 0:
                out_copy(s - 2, *last_parts[1]).start()
        if not last:
            out_copy(s - 2).start()

    def conv012(c, carry):
        for n in range(3):
            @pl.when(c == n)
            def _():
                wait("c%d" % n)
        with jax.named_scope("ab"):
            ab_all(c)

        @pl.when(c == 0)
        def _():
            with jax.named_scope("cd0"):
                cd_all(c, 0, 0)

        @pl.when(c > 0)
        def _():
            with jax.named_scope("cd12"):
                cd_all(c, 1, 2)
        return carry
    lax.fori_loop(0, 3, conv012, 0)
    wait("wm1")
    with jax.named_scope("mod1"):
        sa, ca, ga = mod_part(0, 3)
        modv[0] = ga * (1.0 + ca)
        modv[1] = ga * sa

        def norm01(c, carry):
            for g in range(16):
                wbuf[c, 16 * g:16 * g + 16, :] = norm2_rows(c, 16 * g, c, x1buf.at[c]).reshape(16, D)
            return carry
        lax.fori_loop(0, 2, norm01, 0)
    wait("wm2")
    with jax.named_scope("mod2"):
        sb, cb = mod_part(3, 5)
        modv[2] = 1.0 + cb
        modv[3] = sb
        for c in range(2):
            for g in range(8):
                top, bot = [mod2(wbuf[c, r:r + 16, :].reshape(2, 8, D)) for r in (16 * g, C + 16 * g)]
                store_lhs(lhsb, 64 * c + 8 * g, top, bot)
    def passes(i, s):
        @pl.when(i == 0)
        def _():
            with jax.named_scope("warm"):
                step(s, "warm")
            wait("r1")

        @pl.when(jnp.logical_and(i > 0, i < 3))
        def _():
            with jax.named_scope("main"):
                step(s, "main")

        @pl.when(i >= 3)
        def _():
            with jax.named_scope("tail"):
                step(s, "last")
        return s + jnp.where(i < 3, 2, 1)
    lax.fori_loop(0, 5, passes, 2)

    with jax.named_scope("wait_out"):
        out_copy(4).wait()
        for c in (6, 7):
            for part in last_parts:
                out_copy(c, *part).wait()


@jax.jit
def pallas_adaLN_cond__ssm_conv_h3__glu_gated_bilinear__prompt_kernel(A_q, A_k, A_v, A_shift_k, A_ssm_k, A_ssm_D, B_x, B_w_gate, B_w_up, B_w_down, c, w_mod):
    cst = jnp.asarray(_dft_consts(), dtype=BF16)
    any_spec = pl.BlockSpec(memory_space=pl.ANY)
    out = pl.pallas_call(
        _kernel,
        grid=(1,),
        in_specs=[any_spec] * 12,
        out_specs=any_spec,
        out_shape=jax.ShapeDtypeStruct((NC, M, D), BF16),
        scratch_shapes=[
            pltpu.VMEM((NC, M, D), BF16), pltpu.VMEM((NC, M, D), BF16), pltpu.VMEM((NC, M, D), BF16),
            pltpu.VMEM((D, S), BF16),
            pltpu.VMEM((D, FF), BF16), pltpu.VMEM((D, FF), BF16), pltpu.VMEM((FF, D), BF16),
            pltpu.VMEM((D, 6 * D), BF16),
            pltpu.VMEM((3 * C, C), BF16),
            pltpu.VMEM((NC, M, D), BF16),
            pltpu.VMEM((LT, 32 + S + 2 * M, 128), F32),
            pltpu.VMEM((NB + 1, LT, 16, 24, 128), F32),
            pltpu.VMEM((NB, LT, 16, 24, 128), F32),
            pltpu.VMEM((NC + 1, LT, 8, 32, 128), F32),
            pltpu.VMEM((3, LT, M, 128), F32),
            pltpu.VMEM((NC + 2, M, D), F32),
            pltpu.VMEM(((NC + 2) * 64, 16 * 128), U32),
            pltpu.VMEM((128 + 128, 96 * 128), U32),
            pltpu.VMEM((384 + 64, 16 * 128), U32),
            pltpu.VMEM((128 + 32, 9 * 640), U32),
            pltpu.VMEM((2 * 64, 9 * 128), U32),
            pltpu.VMEM((2, M, D), F32),
            pltpu.VMEM((8, 8, D), F32),
            pltpu.VMEM((4, 8, D), F32),
            pltpu.VMEM((4, D), BF16), pltpu.VMEM((D,), BF16), pltpu.VMEM((1, D), BF16),
            pltpu.VMEM((14, 1, 128), F32),
            pltpu.SemaphoreType.DMA((13,)),
            pltpu.SemaphoreType.DMA(()),
        ],
        compiler_params=pltpu.CompilerParams(vmem_limit_bytes=120 * 1024 * 1024,
                                             disable_bounds_checks=X_NOCHK, disable_semaphore_checks=X_NOCHK),
        name="fused_h3_glu",
    )(A_q.reshape(NC, M, D), A_k.reshape(NC, M, D), A_v.reshape(NC, M, D), A_shift_k.T, A_ssm_k, A_ssm_D,
      B_w_gate, B_w_up, B_w_down, c, w_mod, cst)
    return out.reshape(1, S, D)
```

```python
import numpy as np
import jax
import jax.numpy as jnp
from jax import lax
import jax.experimental.pallas as pl
import jax.experimental.pallas.tpu as pltpu

S, D, FF = 2048, 640, 1536
C = 128
NB = S // C
M = 256
NC = S // M
LT = D // 128
EPS = 1e-5
F32 = jnp.float32
BF16 = jnp.bfloat16
U32 = jnp.uint32


def _dft_consts():
    r = np.arange(C)
    theta = np.pi * (4 * r + 1) / (2 * C)
    c = np.arange(C)
    ang = theta[:, None] * c[None, :]
    cs = np.stack([np.cos(ang), -np.sin(ang)], axis=0)
    fm = cs.reshape(2, 2, 8, 8, C).transpose(2, 1, 0, 3, 4).reshape(2 * C, C)
    a = np.concatenate([np.arange(0, C, 2), np.arange(1, C, 2)])
    ang2 = a[:, None] * theta[None, :64]
    g = np.zeros((C, 8, 2, 8))
    g[:, :, 0] = np.cos(ang2).reshape(C, 8, 8) / C
    g[:, :, 1] = -np.sin(ang2).reshape(C, 8, 8) / C
    g = g.reshape(C, C)
    return np.concatenate([fm, g], axis=0).astype(np.float32)


C_SLOTS = tuple(range(16, 96, 2))
D_SLOT = 96
AB_SLOT = 2
E_SLOTS = tuple(x for x in (97, 99, 101, 103, 105, 107, 109, 111) for _ in range(4))
WK_SLOTS = (75, 77, 79, 81, 83, 85, 87, 89)
WWK_SLOTS = (99, 100, 101, 102, 103, 104, 105, 106)
X_FAST = False
X_NOCHK = True
X_WKS = 4
WC_SLOTS = tuple(sorted(2 * list(range(60, 80))))
W_WAITS = {0: ("p0",), 16: ("p1",), 48: ("p3",), 80: ("p5",), 96: ("wd",)}
W_AB = 50
W_CMIN = 1
W_D = 80
W_MOD = 97
W_WIDE = False
WE_SLOTS = tuple(x for x in (87, 93, 99, 101, 104, 106, 109, 111) for _ in range(4))


def _mo(x, m):
    return x if isinstance(x, int) else pl.multiple_of(x, m)


def _ls(t):
    return slice(t * 128, (t + 1) * 128)


def _pack(x):
    return pltpu.bitcast(x.astype(BF16), U32)


def _asums(a11, a12, a21, a22):
    return [a11 + a22, a21 + a22, a11, a22, a11 + a12, a21 - a11, a12 - a22]


def _ln(x, fast=False):
    m = jnp.sum(x, axis=-1, keepdims=True) * (1.0 / D)
    if fast:
        ms = jnp.sum(x * x, axis=-1, keepdims=True) * (1.0 / D)
        return (x - m) * lax.rsqrt(jnp.maximum(ms - m * m, 0.0) + EPS)
    xc = x - m
    var = jnp.sum(xc * xc, axis=-1, keepdims=True) * (1.0 / D)
    return xc * lax.rsqrt(var + EPS)


def _kernel(q_h, k_h, v_h, sh_h, sk_h, sd_h, wg_h, wu_h, wd_h, c_h, wm_h, cst_h,
            o_h,
            q_v, k_v, v_v, sk_v, wg_v, wu_v, wd_v, wm_v, cst_v,
            o_v, kbuf, xf, kf, qbuf, ybuf, x1buf, lhsb, wgu, wdn, dlb, dl5, wbuf, modv, shb,
            sh_v, sd_v, c_v, pad_v,
            sem_in, sem_out):
    def k_in(c0, c1):
        return [(k_h.at[c0:c1], k_v.at[c0:c1])]

    def conv_in(c0, c1, with_k=True):
        cols = pl.ds(c0 * M, (c1 - c0) * M)
        return ([(sk_h.at[:, cols], sk_v.at[:, cols])] + (k_in(c0, c1) if with_k else [])
                + [(v_h.at[c0:c1], v_v.at[c0:c1])])

    def q_in(c0, c1):
        return [(q_h.at[c0:c1], q_v.at[c0:c1])]

    def gu_in(p0, p1):
        cols = pl.ds(p0 * 256, (p1 - p0) * 256)
        return [(wg_h.at[:, cols], wg_v.at[:, cols]), (wu_h.at[:, cols], wu_v.at[:, cols])]

    def wm_in(n0, n1):
        cols = pl.ds(n0 * D, (n1 - n0) * D)
        return [(wm_h.at[:, cols], wm_v.at[:, cols])]

    dma = dict(
        small=[(cst_h, cst_v), (sh_h, sh_v), (sd_h, sd_v), (c_h, c_v)],
        c0=conv_in(0, 1),
        c1=conv_in(1, 2),
        c2=conv_in(2, 3),
        wm1=q_in(0, 2) + wm_in(0, 3),
        wm2=wm_in(3, 5),
        p0=gu_in(0, 1),
        p1=gu_in(1, 3),
        p3=conv_in(3, 4) + gu_in(3, 5),
        p5=gu_in(5, 6) + q_in(2, 4) + k_in(4, 6) + wm_in(5, 6),
        wd=[(wd_h, wd_v)],
        r1=conv_in(4, 6, False) + k_in(6, 8),
        r2=q_in(4, 8) + conv_in(6, 8, False),
    )
    dma = {name: [pltpu.make_async_copy(a, b, sem_in.at[n]) for a, b in grp]
           for n, (name, grp) in enumerate(dma.items())}

    def wait(name):
        with jax.named_scope("w_" + name):
            for cp in dma[name]:
                cp.wait()

    def out_copy(i, rows=None, cols=None):
        if rows is None:
            return pltpu.make_async_copy(o_v.at[pl.ds(i, 2)], o_h.at[pl.ds(i, 2)], sem_out)
        return pltpu.make_async_copy(o_v.at[i, rows, cols], o_h.at[i, rows, cols], sem_out)

    last_parts = [(slice(None), _ls(4)), (slice(None), slice(0, 256)), (slice(C, M), _ls(2)),
                  (slice(0, C), _ls(3)), (slice(0, C), _ls(2)), (slice(C, M), _ls(3))]

    for grp in dma.values():
        for cp in grp:
            cp.start()

    for t in range(LT):
        kbuf[t, 24:32, :] = jnp.zeros((8, 128), F32)
    xf[0] = jnp.zeros((LT, 16, 24, 128), F32)
    qbuf[0] = jnp.zeros((LT, 8, 32, 128), F32)
    pad_v[...] = jnp.zeros(pad_v.shape, F32)
    wait("small")
    sh = sh_v[...].astype(F32)
    modv[5] = jnp.broadcast_to(sd_v[...].astype(F32).reshape(1, D), (8, D))
    modv[6] = jnp.zeros((8, D), F32)
    for j in range(4):
        shb[j] = jnp.broadcast_to(sh[j:j + 1, :], (8, D))

    def widen_next_k(s, part, gate):
        kbuf[0, pl.ds(pl.multiple_of(8 * (s % 2048), 8), 8), :] = gate
        r0 = _mo(s * M, M)
        n = 2 * M // (len(WK_SLOTS) * X_WKS)
        ch, r = divmod(part * n, M)
        kk = k_v[jnp.minimum(s + 2 + ch, NC - 1), r:r + n, :].astype(F32)
        for t in range(LT):
            kbuf[t, pl.ds(r0 + 32 + 2 * M + part * n, n), :] = kk[:, _ls(t)]

    def stage_a(c, t, widen=True):
        r0 = _mo(c * M, M)
        ls = _ls(t)
        if widen:
            kk = k_v[c, :, ls].astype(F32)
            kbuf[t, pl.ds(r0 + 32, M), :] = kk
        else:
            kk = kbuf[t, pl.ds(r0 + 32, M), :]
        acc = kk.reshape(32, 8, 128) * shb[0, :, ls][None]
        for j in range(1, 4):
            acc = acc + kbuf[t, pl.ds(r0 + 32 - j, M), :].reshape(32, 8, 128) * shb[j, :, ls][None]
        kv = acc.reshape(M, 128) * v_v[c, :, ls].astype(F32)
        for b in range(2):
            r = jnp.dot(cst_v[0:2 * C, :], kv[b * C:(b + 1) * C].astype(BF16),
                        preferred_element_type=F32).reshape(16, 16, 128)
            xf[2 * c + 1 + b, t, :, 0:16, :] = r
            xf[2 * c + 1 + b, t, :, 16:24, :] = r[:, 0:8, :] + r[:, 8:16, :]

    def stage_b(c, t, maybe_first=False):
        for b in range(2):
            kb = sk_v[_ls(t), pl.ds(_mo(c * M + b * C, C), C)]
            r = lax.dot_general(cst_v[0:2 * C, :], kb, (((1,), (1,)), ((), ())),
                                preferred_element_type=F32).reshape(16, 16, 128)
            cc = r[:, 0:8, :]
            d = r[:, 8:16, :]
            if maybe_first and b == 0:
                cc = cc + modv[5 + jnp.minimum(c, 1), :, _ls(t)][None]
            kf[2 * c + b, t, :, 0:8, :] = d - cc
            kf[2 * c + b, t, :, 8:16, :] = cc + d
            kf[2 * c + b, t, :, 16:24, :] = cc

    def lag_idx(c, cmin, cmax, nout):
        top = 2 * c + nout - 1
        nlag = 2 * cmax + nout
        jok = 2 * cmin + nout - 1
        kidx = [j if j <= jok else jnp.minimum(j, top) for j in range(nlag)]
        xidx = [top + 1 - j if j <= jok + 1 else jnp.maximum(top + 1 - j, 0) for j in range(nlag)]
        return kidx, xidx, nout

    def block_conv(idx, t, us):
        kidx, xidx, nout = idx
        xs = []
        acc = [None] * nout
        for j in reversed(range(len(kidx))):
            k = kf[kidx[j], t, us]
            xs = [xf[xidx[j], t, us]] + xs[:nout - 1]
            for o in reversed(range(len(xs))):
                p = k * xs[o]
                acc[o] = p if acc[o] is None else acc[o] + p
        return [(a[..., 16:24, :] - a[..., 8:16, :], a[..., 16:24, :] + a[..., 0:8, :]) for a in reversed(acc)]

    def cone(c, idx, t, u, pin=None):
        nout = idx[2]
        if nout == 2:
            ri = [((re[0], im[0]), (re[1], im[1])) for re, im in block_conv(idx, t, slice(2 * u, 2 * u + 2))]
        else:
            hs = []
            for h in range(2):
                hs.append(block_conv(idx, t, 2 * u + h))
                tot = [re + im for re, im in hs[h]]
                pin(h, (tot[0] + tot[1]) + (tot[2] + tot[3]))
            ri = list(zip(*hs))
        qs = [(h0[0] + h1[0], h0[1] + h1[1], h0[0] - h1[0], h0[1] - h1[1]) for h0, h1 in ri]
        qv = qbuf.at[pl.ds(c, nout // 2 + 1)]
        qv[nout // 2, t, u] = jnp.concatenate(qs[-1], axis=0)
        prev = qv[0, t, u]
        pv = (prev[0:8], prev[8:16], prev[16:24], prev[24:32])
        res = []
        for cur in qs:
            res.append(jnp.concatenate([cur[0] - pv[1], cur[1] + pv[0]], axis=0))
            res.append(jnp.concatenate([cur[2] - pv[3], cur[3] + pv[2]], axis=0))
            pv = cur
        return res

    def stage_d(yi, t, wfn):
        for b in range(2):
            for par in range(2):
                g = cst_v[2 * C + 64 * par:2 * C + 64 * (par + 1), :]
                y = jnp.dot(g, wfn(2 * b + par), preferred_element_type=F32)
                ybuf[yi, t, pl.ds(b * C + par, 64, stride=2), :] = y

    def ab_all(c):
        for t in range(LT):
            stage_b(c, t, True)
            stage_a(c, t)

    def cd_all(c, cmin, cmax):
        idx = lag_idx(c, cmin, cmax, 2)
        for t in range(LT):
            eo = [cone(c, idx, t, u) for u in range(8)]
            stage_d(c, t, lambda n: jnp.concatenate([e[n] for e in eo], axis=0).astype(BF16))

    def norm2_rows(c, r0, yi, x1dst):
        rows = slice(r0, r0 + 16)
        x = q_v[c, rows, :].astype(F32).reshape(2, 8, D)
        y = jnp.concatenate([ybuf[yi, t, rows, :] for t in range(LT)], axis=1).reshape(2, 8, D)
        x1 = x + (_ln(x, X_FAST) * modv[0][None] + modv[1][None]) * y
        x1dst[rows, :] = x1.reshape(16, D)
        return _ln(x1, X_FAST)

    def mod2(n2):
        return (n2 * modv[2][None] + modv[3][None]).reshape(16, D)

    def store_lhs(dst, r8, top, bot):
        rows = slice(r8, r8 + 8)
        for kt in range(2):
            ss = _asums(top[:, _ls(kt)], top[:, _ls(2 + kt)], bot[:, _ls(kt)], bot[:, _ls(2 + kt)])
            for i in range(7):
                dst[rows, _ls(2 * i + kt)] = _pack(ss[i])
        dst[rows, _ls(14)] = _pack(top[:, _ls(4)])
        dst[rows, _ls(15)] = _pack(bot[:, _ls(4)])
        return ss[0]

    def mod_part(n0, n1):
        cf = c_v[...].astype(F32)
        sc = cf * (1.0 / (1.0 + jnp.exp(-cf)))
        lhs = jnp.broadcast_to(sc, (16, D)).astype(BF16)
        mod = jnp.dot(lhs, wm_v[:, n0 * D:n1 * D], preferred_element_type=F32)[0:8]
        return [mod[:, n * D:(n + 1) * D] for n in range(n1 - n0)]

    bspec = [((0, 0), (1, 1)), ((0, 0), None), ((0, 1), (1, 1)), ((1, 0), (0, 0)),
             ((1, 1), None), ((0, 0), (0, 1)), ((1, 0), (1, 1))]

    def bsum(quad, i):
        qa, qb = bspec[i]
        if qb is None:
            return pltpu.bitcast(quad(*qa), U32)
        return _pack(quad(*qa).astype(F32) - quad(*qb).astype(F32))

    def prep_gu(col):
        p, mat, i = col // 16, (col // 8) % 2, col % 8
        w = (wg_v, wu_v)[mat]
        if i == 7:
            for cc in range(2):
                wgu[64 * cc:64 * cc + 64, _ls(col)] = pltpu.bitcast(w[512:640, _ls(2 * p + cc)], U32)
        else:
            wgu[0:128, _ls(col)] = bsum(lambda r, c: w[256 * r:256 * r + 256, _ls(2 * p + c)], i)

    def prep_dn(col):
        for p in range(6):
            if col >= 14:
                val = pltpu.bitcast(wd_v[_ls(2 * p + col - 14), _ls(4)], U32)
            else:
                val = bsum(lambda r, c: wd_v[_ls(2 * p + r), _ls(2 * (col // 7) + c)], col % 7)
            wdn[64 * p:64 * p + 64, _ls(col)] = val

    def step(s, mode):
        warm, main, last = mode == "warm", mode == "main", mode == "last"
        nch = 1 if last else 2
        R = 64 * nch
        off = 128 * (s % 2)
        lv = lhsb.at[pl.ds(pl.multiple_of((s - 2) * 64, 64), 2 * R)]
        x1v = x1buf.at[pl.ds(s - 2, 2 * nch)]
        dl_w = dlb.at[pl.ds(pl.multiple_of((s % 2) * 32, 32), R)]
        dl_r = dlb.at[pl.ds(pl.multiple_of(((s + 2) % 2) * 32, 32), R)]

        items = [[] for _ in range(112)]
        if warm:
            c0, nout = s + 1, 2
            idx = lag_idx(c0, W_CMIN, 3, nout)
            items[W_D].append(("d", 0))
            for m, names in W_WAITS.items():
                for name in names:
                    items[m].append(("w", name))
            items[W_AB].append(("ab", 0))
            items[W_MOD].append(("mod", 0))
            c_slots, e_slots, yis = WC_SLOTS, WE_SLOTS, (2, 0)
        elif main:
            c0, nout = s, 4
            idx = lag_idx(c0, 4, 6, nout)
            items[AB_SLOT].append(("ab", 0))
            items[D_SLOT].append(("d", 0))
            c_slots, e_slots, yis = C_SLOTS, E_SLOTS, (0, 1)
        if not last:
            for n, m in enumerate(WWK_SLOTS if warm else WK_SLOTS):
                items[m].append(("wk", n))
            for p in range(40):
                items[c_slots[p]].append(("c", p))
            for g in range(32):
                items[e_slots[g]].append(("e", g))
        tops, hist, where = {}, {}, {}
        slot = [0]

        def pin_rows(nrows, n):
            return pl.ds(_mo(nrows + off + 8 * n, 8), 8)

        def hook(ref, nrows, col):
            m = slot[0]
            slot[0] += 1
            npin = 0
            todo = [x for x in items[m] if x[0] not in ("c", "e")]
            if warm:
                todo.append(("prep", col))
            todo += [x for x in items[m] if x[0] in ("c", "e")]
            for kind, p in todo:
                if kind == "w":
                    wait(p)
                elif kind == "prep":
                    (prep_gu if m < 96 else prep_dn)(p)
                elif kind == "mod":
                    modv[4] = mod_part(5, 6)[0]
                elif kind == "ab":
                    if warm and W_WIDE:
                        rw = pl.multiple_of(8 * ((s + (32 + 3 * M) // 8 - 2) % 2048), 8)
                        kk = k_v[c0].astype(F32)
                        for t in range(LT):
                            kbuf[t, pl.ds(rw, M), :] = kk[:, _ls(t)]
                    for ch in range(nout // 2):
                        for t in range(LT):
                            stage_b(c0 + ch, t)
                            stage_a(c0 + ch, t, warm and not W_WIDE)
                elif kind == "wk":
                    for r in range(X_WKS):
                        r0 = 8 * (32 * r // X_WKS)
                        widen_next_k(s, X_WKS * p + r, hist[m - 1][r0:r0 + 8])
                elif kind == "d":
                    for ch in range(nout // 2):
                        for t in range(LT):
                            def wfn(n):
                                parts = []
                                for u in range(8):
                                    rf, nr, cl = where[8 * t + u]
                                    parts.append(rf[pin_rows(nr, 8 * ch + n), _ls(cl)])
                                return pltpu.bitcast(jnp.concatenate(parts, axis=0), BF16)
                            stage_d(ch, t, wfn)
                    if main:
                        out_copy(s - 4).wait()

                        @pl.when(s == 4)
                        def _():
                            wait("r2")
                elif kind == "c":
                    def pin(h, val):
                        ref[pin_rows(nrows, 15 - 3 * h), _ls(col)] = pltpu.bitcast(val, U32)
                    res = cone(c0, idx, p // 8, p % 8, pin)
                    n0 = (4 - npin) if warm else 0
                    for n in range(2 * nout):
                        ref[pin_rows(nrows, n0 + n % 4 + 8 * (n // 4)), _ls(col)] = _pack(res[n])
                    where[p] = (ref, nrows + 8 * n0, col)
                    npin += 2 * nout
                else:
                    ch, g, half = p // 16, (p % 16) // 2, p % 2
                    h2 = mod2(norm2_rows(s + ch, 16 * g + C * half, yis[ch], x1v.at[2 + ch]))
                    if half == 0:
                        tops[g] = h2
                        val = h2[:, _ls(4)]
                    else:
                        val = store_lhs(lv, R + 64 * ch + 8 * g, tops[g], h2)
                    ref[pin_rows(nrows, npin), _ls(col)] = _pack(val)
                    npin += 1
                assert npin <= 8

        def dot(a, w):
            r = jnp.dot(pltpu.bitcast(a, BF16), pltpu.bitcast(w, BF16), preferred_element_type=F32)
            hist.setdefault(slot[0] - 1, r)
            return r

        def strassen(lhs, ref, nrows, base, left):
            def m(i):
                hook(ref, nrows, base + i - 1)
                return dot(lhs(i - 1), ref[0:nrows, _ls(base + i - 1)])
            m2 = m(2)
            m4 = m(4)
            c21 = m2 + m4
            m3 = m(3)
            m5 = m(5)
            c12 = m3 + m5
            c11 = m4 + m5
            c22 = m3 + m2
            m1 = m(1)
            m7 = m(7)
            c11 = c11 + m1 + m7
            c22 = c22 - m1
            c22 = c22 - m(6)
            if left is not None:
                hook(ref, nrows, base + 7)
                c22 = c22 + left(1, 1)
                c11 = c11 + left(0, 0)
                c12 = c12 + left(0, 1)
                c21 = c21 + left(1, 0)
            return c11, c12, c21, c22

        for p in range(6):
            res = []
            for mat in range(2):
                base = (2 * p + mat) * 8
                res.append(strassen(
                    lambda i: lv[0:R, 256 * i:256 * i + 256], wgu, 128, base,
                    lambda r, c: dot(lv[0:R, _ls(14 + r)], wgu[64 * c:64 * c + 64, _ls(base + 7)])))
            hq = [res[0][i] * res[1][i] for i in range(4)]
            for i, x in enumerate(_asums(*hq) + [hq[1], hq[2]]):
                if p < 5:
                    dl_w[:, _ls(5 * i + p)] = _pack(x)
                else:
                    dl5[0:R, _ls(i)] = _pack(x)

        def dla(i):
            return dl_r[:, 640 * i:640 * i + 640]

        def dlz(i):
            return dl5[0:R, _ls(i)]

        def dl(i):
            return jnp.concatenate([dla(i), dlz(i)], axis=1)

        def emit(r, n, o):
            rows = slice(r * C, (r + 1) * C)
            for ch in range(nch):
                res = (x1v[ch, rows, _ls(n)].reshape(16, 8, 128)
                       + o[ch * C:(ch + 1) * C].reshape(16, 8, 128) * modv[4, :, _ls(n)][None])
                o_v[s - 2 + ch, rows, _ls(n)] = res.reshape(C, 128).astype(BF16)

        hook(wdn, 384, 14)
        ta = dot(dla(2), wdn[0:320, _ls(14)])
        tb = dot(dla(8), wdn[0:320, _ls(14)])
        ta = ta + dot(dlz(2), wdn[320:384, _ls(14)])
        tb = tb + dot(dlz(8), wdn[320:384, _ls(14)])
        hook(wdn, 384, 15)
        emit(0, 4, ta + dot(dl(7), wdn[0:384, _ls(15)]))
        emit(1, 4, tb + dot(dl(3), wdn[0:384, _ls(15)]))
        if last:
            out_copy(s - 2, *last_parts[0]).start()
        for pp in range(2):
            cs = strassen(dl, wdn, 384, 7 * pp, None)
            for n, i in enumerate((2, 1, 0, 3)):
                emit(i // 2, 2 * pp + i % 2, cs[i])
                if last and pp == 1:
                    out_copy(s - 2, *last_parts[2 + n]).start()
            if last and pp == 0:
                out_copy(s - 2, *last_parts[1]).start()
        if not last:
            out_copy(s - 2).start()

    def conv012(c, carry):
        for n in range(3):
            @pl.when(c == n)
            def _():
                wait("c%d" % n)
        with jax.named_scope("ab"):
            ab_all(c)

        @pl.when(c == 0)
        def _():
            with jax.named_scope("cd0"):
                cd_all(c, 0, 0)

        @pl.when(c > 0)
        def _():
            with jax.named_scope("cd12"):
                cd_all(c, 1, 2)
        return carry
    lax.fori_loop(0, 3, conv012, 0)
    wait("wm1")
    with jax.named_scope("mod1"):
        sa, ca, ga = mod_part(0, 3)
        modv[0] = ga * (1.0 + ca)
        modv[1] = ga * sa

        def norm01(c, carry):
            for g in range(16):
                wbuf[c, 16 * g:16 * g + 16, :] = norm2_rows(c, 16 * g, c, x1buf.at[c]).reshape(16, D)
            return carry
        lax.fori_loop(0, 2, norm01, 0)
    wait("wm2")
    with jax.named_scope("mod2"):
        sb, cb = mod_part(3, 5)
        modv[2] = 1.0 + cb
        modv[3] = sb
        for c in range(2):
            for g in range(8):
                top, bot = [mod2(wbuf[c, r:r + 16, :].reshape(2, 8, D)) for r in (16 * g, C + 16 * g)]
                store_lhs(lhsb, 64 * c + 8 * g, top, bot)
    def passes(i, s):
        @pl.when(i == 0)
        def _():
            with jax.named_scope("warm"):
                step(s, "warm")
            wait("r1")

        @pl.when(jnp.logical_and(i > 0, i < 3))
        def _():
            with jax.named_scope("main"):
                step(s, "main")

        @pl.when(i >= 3)
        def _():
            with jax.named_scope("tail"):
                step(s, "last")
        return s + jnp.where(i < 3, 2, 1)
    lax.fori_loop(0, 5, passes, 2)

    with jax.named_scope("wait_out"):
        out_copy(4).wait()
        for c in (6, 7):
            for part in last_parts:
                out_copy(c, *part).wait()


@jax.jit
def pallas_adaLN_cond__ssm_conv_h3__glu_gated_bilinear__prompt_kernel(A_q, A_k, A_v, A_shift_k, A_ssm_k, A_ssm_D, B_x, B_w_gate, B_w_up, B_w_down, c, w_mod):
    cst = jnp.asarray(_dft_consts(), dtype=BF16)
    any_spec = pl.BlockSpec(memory_space=pl.ANY)
    out = pl.pallas_call(
        _kernel,
        grid=(1,),
        in_specs=[any_spec] * 12,
        out_specs=any_spec,
        out_shape=jax.ShapeDtypeStruct((NC, M, D), BF16),
        scratch_shapes=[
            pltpu.VMEM((NC, M, D), BF16), pltpu.VMEM((NC, M, D), BF16), pltpu.VMEM((NC, M, D), BF16),
            pltpu.VMEM((D, S), BF16),
            pltpu.VMEM((D, FF), BF16), pltpu.VMEM((D, FF), BF16), pltpu.VMEM((FF, D), BF16),
            pltpu.VMEM((D, 6 * D), BF16),
            pltpu.VMEM((3 * C, C), BF16),
            pltpu.VMEM((NC, M, D), BF16),
            pltpu.VMEM((LT, 32 + S + 2 * M, 128), F32),
            pltpu.VMEM((NB + 1, LT, 16, 24, 128), F32),
            pltpu.VMEM((NB, LT, 16, 24, 128), F32),
            pltpu.VMEM((NC + 1, LT, 8, 32, 128), F32),
            pltpu.VMEM((3, LT, M, 128), F32),
            pltpu.VMEM((NC + 2, M, D), F32),
            pltpu.VMEM(((NC + 2) * 64, 16 * 128), U32),
            pltpu.VMEM((128 + 128, 96 * 128), U32),
            pltpu.VMEM((384 + 64, 16 * 128), U32),
            pltpu.VMEM((128 + 32, 9 * 640), U32),
            pltpu.VMEM((2 * 64, 9 * 128), U32),
            pltpu.VMEM((2, M, D), F32),
            pltpu.VMEM((8, 8, D), F32),
            pltpu.VMEM((4, 8, D), F32),
            pltpu.VMEM((4, D), BF16), pltpu.VMEM((D,), BF16), pltpu.VMEM((1, D), BF16),
            pltpu.VMEM((14, 1, 128), F32),
            pltpu.SemaphoreType.DMA((13,)),
            pltpu.SemaphoreType.DMA(()),
        ],
        compiler_params=pltpu.CompilerParams(vmem_limit_bytes=120 * 1024 * 1024,
                                             disable_bounds_checks=X_NOCHK, disable_semaphore_checks=X_NOCHK),
        name="fused_h3_glu",
    )(A_q.reshape(NC, M, D), A_k.reshape(NC, M, D), A_v.reshape(NC, M, D), A_shift_k.T, A_ssm_k, A_ssm_D,
      B_w_gate, B_w_up, B_w_down, c, w_mod, cst)
    return out.reshape(1, S, D)
```

```python
import numpy as np
import jax
import jax.numpy as jnp
from jax import lax
import jax.experimental.pallas as pl
import jax.experimental.pallas.tpu as pltpu

S, D, FF = 2048, 640, 1536
C = 128
NB = S // C
M = 256
NC = S // M
LT = D // 128
EPS = 1e-5
F32 = jnp.float32
BF16 = jnp.bfloat16
U32 = jnp.uint32


def _dft_consts():
    r = np.arange(C)
    theta = np.pi * (4 * r + 1) / (2 * C)
    c = np.arange(C)
    ang = theta[:, None] * c[None, :]
    cs = np.stack([np.cos(ang), -np.sin(ang)], axis=0)
    fm = cs.reshape(2, 2, 8, 8, C).transpose(2, 1, 0, 3, 4).reshape(2 * C, C)
    a = np.concatenate([np.arange(0, C, 2), np.arange(1, C, 2)])
    ang2 = a[:, None] * theta[None, :64]
    g = np.zeros((C, 8, 2, 8))
    g[:, :, 0] = np.cos(ang2).reshape(C, 8, 8) / C
    g[:, :, 1] = -np.sin(ang2).reshape(C, 8, 8) / C
    g = g.reshape(C, C)
    return np.concatenate([fm, g], axis=0).astype(np.float32)


C_SLOTS = tuple(range(56, 96))
D_SLOT = 96
AB_SLOT = 2
E_SLOTS = tuple(x for x in (97, 99, 101, 103, 105, 107, 109, 111) for _ in range(4))
WK_SLOTS = (75, 77, 79, 81, 83, 85, 87, 89)
WWK_SLOTS = (99, 100, 101, 102, 103, 104, 105, 106)
X_FAST = False
X_NOCHK = True
X_WKS = 4
WC_SLOTS = tuple(sorted(2 * list(range(60, 80))))
W_WAITS = {0: ("p0",), 16: ("p1",), 48: ("p3",), 80: ("p5",), 96: ("wd",)}
W_AB = 52
W_CMIN = 1
W_D = 80
W_MOD = 97
W_WIDE = True
WE_SLOTS = tuple(x for x in (90, 97, 99, 102, 104, 107, 109, 111) for _ in range(4))


def _mo(x, m):
    return x if isinstance(x, int) else pl.multiple_of(x, m)


def _ls(t):
    return slice(t * 128, (t + 1) * 128)


def _pack(x):
    return pltpu.bitcast(x.astype(BF16), U32)


def _asums(a11, a12, a21, a22):
    return [a11 + a22, a21 + a22, a11, a22, a11 + a12, a21 - a11, a12 - a22]


def _ln(x, fast=False):
    m = jnp.sum(x, axis=-1, keepdims=True) * (1.0 / D)
    if fast:
        ms = jnp.sum(x * x, axis=-1, keepdims=True) * (1.0 / D)
        return (x - m) * lax.rsqrt(jnp.maximum(ms - m * m, 0.0) + EPS)
    xc = x - m
    var = jnp.sum(xc * xc, axis=-1, keepdims=True) * (1.0 / D)
    return xc * lax.rsqrt(var + EPS)


def _kernel(q_h, k_h, v_h, sh_h, sk_h, sd_h, wg_h, wu_h, wd_h, c_h, wm_h, cst_h,
            o_h,
            q_v, k_v, v_v, sk_v, wg_v, wu_v, wd_v, wm_v, cst_v,
            o_v, kbuf, xf, kf, qbuf, ybuf, x1buf, lhsb, wgu, wdn, dlb, dl5, wbuf, modv, shb,
            sh_v, sd_v, c_v, pad_v,
            sem_in, sem_out):
    def k_in(c0, c1):
        return [(k_h.at[c0:c1], k_v.at[c0:c1])]

    def conv_in(c0, c1, with_k=True):
        cols = pl.ds(c0 * M, (c1 - c0) * M)
        return ([(sk_h.at[:, cols], sk_v.at[:, cols])] + (k_in(c0, c1) if with_k else [])
                + [(v_h.at[c0:c1], v_v.at[c0:c1])])

    def q_in(c0, c1):
        return [(q_h.at[c0:c1], q_v.at[c0:c1])]

    def gu_in(p0, p1):
        cols = pl.ds(p0 * 256, (p1 - p0) * 256)
        return [(wg_h.at[:, cols], wg_v.at[:, cols]), (wu_h.at[:, cols], wu_v.at[:, cols])]

    def wm_in(n0, n1):
        cols = pl.ds(n0 * D, (n1 - n0) * D)
        return [(wm_h.at[:, cols], wm_v.at[:, cols])]

    dma = dict(
        small=[(cst_h, cst_v), (sh_h, sh_v), (sd_h, sd_v), (c_h, c_v)],
        c0=conv_in(0, 1),
        c1=conv_in(1, 2),
        c2=conv_in(2, 3),
        wm1=q_in(0, 2) + wm_in(0, 3),
        wm2=wm_in(3, 5),
        p0=gu_in(0, 1),
        p1=gu_in(1, 3),
        p3=conv_in(3, 4) + gu_in(3, 5),
        p5=gu_in(5, 6) + q_in(2, 4) + k_in(4, 6) + wm_in(5, 6),
        wd=[(wd_h, wd_v)],
        r1=conv_in(4, 6, False) + k_in(6, 8),
        r2=q_in(4, 8) + conv_in(6, 8, False),
    )
    dma = {name: [pltpu.make_async_copy(a, b, sem_in.at[n]) for a, b in grp]
           for n, (name, grp) in enumerate(dma.items())}

    def wait(name):
        with jax.named_scope("w_" + name):
            for cp in dma[name]:
                cp.wait()

    def out_copy(i, rows=None, cols=None):
        if rows is None:
            return pltpu.make_async_copy(o_v.at[pl.ds(i, 2)], o_h.at[pl.ds(i, 2)], sem_out)
        return pltpu.make_async_copy(o_v.at[i, rows, cols], o_h.at[i, rows, cols], sem_out)

    last_parts = [(slice(None), _ls(4)), (slice(None), slice(0, 256)), (slice(C, M), _ls(2)),
                  (slice(0, C), _ls(3)), (slice(0, C), _ls(2)), (slice(C, M), _ls(3))]

    for grp in dma.values():
        for cp in grp:
            cp.start()

    for t in range(LT):
        kbuf[t, 24:32, :] = jnp.zeros((8, 128), F32)
    xf[0] = jnp.zeros((LT, 16, 24, 128), F32)
    qbuf[0] = jnp.zeros((LT, 8, 32, 128), F32)
    pad_v[...] = jnp.zeros(pad_v.shape, F32)
    wait("small")
    sh = sh_v[...].astype(F32)
    modv[5] = jnp.broadcast_to(sd_v[...].astype(F32).reshape(1, D), (8, D))
    modv[6] = jnp.zeros((8, D), F32)
    for j in range(4):
        shb[j] = jnp.broadcast_to(sh[j:j + 1, :], (8, D))

    def widen_next_k(s, part, gate):
        kbuf[0, pl.ds(pl.multiple_of(8 * (s % 2048), 8), 8), :] = gate
        r0 = _mo(s * M, M)
        n = 2 * M // (len(WK_SLOTS) * X_WKS)
        ch, r = divmod(part * n, M)
        kk = k_v[jnp.minimum(s + 2 + ch, NC - 1), r:r + n, :].astype(F32)
        for t in range(LT):
            kbuf[t, pl.ds(r0 + 32 + 2 * M + part * n, n), :] = kk[:, _ls(t)]

    def stage_a(c, t, widen=True):
        r0 = _mo(c * M, M)
        ls = _ls(t)
        if widen:
            kk = k_v[c, :, ls].astype(F32)
            kbuf[t, pl.ds(r0 + 32, M), :] = kk
        else:
            kk = kbuf[t, pl.ds(r0 + 32, M), :]
        acc = kk.reshape(32, 8, 128) * shb[0, :, ls][None]
        for j in range(1, 4):
            acc = acc + kbuf[t, pl.ds(r0 + 32 - j, M), :].reshape(32, 8, 128) * shb[j, :, ls][None]
        kv = acc.reshape(M, 128) * v_v[c, :, ls].astype(F32)
        for b in range(2):
            r = jnp.dot(cst_v[0:2 * C, :], kv[b * C:(b + 1) * C].astype(BF16),
                        preferred_element_type=F32).reshape(16, 16, 128)
            xf[2 * c + 1 + b, t, :, 0:16, :] = r
            xf[2 * c + 1 + b, t, :, 16:24, :] = r[:, 0:8, :] + r[:, 8:16, :]

    def stage_b(c, t, maybe_first=False):
        for b in range(2):
            kb = sk_v[_ls(t), pl.ds(_mo(c * M + b * C, C), C)]
            r = lax.dot_general(cst_v[0:2 * C, :], kb, (((1,), (1,)), ((), ())),
                                preferred_element_type=F32).reshape(16, 16, 128)
            cc = r[:, 0:8, :]
            d = r[:, 8:16, :]
            if maybe_first and b == 0:
                cc = cc + modv[5 + jnp.minimum(c, 1), :, _ls(t)][None]
            kf[2 * c + b, t, :, 0:8, :] = d - cc
            kf[2 * c + b, t, :, 8:16, :] = cc + d
            kf[2 * c + b, t, :, 16:24, :] = cc

    def lag_idx(c, cmin, cmax, nout):
        top = 2 * c + nout - 1
        nlag = 2 * cmax + nout
        jok = 2 * cmin + nout - 1
        kidx = [j if j <= jok else jnp.minimum(j, top) for j in range(nlag)]
        xidx = [top + 1 - j if j <= jok + 1 else jnp.maximum(top + 1 - j, 0) for j in range(nlag)]
        return kidx, xidx, nout

    def block_conv(idx, t, us):
        kidx, xidx, nout = idx
        xs = []
        acc = [None] * nout
        for j in reversed(range(len(kidx))):
            k = kf[kidx[j], t, us]
            xs = [xf[xidx[j], t, us]] + xs[:nout - 1]
            for o in reversed(range(len(xs))):
                p = k * xs[o]
                acc[o] = p if acc[o] is None else acc[o] + p
        return [(a[..., 16:24, :] - a[..., 8:16, :], a[..., 16:24, :] + a[..., 0:8, :]) for a in reversed(acc)]

    def cone(c, idx, t, u, pin=None):
        nout = idx[2]
        if nout == 2:
            ri = [((re[0], im[0]), (re[1], im[1])) for re, im in block_conv(idx, t, slice(2 * u, 2 * u + 2))]
        else:
            hs = []
            for h in range(2):
                hs.append(block_conv(idx, t, 2 * u + h))
                tot = [re + im for re, im in hs[h]]
                pin(h, (tot[0] + tot[1]) + (tot[2] + tot[3]))
            ri = list(zip(*hs))
        qs = [(h0[0] + h1[0], h0[1] + h1[1], h0[0] - h1[0], h0[1] - h1[1]) for h0, h1 in ri]
        qv = qbuf.at[pl.ds(c, nout // 2 + 1)]
        qv[nout // 2, t, u] = jnp.concatenate(qs[-1], axis=0)
        prev = qv[0, t, u]
        pv = (prev[0:8], prev[8:16], prev[16:24], prev[24:32])
        res = []
        for cur in qs:
            res.append(jnp.concatenate([cur[0] - pv[1], cur[1] + pv[0]], axis=0))
            res.append(jnp.concatenate([cur[2] - pv[3], cur[3] + pv[2]], axis=0))
            pv = cur
        return res

    def stage_d(yi, t, wfn):
        for b in range(2):
            for par in range(2):
                g = cst_v[2 * C + 64 * par:2 * C + 64 * (par + 1), :]
                y = jnp.dot(g, wfn(2 * b + par), preferred_element_type=F32)
                ybuf[yi, t, pl.ds(b * C + par, 64, stride=2), :] = y

    def ab_all(c):
        for t in range(LT):
            stage_b(c, t, True)
            stage_a(c, t)

    def cd_all(c, cmin, cmax):
        idx = lag_idx(c, cmin, cmax, 2)
        for t in range(LT):
            eo = [cone(c, idx, t, u) for u in range(8)]
            stage_d(c, t, lambda n: jnp.concatenate([e[n] for e in eo], axis=0).astype(BF16))

    def norm2_rows(c, r0, yi, x1dst):
        rows = slice(r0, r0 + 16)
        x = q_v[c, rows, :].astype(F32).reshape(2, 8, D)
        y = jnp.concatenate([ybuf[yi, t, rows, :] for t in range(LT)], axis=1).reshape(2, 8, D)
        x1 = x + (_ln(x, X_FAST) * modv[0][None] + modv[1][None]) * y
        x1dst[rows, :] = x1.reshape(16, D)
        return _ln(x1, X_FAST)

    def mod2(n2):
        return (n2 * modv[2][None] + modv[3][None]).reshape(16, D)

    def store_lhs(dst, r8, top, bot):
        rows = slice(r8, r8 + 8)
        for kt in range(2):
            ss = _asums(top[:, _ls(kt)], top[:, _ls(2 + kt)], bot[:, _ls(kt)], bot[:, _ls(2 + kt)])
            for i in range(7):
                dst[rows, _ls(2 * i + kt)] = _pack(ss[i])
        dst[rows, _ls(14)] = _pack(top[:, _ls(4)])
        dst[rows, _ls(15)] = _pack(bot[:, _ls(4)])
        return ss[0]

    def mod_part(n0, n1):
        cf = c_v[...].astype(F32)
        sc = cf * (1.0 / (1.0 + jnp.exp(-cf)))
        lhs = jnp.broadcast_to(sc, (16, D)).astype(BF16)
        mod = jnp.dot(lhs, wm_v[:, n0 * D:n1 * D], preferred_element_type=F32)[0:8]
        return [mod[:, n * D:(n + 1) * D] for n in range(n1 - n0)]

    bspec = [((0, 0), (1, 1)), ((0, 0), None), ((0, 1), (1, 1)), ((1, 0), (0, 0)),
             ((1, 1), None), ((0, 0), (0, 1)), ((1, 0), (1, 1))]

    def bsum(quad, i):
        qa, qb = bspec[i]
        if qb is None:
            return pltpu.bitcast(quad(*qa), U32)
        return _pack(quad(*qa).astype(F32) - quad(*qb).astype(F32))

    def prep_gu(col):
        p, mat, i = col // 16, (col // 8) % 2, col % 8
        w = (wg_v, wu_v)[mat]
        if i == 7:
            for cc in range(2):
                wgu[64 * cc:64 * cc + 64, _ls(col)] = pltpu.bitcast(w[512:640, _ls(2 * p + cc)], U32)
        else:
            wgu[0:128, _ls(col)] = bsum(lambda r, c: w[256 * r:256 * r + 256, _ls(2 * p + c)], i)

    def prep_dn(col):
        for p in range(6):
            if col >= 14:
                val = pltpu.bitcast(wd_v[_ls(2 * p + col - 14), _ls(4)], U32)
            else:
                val = bsum(lambda r, c: wd_v[_ls(2 * p + r), _ls(2 * (col // 7) + c)], col % 7)
            wdn[64 * p:64 * p + 64, _ls(col)] = val

    def step(s, mode):
        warm, main, last = mode == "warm", mode == "main", mode == "last"
        nch = 1 if last else 2
        R = 64 * nch
        off = 128 * (s % 2)
        lv = lhsb.at[pl.ds(pl.multiple_of((s - 2) * 64, 64), 2 * R)]
        x1v = x1buf.at[pl.ds(s - 2, 2 * nch)]
        dl_w = dlb.at[pl.ds(pl.multiple_of((s % 2) * 32, 32), R)]
        dl_r = dlb.at[pl.ds(pl.multiple_of(((s + 2) % 2) * 32, 32), R)]

        items = [[] for _ in range(112)]
        if warm:
            c0, nout = s + 1, 2
            idx = lag_idx(c0, W_CMIN, 3, nout)
            items[W_D].append(("d", 0))
            for m, names in W_WAITS.items():
                for name in names:
                    items[m].append(("w", name))
            items[W_AB].append(("ab", 0))
            items[W_MOD].append(("mod", 0))
            c_slots, e_slots, yis = WC_SLOTS, WE_SLOTS, (2, 0)
        elif main:
            c0, nout = s, 4
            idx = lag_idx(c0, 4, 6, nout)
            items[AB_SLOT].append(("ab", 0))
            items[D_SLOT].append(("d", 0))
            c_slots, e_slots, yis = C_SLOTS, E_SLOTS, (0, 1)
        if not last:
            for n, m in enumerate(WWK_SLOTS if warm else WK_SLOTS):
                items[m].append(("wk", n))
            for p in range(40):
                items[c_slots[p]].append(("c", p))
            for g in range(32):
                items[e_slots[g]].append(("e", g))
        tops, hist, where = {}, {}, {}
        slot = [0]

        def pin_rows(nrows, n):
            return pl.ds(_mo(nrows + off + 8 * n, 8), 8)

        def hook(ref, nrows, col):
            m = slot[0]
            slot[0] += 1
            npin = 0
            todo = [x for x in items[m] if x[0] not in ("c", "e")]
            if warm:
                todo.append(("prep", col))
            todo += [x for x in items[m] if x[0] in ("c", "e")]
            for kind, p in todo:
                if kind == "w":
                    wait(p)
                elif kind == "prep":
                    (prep_gu if m < 96 else prep_dn)(p)
                elif kind == "mod":
                    modv[4] = mod_part(5, 6)[0]
                elif kind == "ab":
                    if warm and W_WIDE:
                        rw = pl.multiple_of(8 * ((s + (32 + 3 * M) // 8 - 2) % 2048), 8)
                        kk = k_v[c0].astype(F32)
                        for t in range(LT):
                            kbuf[t, pl.ds(rw, M), :] = kk[:, _ls(t)]
                    for ch in range(nout // 2):
                        for t in range(LT):
                            stage_b(c0 + ch, t)
                            stage_a(c0 + ch, t, warm and not W_WIDE)
                elif kind == "wk":
                    for r in range(X_WKS):
                        r0 = 8 * (32 * r // X_WKS)
                        widen_next_k(s, X_WKS * p + r, hist[m - 1][r0:r0 + 8])
                elif kind == "d":
                    for ch in range(nout // 2):
                        for t in range(LT):
                            def wfn(n):
                                parts = []
                                for u in range(8):
                                    rf, nr, cl = where[8 * t + u]
                                    parts.append(rf[pin_rows(nr, 8 * ch + n), _ls(cl)])
                                return pltpu.bitcast(jnp.concatenate(parts, axis=0), BF16)
                            stage_d(ch, t, wfn)
                    if main:
                        out_copy(s - 4).wait()

                        @pl.when(s == 4)
                        def _():
                            wait("r2")
                elif kind == "c":
                    def pin(h, val):
                        ref[pin_rows(nrows, 15 - 3 * h), _ls(col)] = pltpu.bitcast(val, U32)
                    res = cone(c0, idx, p // 8, p % 8, pin)
                    n0 = (4 - npin) if warm else 0
                    for n in range(2 * nout):
                        ref[pin_rows(nrows, n0 + n % 4 + 8 * (n // 4)), _ls(col)] = _pack(res[n])
                    where[p] = (ref, nrows + 8 * n0, col)
                    npin += 2 * nout
                else:
                    ch, g, half = p // 16, (p % 16) // 2, p % 2
                    h2 = mod2(norm2_rows(s + ch, 16 * g + C * half, yis[ch], x1v.at[2 + ch]))
                    if half == 0:
                        tops[g] = h2
                        val = h2[:, _ls(4)]
                    else:
                        val = store_lhs(lv, R + 64 * ch + 8 * g, tops[g], h2)
                    ref[pin_rows(nrows, npin), _ls(col)] = _pack(val)
                    npin += 1
                assert npin <= 8

        def dot(a, w):
            r = jnp.dot(pltpu.bitcast(a, BF16), pltpu.bitcast(w, BF16), preferred_element_type=F32)
            hist.setdefault(slot[0] - 1, r)
            return r

        def strassen(lhs, ref, nrows, base, left):
            def m(i):
                hook(ref, nrows, base + i - 1)
                return dot(lhs(i - 1), ref[0:nrows, _ls(base + i - 1)])
            m2 = m(2)
            m4 = m(4)
            c21 = m2 + m4
            m3 = m(3)
            m5 = m(5)
            c12 = m3 + m5
            c11 = m4 + m5
            c22 = m3 + m2
            m1 = m(1)
            m7 = m(7)
            c11 = c11 + m1 + m7
            c22 = c22 - m1
            c22 = c22 - m(6)
            if left is not None:
                hook(ref, nrows, base + 7)
                c22 = c22 + left(1, 1)
                c11 = c11 + left(0, 0)
                c12 = c12 + left(0, 1)
                c21 = c21 + left(1, 0)
            return c11, c12, c21, c22

        for p in range(6):
            res = []
            for mat in range(2):
                base = (2 * p + mat) * 8
                res.append(strassen(
                    lambda i: lv[0:R, 256 * i:256 * i + 256], wgu, 128, base,
                    lambda r, c: dot(lv[0:R, _ls(14 + r)], wgu[64 * c:64 * c + 64, _ls(base + 7)])))
            hq = [res[0][i] * res[1][i] for i in range(4)]
            for i, x in enumerate(_asums(*hq) + [hq[1], hq[2]]):
                if p < 5:
                    dl_w[:, _ls(5 * i + p)] = _pack(x)
                else:
                    dl5[0:R, _ls(i)] = _pack(x)

        def dla(i):
            return dl_r[:, 640 * i:640 * i + 640]

        def dlz(i):
            return dl5[0:R, _ls(i)]

        def dl(i):
            return jnp.concatenate([dla(i), dlz(i)], axis=1)

        def emit(r, n, o):
            rows = slice(r * C, (r + 1) * C)
            for ch in range(nch):
                res = (x1v[ch, rows, _ls(n)].reshape(16, 8, 128)
                       + o[ch * C:(ch + 1) * C].reshape(16, 8, 128) * modv[4, :, _ls(n)][None])
                o_v[s - 2 + ch, rows, _ls(n)] = res.reshape(C, 128).astype(BF16)

        hook(wdn, 384, 14)
        ta = dot(dla(2), wdn[0:320, _ls(14)])
        tb = dot(dla(8), wdn[0:320, _ls(14)])
        ta = ta + dot(dlz(2), wdn[320:384, _ls(14)])
        tb = tb + dot(dlz(8), wdn[320:384, _ls(14)])
        hook(wdn, 384, 15)
        emit(0, 4, ta + dot(dl(7), wdn[0:384, _ls(15)]))
        emit(1, 4, tb + dot(dl(3), wdn[0:384, _ls(15)]))
        if last:
            out_copy(s - 2, *last_parts[0]).start()
        for pp in range(2):
            cs = strassen(dl, wdn, 384, 7 * pp, None)
            for n, i in enumerate((2, 1, 0, 3)):
                emit(i // 2, 2 * pp + i % 2, cs[i])
                if last and pp == 1:
                    out_copy(s - 2, *last_parts[2 + n]).start()
            if last and pp == 0:
                out_copy(s - 2, *last_parts[1]).start()
        if not last:
            out_copy(s - 2).start()

    def conv012(c, carry):
        for n in range(3):
            @pl.when(c == n)
            def _():
                wait("c%d" % n)
        with jax.named_scope("ab"):
            ab_all(c)

        @pl.when(c == 0)
        def _():
            with jax.named_scope("cd0"):
                cd_all(c, 0, 0)

        @pl.when(c > 0)
        def _():
            with jax.named_scope("cd12"):
                cd_all(c, 1, 2)
        return carry
    lax.fori_loop(0, 3, conv012, 0)
    wait("wm1")
    with jax.named_scope("mod1"):
        sa, ca, ga = mod_part(0, 3)
        modv[0] = ga * (1.0 + ca)
        modv[1] = ga * sa

        def norm01(c, carry):
            for g in range(16):
                wbuf[c, 16 * g:16 * g + 16, :] = norm2_rows(c, 16 * g, c, x1buf.at[c]).reshape(16, D)
            return carry
        lax.fori_loop(0, 2, norm01, 0)

    def passes(i, s):
        @pl.when(i == 0)
        def _():
            wait("wm2")
            with jax.named_scope("mod2"):
                sb, cb = mod_part(3, 5)
                modv[2] = 1.0 + cb
                modv[3] = sb
                for c in range(2):
                    for g in range(8):
                        top, bot = [mod2(wbuf[c, r:r + 16, :].reshape(2, 8, D)) for r in (16 * g, C + 16 * g)]
                        store_lhs(lhsb, 64 * c + 8 * g, top, bot)
            with jax.named_scope("warm"):
                step(s, "warm")
            wait("r1")

        @pl.when(jnp.logical_and(i > 0, i < 3))
        def _():
            with jax.named_scope("main"):
                step(s, "main")

        @pl.when(i >= 3)
        def _():
            with jax.named_scope("tail"):
                step(s, "last")
        return s + jnp.where(i < 3, 2, 1)
    lax.fori_loop(0, 5, passes, 2)

    with jax.named_scope("wait_out"):
        out_copy(4).wait()
        for c in (6, 7):
            for part in last_parts:
                out_copy(c, *part).wait()


@jax.jit
def pallas_adaLN_cond__ssm_conv_h3__glu_gated_bilinear__prompt_kernel(A_q, A_k, A_v, A_shift_k, A_ssm_k, A_ssm_D, B_x, B_w_gate, B_w_up, B_w_down, c, w_mod):
    cst = jnp.asarray(_dft_consts(), dtype=BF16)
    any_spec = pl.BlockSpec(memory_space=pl.ANY)
    out = pl.pallas_call(
        _kernel,
        grid=(1,),
        in_specs=[any_spec] * 12,
        out_specs=any_spec,
        out_shape=jax.ShapeDtypeStruct((NC, M, D), BF16),
        scratch_shapes=[
            pltpu.VMEM((NC, M, D), BF16), pltpu.VMEM((NC, M, D), BF16), pltpu.VMEM((NC, M, D), BF16),
            pltpu.VMEM((D, S), BF16),
            pltpu.VMEM((D, FF), BF16), pltpu.VMEM((D, FF), BF16), pltpu.VMEM((FF, D), BF16),
            pltpu.VMEM((D, 6 * D), BF16),
            pltpu.VMEM((3 * C, C), BF16),
            pltpu.VMEM((NC, M, D), BF16),
            pltpu.VMEM((LT, 32 + S + 2 * M, 128), F32),
            pltpu.VMEM((NB + 1, LT, 16, 24, 128), F32),
            pltpu.VMEM((NB, LT, 16, 24, 128), F32),
            pltpu.VMEM((NC + 1, LT, 8, 32, 128), F32),
            pltpu.VMEM((3, LT, M, 128), F32),
            pltpu.VMEM((NC + 2, M, D), F32),
            pltpu.VMEM(((NC + 2) * 64, 16 * 128), U32),
            pltpu.VMEM((128 + 128, 96 * 128), U32),
            pltpu.VMEM((384 + 64, 16 * 128), U32),
            pltpu.VMEM((128 + 32, 9 * 640), U32),
            pltpu.VMEM((2 * 64, 9 * 128), U32),
            pltpu.VMEM((2, M, D), F32),
            pltpu.VMEM((8, 8, D), F32),
            pltpu.VMEM((4, 8, D), F32),
            pltpu.VMEM((4, D), BF16), pltpu.VMEM((D,), BF16), pltpu.VMEM((1, D), BF16),
            pltpu.VMEM((14, 1, 128), F32),
            pltpu.SemaphoreType.DMA((13,)),
            pltpu.SemaphoreType.DMA(()),
        ],
        compiler_params=pltpu.CompilerParams(vmem_limit_bytes=120 * 1024 * 1024,
                                             disable_bounds_checks=X_NOCHK, disable_semaphore_checks=X_NOCHK),
        name="fused_h3_glu",
    )(A_q.reshape(NC, M, D), A_k.reshape(NC, M, D), A_v.reshape(NC, M, D), A_shift_k.T, A_ssm_k, A_ssm_D,
      B_w_gate, B_w_up, B_w_down, c, w_mod, cst)
    return out.reshape(1, S, D)
```

```python
import numpy as np
import jax
import jax.numpy as jnp
from jax import lax
import jax.experimental.pallas as pl
import jax.experimental.pallas.tpu as pltpu

S, D, FF = 2048, 640, 1536
C = 128
NB = S // C
M = 256
NC = S // M
LT = D // 128
EPS = 1e-5
F32 = jnp.float32
BF16 = jnp.bfloat16
U32 = jnp.uint32


def _dft_consts():
    r = np.arange(C)
    theta = np.pi * (4 * r + 1) / (2 * C)
    c = np.arange(C)
    ang = theta[:, None] * c[None, :]
    cs = np.stack([np.cos(ang), -np.sin(ang)], axis=0)
    fm = cs.reshape(2, 2, 8, 8, C).transpose(2, 1, 0, 3, 4).reshape(2 * C, C)
    a = np.concatenate([np.arange(0, C, 2), np.arange(1, C, 2)])
    ang2 = a[:, None] * theta[None, :64]
    g = np.zeros((C, 8, 2, 8))
    g[:, :, 0] = np.cos(ang2).reshape(C, 8, 8) / C
    g[:, :, 1] = -np.sin(ang2).reshape(C, 8, 8) / C
    g = g.reshape(C, C)
    return np.concatenate([fm, g], axis=0).astype(np.float32)


C_SLOTS = tuple(range(56, 96))
D_SLOT = 96
AB_SLOT = 2
E_SLOTS = tuple(x for x in (97, 99, 101, 103, 105, 107, 109, 111) for _ in range(4))
WK_SLOTS = (75, 77, 79, 81, 83, 85, 87, 89)
WWK_SLOTS = (99, 100, 101, 102, 103, 104, 105, 106)
WK_SUB = 4
WC_SLOTS = tuple(sorted(2 * list(range(60, 80))))
W_WAITS = {0: ("p0",), 16: ("p1",), 48: ("p3",), 80: ("p5",), 96: ("wd",)}
W_AB = 52
W_CMIN = 1
W_D = 80
W_MOD = 97
WE_SLOTS = tuple(x for x in (90, 97, 99, 102, 104, 107, 109, 111) for _ in range(4))


def _mo(x, m):
    return x if isinstance(x, int) else pl.multiple_of(x, m)


def _ls(t):
    return slice(t * 128, (t + 1) * 128)


def _pack(x):
    return pltpu.bitcast(x.astype(BF16), U32)


def _asums(a11, a12, a21, a22):
    return [a11 + a22, a21 + a22, a11, a22, a11 + a12, a21 - a11, a12 - a22]


def _ln(x):
    m = jnp.sum(x, axis=-1, keepdims=True) * (1.0 / D)
    xc = x - m
    var = jnp.sum(xc * xc, axis=-1, keepdims=True) * (1.0 / D)
    return xc * lax.rsqrt(var + EPS)


def _kernel(q_h, k_h, v_h, sh_h, sk_h, sd_h, wg_h, wu_h, wd_h, c_h, wm_h, cst_h,
            o_h,
            q_v, k_v, v_v, sk_v, wg_v, wu_v, wd_v, wm_v, cst_v,
            o_v, kbuf, xf, kf, qbuf, ybuf, x1buf, lhsb, wgu, wdn, dlb, dl5, wbuf, modv, shb,
            sh_v, sd_v, c_v, pad_v,
            sem_in, sem_out):
    def k_in(c0, c1):
        return [(k_h.at[c0:c1], k_v.at[c0:c1])]

    def conv_in(c0, c1, with_k=True):
        cols = pl.ds(c0 * M, (c1 - c0) * M)
        return ([(sk_h.at[:, cols], sk_v.at[:, cols])] + (k_in(c0, c1) if with_k else [])
                + [(v_h.at[c0:c1], v_v.at[c0:c1])])

    def q_in(c0, c1):
        return [(q_h.at[c0:c1], q_v.at[c0:c1])]

    def gu_in(p0, p1):
        cols = pl.ds(p0 * 256, (p1 - p0) * 256)
        return [(wg_h.at[:, cols], wg_v.at[:, cols]), (wu_h.at[:, cols], wu_v.at[:, cols])]

    def wm_in(n0, n1):
        cols = pl.ds(n0 * D, (n1 - n0) * D)
        return [(wm_h.at[:, cols], wm_v.at[:, cols])]

    dma = dict(
        small=[(cst_h, cst_v), (sh_h, sh_v), (sd_h, sd_v), (c_h, c_v)],
        c0=conv_in(0, 1),
        c1=conv_in(1, 2),
        c2=conv_in(2, 3),
        wm1=q_in(0, 2) + wm_in(0, 3),
        wm2=wm_in(3, 5),
        p0=gu_in(0, 1),
        p1=gu_in(1, 3),
        p3=conv_in(3, 4) + gu_in(3, 5),
        p5=gu_in(5, 6) + q_in(2, 4) + k_in(4, 6) + wm_in(5, 6),
        wd=[(wd_h, wd_v)],
        r1=conv_in(4, 6, False) + k_in(6, 8),
        r2=q_in(4, 8) + conv_in(6, 8, False),
    )
    dma = {name: [pltpu.make_async_copy(a, b, sem_in.at[n]) for a, b in grp]
           for n, (name, grp) in enumerate(dma.items())}

    def wait(name):
        with jax.named_scope("w_" + name):
            for cp in dma[name]:
                cp.wait()

    def out_copy(i, rows=None, cols=None):
        if rows is None:
            return pltpu.make_async_copy(o_v.at[pl.ds(i, 2)], o_h.at[pl.ds(i, 2)], sem_out)
        return pltpu.make_async_copy(o_v.at[i, rows, cols], o_h.at[i, rows, cols], sem_out)

    last_parts = [(slice(None), _ls(4)), (slice(None), slice(0, 256)), (slice(C, M), _ls(2)),
                  (slice(0, C), _ls(3)), (slice(0, C), _ls(2)), (slice(C, M), _ls(3))]

    for grp in dma.values():
        for cp in grp:
            cp.start()

    for t in range(LT):
        kbuf[t, 24:32, :] = jnp.zeros((8, 128), F32)
    xf[0] = jnp.zeros((LT, 16, 24, 128), F32)
    qbuf[0] = jnp.zeros((LT, 8, 32, 128), F32)
    pad_v[...] = jnp.zeros(pad_v.shape, F32)
    wait("small")
    sh = sh_v[...].astype(F32)
    modv[5] = jnp.broadcast_to(sd_v[...].astype(F32).reshape(1, D), (8, D))
    modv[6] = jnp.zeros((8, D), F32)
    for j in range(4):
        shb[j] = jnp.broadcast_to(sh[j:j + 1, :], (8, D))

    def widen_next_k(s, part, gate):
        kbuf[0, pl.ds(pl.multiple_of(8 * (s % 2048), 8), 8), :] = gate
        r0 = _mo(s * M, M)
        n = 2 * M // (len(WK_SLOTS) * WK_SUB)
        ch, r = divmod(part * n, M)
        kk = k_v[jnp.minimum(s + 2 + ch, NC - 1), r:r + n, :].astype(F32)
        for t in range(LT):
            kbuf[t, pl.ds(r0 + 32 + 2 * M + part * n, n), :] = kk[:, _ls(t)]

    def stage_a(c, t, widen=True):
        r0 = _mo(c * M, M)
        ls = _ls(t)
        if widen:
            kk = k_v[c, :, ls].astype(F32)
            kbuf[t, pl.ds(r0 + 32, M), :] = kk
        else:
            kk = kbuf[t, pl.ds(r0 + 32, M), :]
        acc = kk.reshape(32, 8, 128) * shb[0, :, ls][None]
        for j in range(1, 4):
            acc = acc + kbuf[t, pl.ds(r0 + 32 - j, M), :].reshape(32, 8, 128) * shb[j, :, ls][None]
        kv = acc.reshape(M, 128) * v_v[c, :, ls].astype(F32)
        for b in range(2):
            r = jnp.dot(cst_v[0:2 * C, :], kv[b * C:(b + 1) * C].astype(BF16),
                        preferred_element_type=F32).reshape(16, 16, 128)
            xf[2 * c + 1 + b, t, :, 0:16, :] = r
            xf[2 * c + 1 + b, t, :, 16:24, :] = r[:, 0:8, :] + r[:, 8:16, :]

    def stage_b(c, t, maybe_first=False):
        for b in range(2):
            kb = sk_v[_ls(t), pl.ds(_mo(c * M + b * C, C), C)]
            r = lax.dot_general(cst_v[0:2 * C, :], kb, (((1,), (1,)), ((), ())),
                                preferred_element_type=F32).reshape(16, 16, 128)
            cc = r[:, 0:8, :]
            d = r[:, 8:16, :]
            if maybe_first and b == 0:
                cc = cc + modv[5 + jnp.minimum(c, 1), :, _ls(t)][None]
            kf[2 * c + b, t, :, 0:8, :] = d - cc
            kf[2 * c + b, t, :, 8:16, :] = cc + d
            kf[2 * c + b, t, :, 16:24, :] = cc

    def lag_idx(c, cmin, cmax, nout):
        top = 2 * c + nout - 1
        nlag = 2 * cmax + nout
        jok = 2 * cmin + nout - 1
        kidx = [j if j <= jok else jnp.minimum(j, top) for j in range(nlag)]
        xidx = [top + 1 - j if j <= jok + 1 else jnp.maximum(top + 1 - j, 0) for j in range(nlag)]
        return kidx, xidx, nout

    def block_conv(idx, t, us):
        kidx, xidx, nout = idx
        xs = []
        acc = [None] * nout
        for j in reversed(range(len(kidx))):
            k = kf[kidx[j], t, us]
            xs = [xf[xidx[j], t, us]] + xs[:nout - 1]
            for o in reversed(range(len(xs))):
                p = k * xs[o]
                acc[o] = p if acc[o] is None else acc[o] + p
        return [(a[..., 16:24, :] - a[..., 8:16, :], a[..., 16:24, :] + a[..., 0:8, :]) for a in reversed(acc)]

    def cone(c, idx, t, u, pin=None):
        nout = idx[2]
        if nout == 2:
            ri = [((re[0], im[0]), (re[1], im[1])) for re, im in block_conv(idx, t, slice(2 * u, 2 * u + 2))]
        else:
            hs = []
            for h in range(2):
                hs.append(block_conv(idx, t, 2 * u + h))
                tot = [re + im for re, im in hs[h]]
                pin(h, (tot[0] + tot[1]) + (tot[2] + tot[3]))
            ri = list(zip(*hs))
        qs = [(h0[0] + h1[0], h0[1] + h1[1], h0[0] - h1[0], h0[1] - h1[1]) for h0, h1 in ri]
        qv = qbuf.at[pl.ds(c, nout // 2 + 1)]
        qv[nout // 2, t, u] = jnp.concatenate(qs[-1], axis=0)
        prev = qv[0, t, u]
        pv = (prev[0:8], prev[8:16], prev[16:24], prev[24:32])
        res = []
        for cur in qs:
            res.append(jnp.concatenate([cur[0] - pv[1], cur[1] + pv[0]], axis=0))
            res.append(jnp.concatenate([cur[2] - pv[3], cur[3] + pv[2]], axis=0))
            pv = cur
        return res

    def stage_d(yi, t, wfn):
        for b in range(2):
            for par in range(2):
                g = cst_v[2 * C + 64 * par:2 * C + 64 * (par + 1), :]
                y = jnp.dot(g, wfn(2 * b + par), preferred_element_type=F32)
                ybuf[yi, t, pl.ds(b * C + par, 64, stride=2), :] = y

    def ab_all(c):
        for t in range(LT):
            stage_b(c, t, True)
            stage_a(c, t)

    def cd_all(c, cmin, cmax):
        idx = lag_idx(c, cmin, cmax, 2)
        for t in range(LT):
            eo = [cone(c, idx, t, u) for u in range(8)]
            stage_d(c, t, lambda n: jnp.concatenate([e[n] for e in eo], axis=0).astype(BF16))

    def norm2_rows(c, r0, yi, x1dst):
        rows = slice(r0, r0 + 16)
        x = q_v[c, rows, :].astype(F32).reshape(2, 8, D)
        y = jnp.concatenate([ybuf[yi, t, rows, :] for t in range(LT)], axis=1).reshape(2, 8, D)
        x1 = x + (_ln(x) * modv[0][None] + modv[1][None]) * y
        x1dst[rows, :] = x1.reshape(16, D)
        return _ln(x1)

    def mod2(n2):
        return (n2 * modv[2][None] + modv[3][None]).reshape(16, D)

    def store_lhs(dst, r8, top, bot):
        rows = slice(r8, r8 + 8)
        for kt in range(2):
            ss = _asums(top[:, _ls(kt)], top[:, _ls(2 + kt)], bot[:, _ls(kt)], bot[:, _ls(2 + kt)])
            for i in range(7):
                dst[rows, _ls(2 * i + kt)] = _pack(ss[i])
        dst[rows, _ls(14)] = _pack(top[:, _ls(4)])
        dst[rows, _ls(15)] = _pack(bot[:, _ls(4)])
        return ss[0]

    def mod_part(n0, n1):
        cf = c_v[...].astype(F32)
        sc = cf * (1.0 / (1.0 + jnp.exp(-cf)))
        lhs = jnp.broadcast_to(sc, (16, D)).astype(BF16)
        mod = jnp.dot(lhs, wm_v[:, n0 * D:n1 * D], preferred_element_type=F32)[0:8]
        return [mod[:, n * D:(n + 1) * D] for n in range(n1 - n0)]

    bspec = [((0, 0), (1, 1)), ((0, 0), None), ((0, 1), (1, 1)), ((1, 0), (0, 0)),
             ((1, 1), None), ((0, 0), (0, 1)), ((1, 0), (1, 1))]

    def bsum(quad, i):
        qa, qb = bspec[i]
        if qb is None:
            return pltpu.bitcast(quad(*qa), U32)
        return _pack(quad(*qa).astype(F32) - quad(*qb).astype(F32))

    def prep_gu(col):
        p, mat, i = col // 16, (col // 8) % 2, col % 8
        w = (wg_v, wu_v)[mat]
        if i == 7:
            for cc in range(2):
                wgu[64 * cc:64 * cc + 64, _ls(col)] = pltpu.bitcast(w[512:640, _ls(2 * p + cc)], U32)
        else:
            wgu[0:128, _ls(col)] = bsum(lambda r, c: w[256 * r:256 * r + 256, _ls(2 * p + c)], i)

    def prep_dn(col):
        for p in range(6):
            if col >= 14:
                val = pltpu.bitcast(wd_v[_ls(2 * p + col - 14), _ls(4)], U32)
            else:
                val = bsum(lambda r, c: wd_v[_ls(2 * p + r), _ls(2 * (col // 7) + c)], col % 7)
            wdn[64 * p:64 * p + 64, _ls(col)] = val

    def step(s, mode):
        warm, main, last = mode == "warm", mode == "main", mode == "last"
        nch = 1 if last else 2
        R = 64 * nch
        off = 128 * (s % 2)
        lv = lhsb.at[pl.ds(pl.multiple_of((s - 2) * 64, 64), 2 * R)]
        x1v = x1buf.at[pl.ds(s - 2, 2 * nch)]
        dl_w = dlb.at[pl.ds(pl.multiple_of((s % 2) * 32, 32), R)]
        dl_r = dlb.at[pl.ds(pl.multiple_of(((s + 2) % 2) * 32, 32), R)]

        items = [[] for _ in range(112)]
        if warm:
            c0, nout = s + 1, 2
            idx = lag_idx(c0, W_CMIN, 3, nout)
            items[W_D].append(("d", 0))
            for m, names in W_WAITS.items():
                for name in names:
                    items[m].append(("w", name))
            items[W_AB].append(("ab", 0))
            items[W_MOD].append(("mod", 0))
            c_slots, e_slots, yis = WC_SLOTS, WE_SLOTS, (2, 0)
        elif main:
            c0, nout = s, 4
            idx = lag_idx(c0, 4, 6, nout)
            items[AB_SLOT].append(("ab", 0))
            items[D_SLOT].append(("d", 0))
            c_slots, e_slots, yis = C_SLOTS, E_SLOTS, (0, 1)
        if not last:
            for n, m in enumerate(WWK_SLOTS if warm else WK_SLOTS):
                items[m].append(("wk", n))
            for p in range(40):
                items[c_slots[p]].append(("c", p))
            for g in range(32):
                items[e_slots[g]].append(("e", g))
        tops, hist, where = {}, {}, {}
        slot = [0]

        def pin_rows(nrows, n):
            return pl.ds(_mo(nrows + off + 8 * n, 8), 8)

        def hook(ref, nrows, col):
            m = slot[0]
            slot[0] += 1
            npin = 0
            todo = [x for x in items[m] if x[0] not in ("c", "e")]
            if warm:
                todo.append(("prep", col))
            todo += [x for x in items[m] if x[0] in ("c", "e")]
            for kind, p in todo:
                if kind == "w":
                    wait(p)
                elif kind == "prep":
                    (prep_gu if m < 96 else prep_dn)(p)
                elif kind == "mod":
                    modv[4] = mod_part(5, 6)[0]
                elif kind == "ab":
                    if warm:
                        rw = pl.multiple_of(8 * ((s + (32 + 3 * M) // 8 - 2) % 2048), 8)
                        kk = k_v[c0].astype(F32)
                        for t in range(LT):
                            kbuf[t, pl.ds(rw, M), :] = kk[:, _ls(t)]
                    for ch in range(nout // 2):
                        for t in range(LT):
                            stage_b(c0 + ch, t)
                            stage_a(c0 + ch, t, False)
                elif kind == "wk":
                    for r in range(WK_SUB):
                        r0 = 8 * (32 * r // WK_SUB)
                        widen_next_k(s, WK_SUB * p + r, hist[m - 1][r0:r0 + 8])
                elif kind == "d":
                    for ch in range(nout // 2):
                        for t in range(LT):
                            def wfn(n):
                                parts = []
                                for u in range(8):
                                    rf, nr, cl = where[8 * t + u]
                                    parts.append(rf[pin_rows(nr, 8 * ch + n), _ls(cl)])
                                return pltpu.bitcast(jnp.concatenate(parts, axis=0), BF16)
                            stage_d(ch, t, wfn)
                    if main:
                        out_copy(s - 4).wait()

                        @pl.when(s == 4)
                        def _():
                            wait("r2")
                elif kind == "c":
                    def pin(h, val):
                        ref[pin_rows(nrows, 15 - 3 * h), _ls(col)] = pltpu.bitcast(val, U32)
                    res = cone(c0, idx, p // 8, p % 8, pin)
                    n0 = (4 - npin) if warm else 0
                    for n in range(2 * nout):
                        ref[pin_rows(nrows, n0 + n % 4 + 8 * (n // 4)), _ls(col)] = _pack(res[n])
                    where[p] = (ref, nrows + 8 * n0, col)
                    npin += 2 * nout
                else:
                    ch, g, half = p // 16, (p % 16) // 2, p % 2
                    h2 = mod2(norm2_rows(s + ch, 16 * g + C * half, yis[ch], x1v.at[2 + ch]))
                    if half == 0:
                        tops[g] = h2
                        val = h2[:, _ls(4)]
                    else:
                        val = store_lhs(lv, R + 64 * ch + 8 * g, tops[g], h2)
                    ref[pin_rows(nrows, npin), _ls(col)] = _pack(val)
                    npin += 1
                assert npin <= 8

        def dot(a, w):
            r = jnp.dot(pltpu.bitcast(a, BF16), pltpu.bitcast(w, BF16), preferred_element_type=F32)
            hist.setdefault(slot[0] - 1, r)
            return r

        def strassen(lhs, ref, nrows, base, left):
            def m(i):
                hook(ref, nrows, base + i - 1)
                return dot(lhs(i - 1), ref[0:nrows, _ls(base + i - 1)])
            m2 = m(2)
            m4 = m(4)
            c21 = m2 + m4
            m3 = m(3)
            m5 = m(5)
            c12 = m3 + m5
            c11 = m4 + m5
            c22 = m3 + m2
            m1 = m(1)
            m7 = m(7)
            c11 = c11 + m1 + m7
            c22 = c22 - m1
            c22 = c22 - m(6)
            if left is not None:
                hook(ref, nrows, base + 7)
                c22 = c22 + left(1, 1)
                c11 = c11 + left(0, 0)
                c12 = c12 + left(0, 1)
                c21 = c21 + left(1, 0)
            return c11, c12, c21, c22

        for p in range(6):
            res = []
            for mat in range(2):
                base = (2 * p + mat) * 8
                res.append(strassen(
                    lambda i: lv[0:R, 256 * i:256 * i + 256], wgu, 128, base,
                    lambda r, c: dot(lv[0:R, _ls(14 + r)], wgu[64 * c:64 * c + 64, _ls(base + 7)])))
            hq = [res[0][i] * res[1][i] for i in range(4)]
            for i, x in enumerate(_asums(*hq) + [hq[1], hq[2]]):
                if p < 5:
                    dl_w[:, _ls(5 * i + p)] = _pack(x)
                else:
                    dl5[0:R, _ls(i)] = _pack(x)

        def dla(i):
            return dl_r[:, 640 * i:640 * i + 640]

        def dlz(i):
            return dl5[0:R, _ls(i)]

        def dl(i):
            return jnp.concatenate([dla(i), dlz(i)], axis=1)

        def emit(r, n, o):
            rows = slice(r * C, (r + 1) * C)
            for ch in range(nch):
                res = (x1v[ch, rows, _ls(n)].reshape(16, 8, 128)
                       + o[ch * C:(ch + 1) * C].reshape(16, 8, 128) * modv[4, :, _ls(n)][None])
                o_v[s - 2 + ch, rows, _ls(n)] = res.reshape(C, 128).astype(BF16)

        hook(wdn, 384, 14)
        ta = dot(dla(2), wdn[0:320, _ls(14)])
        tb = dot(dla(8), wdn[0:320, _ls(14)])
        ta = ta + dot(dlz(2), wdn[320:384, _ls(14)])
        tb = tb + dot(dlz(8), wdn[320:384, _ls(14)])
        hook(wdn, 384, 15)
        emit(0, 4, ta + dot(dl(7), wdn[0:384, _ls(15)]))
        emit(1, 4, tb + dot(dl(3), wdn[0:384, _ls(15)]))
        if last:
            out_copy(s - 2, *last_parts[0]).start()
        for pp in range(2):
            cs = strassen(dl, wdn, 384, 7 * pp, None)
            for n, i in enumerate((2, 1, 0, 3)):
                emit(i // 2, 2 * pp + i % 2, cs[i])
                if last and pp == 1:
                    out_copy(s - 2, *last_parts[2 + n]).start()
            if last and pp == 0:
                out_copy(s - 2, *last_parts[1]).start()
        if not last:
            out_copy(s - 2).start()

    def conv012(c, carry):
        for n in range(3):
            @pl.when(c == n)
            def _():
                wait("c%d" % n)
        with jax.named_scope("ab"):
            ab_all(c)

        @pl.when(c == 0)
        def _():
            with jax.named_scope("cd0"):
                cd_all(c, 0, 0)

        @pl.when(c > 0)
        def _():
            with jax.named_scope("cd12"):
                cd_all(c, 1, 2)
        return carry
    lax.fori_loop(0, 3, conv012, 0)
    wait("wm1")
    with jax.named_scope("mod1"):
        sa, ca, ga = mod_part(0, 3)
        modv[0] = ga * (1.0 + ca)
        modv[1] = ga * sa

        def norm01(c, carry):
            for g in range(16):
                wbuf[c, 16 * g:16 * g + 16, :] = norm2_rows(c, 16 * g, c, x1buf.at[c]).reshape(16, D)
            return carry
        lax.fori_loop(0, 2, norm01, 0)

    def passes(i, s):
        @pl.when(i == 0)
        def _():
            wait("wm2")
            with jax.named_scope("mod2"):
                sb, cb = mod_part(3, 5)
                modv[2] = 1.0 + cb
                modv[3] = sb
                for c in range(2):
                    for g in range(8):
                        top, bot = [mod2(wbuf[c, r:r + 16, :].reshape(2, 8, D)) for r in (16 * g, C + 16 * g)]
                        store_lhs(lhsb, 64 * c + 8 * g, top, bot)
            with jax.named_scope("warm"):
                step(s, "warm")
            wait("r1")

        @pl.when(jnp.logical_and(i > 0, i < 3))
        def _():
            with jax.named_scope("main"):
                step(s, "main")

        @pl.when(i >= 3)
        def _():
            with jax.named_scope("tail"):
                step(s, "last")
        return s + jnp.where(i < 3, 2, 1)
    lax.fori_loop(0, 5, passes, 2)

    with jax.named_scope("wait_out"):
        out_copy(4).wait()
        for c in (6, 7):
            for part in last_parts:
                out_copy(c, *part).wait()


@jax.jit
def pallas_adaLN_cond__ssm_conv_h3__glu_gated_bilinear__prompt_kernel(A_q, A_k, A_v, A_shift_k, A_ssm_k, A_ssm_D, B_x, B_w_gate, B_w_up, B_w_down, c, w_mod):
    cst = jnp.asarray(_dft_consts(), dtype=BF16)
    any_spec = pl.BlockSpec(memory_space=pl.ANY)
    out = pl.pallas_call(
        _kernel,
        grid=(1,),
        in_specs=[any_spec] * 12,
        out_specs=any_spec,
        out_shape=jax.ShapeDtypeStruct((NC, M, D), BF16),
        scratch_shapes=[
            pltpu.VMEM((NC, M, D), BF16), pltpu.VMEM((NC, M, D), BF16), pltpu.VMEM((NC, M, D), BF16),
            pltpu.VMEM((D, S), BF16),
            pltpu.VMEM((D, FF), BF16), pltpu.VMEM((D, FF), BF16), pltpu.VMEM((FF, D), BF16),
            pltpu.VMEM((D, 6 * D), BF16),
            pltpu.VMEM((3 * C, C), BF16),
            pltpu.VMEM((NC, M, D), BF16),
            pltpu.VMEM((LT, 32 + S + 2 * M, 128), F32),
            pltpu.VMEM((NB + 1, LT, 16, 24, 128), F32),
            pltpu.VMEM((NB, LT, 16, 24, 128), F32),
            pltpu.VMEM((NC + 1, LT, 8, 32, 128), F32),
            pltpu.VMEM((3, LT, M, 128), F32),
            pltpu.VMEM((NC + 2, M, D), F32),
            pltpu.VMEM(((NC + 2) * 64, 16 * 128), U32),
            pltpu.VMEM((128 + 128, 96 * 128), U32),
            pltpu.VMEM((384 + 64, 16 * 128), U32),
            pltpu.VMEM((128 + 32, 9 * 640), U32),
            pltpu.VMEM((2 * 64, 9 * 128), U32),
            pltpu.VMEM((2, M, D), F32),
            pltpu.VMEM((8, 8, D), F32),
            pltpu.VMEM((4, 8, D), F32),
            pltpu.VMEM((4, D), BF16), pltpu.VMEM((D,), BF16), pltpu.VMEM((1, D), BF16),
            pltpu.VMEM((14, 1, 128), F32),
            pltpu.SemaphoreType.DMA((13,)),
            pltpu.SemaphoreType.DMA(()),
        ],
        compiler_params=pltpu.CompilerParams(vmem_limit_bytes=120 * 1024 * 1024,
                                             disable_bounds_checks=True, disable_semaphore_checks=True),
        name="fused_h3_glu",
    )(A_q.reshape(NC, M, D), A_k.reshape(NC, M, D), A_v.reshape(NC, M, D), A_shift_k.T, A_ssm_k, A_ssm_D,
      B_w_gate, B_w_up, B_w_down, c, w_mod, cst)
    return out.reshape(1, S, D)
```

```python
import numpy as np
import jax
import jax.numpy as jnp
from jax import lax
import jax.experimental.pallas as pl
import jax.experimental.pallas.tpu as pltpu

S, D, FF = 2048, 640, 1536
C = 128
NB = S // C
M = 256
NC = S // M
LT = D // 128
EPS = 1e-5
F32 = jnp.float32
BF16 = jnp.bfloat16
U32 = jnp.uint32


def _dft_consts():
    r = np.arange(C)
    theta = np.pi * (4 * r + 1) / (2 * C)
    c = np.arange(C)
    ang = theta[:, None] * c[None, :]
    cs = np.stack([np.cos(ang), -np.sin(ang)], axis=0)
    fm = cs.reshape(2, 2, 8, 8, C).transpose(2, 1, 0, 3, 4).reshape(2 * C, C)
    a = np.concatenate([np.arange(0, C, 2), np.arange(1, C, 2)])
    ang2 = a[:, None] * theta[None, :64]
    g = np.zeros((C, 8, 2, 8))
    g[:, :, 0] = np.cos(ang2).reshape(C, 8, 8) / C
    g[:, :, 1] = -np.sin(ang2).reshape(C, 8, 8) / C
    g = g.reshape(C, C)
    return np.concatenate([fm, g], axis=0).astype(np.float32)


C_SLOTS = tuple(range(56, 96))
D_SLOT = 96
AB_SLOT = 2
E_SLOTS = tuple(x for x in (97, 99, 101, 103, 105, 107, 109, 111) for _ in range(4))
WK_SLOTS = (75, 77, 79, 81, 83, 85, 87, 89)
WK_SUB = 4
WC_SLOTS = tuple(sorted(3 * [x for x in range(68, 79) if x % 8 != 7] + [x for x in range(84, 95) if x % 8 != 7]))
W_WAITS = {0: ("p0",), 16: ("p1",), 48: ("p3",), 80: ("p5",), 96: ("wd",)}
W_AB = 50
W_CMIN = 1
W_D = 96
W_MOD = 96
WE_SLOTS = tuple(x for x in (97, 99, 101, 103, 105, 107, 109, 111) for _ in range(4))


def _mo(x, m):
    return x if isinstance(x, int) else pl.multiple_of(x, m)


def _ls(t):
    return slice(t * 128, (t + 1) * 128)


def _pack(x):
    return pltpu.bitcast(x.astype(BF16), U32)


def _asums(a11, a12, a21, a22):
    return [a11 + a22, a21 + a22, a11, a22, a11 + a12, a21 - a11, a12 - a22]


def _ln(x):
    m = jnp.sum(x, axis=-1, keepdims=True) * (1.0 / D)
    xc = x - m
    var = jnp.sum(xc * xc, axis=-1, keepdims=True) * (1.0 / D)
    return xc * lax.rsqrt(var + EPS)


def _kernel(q_h, k_h, v_h, sh_h, sk_h, sd_h, wg_h, wu_h, wd_h, c_h, wm_h, cst_h,
            o_h,
            q_v, k_v, v_v, sk_v, wg_v, wu_v, wd_v, wm_v, cst_v,
            o_v, kbuf, xf, kf, qbuf, ybuf, x1buf, lhsb, wgu, wdn, dlb, dl5, wbuf, accb, modv, shb,
            sh_v, sd_v, c_v, pad_v,
            sem_in, sem_out):
    def k_in(c0, c1):
        return [(k_h.at[c0:c1], k_v.at[c0:c1])]

    def conv_in(c0, c1, with_k=True):
        cols = pl.ds(c0 * M, (c1 - c0) * M)
        return ([(sk_h.at[:, cols], sk_v.at[:, cols])] + (k_in(c0, c1) if with_k else [])
                + [(v_h.at[c0:c1], v_v.at[c0:c1])])

    def q_in(c0, c1):
        return [(q_h.at[c0:c1], q_v.at[c0:c1])]

    def gu_in(p0, p1):
        cols = pl.ds(p0 * 256, (p1 - p0) * 256)
        return [(wg_h.at[0:512, cols], wg_v.at[0:512, cols]), (wu_h.at[0:512, cols], wu_v.at[0:512, cols])]

    def wm_cols(c0, c1):
        return [(wm_h.at[:, c0:c1], wm_v.at[:, c0:c1])]

    def wm_in(n0, n1):
        cols = pl.ds(n0 * D, (n1 - n0) * D)
        return [(wm_h.at[:, cols], wm_v.at[:, cols])]

    dma = dict(
        small=[(cst_h, cst_v), (sh_h, sh_v), (sd_h, sd_v), (c_h, c_v)],
        k0=k_in(0, 1),
        c0=conv_in(0, 1, False),
        k1=k_in(1, 2),
        c1=conv_in(1, 2, False),
        k2=k_in(2, 3),
        c2=conv_in(2, 3, False),
        q01=q_in(0, 2),
        wm1=wm_in(0, 3),
        k4=(wm_cols(4 * D - 128, 4 * D) + wm_cols(5 * D - 128, 5 * D)
            + [(wg_h.at[512:640], wg_v.at[512:640]), (wu_h.at[512:640], wu_v.at[512:640])]),
        wm2=wm_cols(3 * D, 4 * D - 128) + wm_cols(4 * D, 5 * D - 128),
        p0=gu_in(0, 1),
        p1=gu_in(1, 3),
        p3=conv_in(3, 4) + gu_in(3, 5),
        p5=gu_in(5, 6) + q_in(2, 4) + wm_in(5, 6),
        wd=[(wd_h, wd_v)],
        r1=conv_in(4, 6) + k_in(6, 8),
        r2=q_in(4, 8) + conv_in(6, 8, False),
    )
    dma = {name: [pltpu.make_async_copy(a, b, sem_in.at[n]) for a, b in grp]
           for n, (name, grp) in enumerate(dma.items())}

    def wait(name):
        with jax.named_scope("w_" + name):
            for cp in dma[name]:
                cp.wait()

    def out_copy(i, rows=None, cols=None):
        if rows is None:
            return pltpu.make_async_copy(o_v.at[pl.ds(i, 2)], o_h.at[pl.ds(i, 2)], sem_out)
        return pltpu.make_async_copy(o_v.at[i, rows, cols], o_h.at[i, rows, cols], sem_out)

    last_parts = [(slice(None), _ls(4)), (slice(None), slice(0, 256)), (slice(C, M), _ls(2)),
                  (slice(0, C), _ls(3)), (slice(0, C), _ls(2)), (slice(C, M), _ls(3))]

    for grp in dma.values():
        for cp in grp:
            cp.start()

    def zero_init(t, carry):
        kbuf[t, 24:32, :] = jnp.zeros((8, 128), F32)
        xf[0, t] = jnp.zeros((16, 24, 128), F32)
        qbuf[0, t] = jnp.zeros((8, 32, 128), F32)
        return carry
    lax.fori_loop(0, LT, zero_init, 0)
    pad_v[...] = jnp.zeros(pad_v.shape, F32)
    wait("small")
    sh = sh_v[...].astype(F32)
    modv[5] = jnp.broadcast_to(sd_v[...].astype(F32).reshape(1, D), (8, D))
    modv[6] = jnp.zeros((8, D), F32)
    for j in range(4):
        shb[j] = jnp.broadcast_to(sh[j:j + 1, :], (8, D))

    def widen_next_k(s, part, gate):
        kbuf[0, pl.ds(pl.multiple_of(8 * (s % 2048), 8), 8), :] = gate
        r0 = _mo(s * M, M)
        n = 2 * M // (len(WK_SLOTS) * WK_SUB)
        ch, r = divmod(part * n, M)
        kk = k_v[jnp.minimum(s + 2 + ch, NC - 1), r:r + n, :].astype(F32)
        for t in range(LT):
            kbuf[t, pl.ds(r0 + 32 + 2 * M + part * n, n), :] = kk[:, _ls(t)]

    def stage_a(c, t):
        r0 = _mo(c * M, M)
        ls = _ls(t)
        kk = kbuf[t, pl.ds(r0 + 32, M), :]
        acc = kk.reshape(32, 8, 128) * shb[0, :, ls][None]
        for j in range(1, 4):
            acc = acc + kbuf[t, pl.ds(r0 + 32 - j, M), :].reshape(32, 8, 128) * shb[j, :, ls][None]
        kv = acc.reshape(M, 128) * v_v[c, :, ls].astype(F32)
        for b in range(2):
            r = jnp.dot(cst_v[0:2 * C, :], kv[b * C:(b + 1) * C].astype(BF16),
                        preferred_element_type=F32).reshape(16, 16, 128)
            xf[2 * c + 1 + b, t, :, 0:16, :] = r
            xf[2 * c + 1 + b, t, :, 16:24, :] = r[:, 0:8, :] + r[:, 8:16, :]

    def stage_b(c, t, maybe_first=False):
        for b in range(2):
            kb = sk_v[_ls(t), pl.ds(_mo(c * M + b * C, C), C)]
            r = lax.dot_general(cst_v[0:2 * C, :], kb, (((1,), (1,)), ((), ())),
                                preferred_element_type=F32).reshape(16, 16, 128)
            cc = r[:, 0:8, :]
            d = r[:, 8:16, :]
            if maybe_first and b == 0:
                cc = cc + modv[5 + jnp.minimum(c, 1), :, _ls(t)][None]
            kf[2 * c + b, t, :, 0:8, :] = d - cc
            kf[2 * c + b, t, :, 8:16, :] = cc + d
            kf[2 * c + b, t, :, 16:24, :] = cc

    def lag_idx(c, cmin, cmax, nout):
        top = 2 * c + nout - 1
        nlag = 2 * cmax + nout
        jok = 2 * cmin + nout - 1
        kidx = [j if j <= jok else jnp.minimum(j, top) for j in range(nlag)]
        xidx = [top + 1 - j if j <= jok + 1 else jnp.maximum(top + 1 - j, 0) for j in range(nlag)]
        return kidx, xidx, nout

    def block_conv(idx, t, us):
        kidx, xidx, nout = idx
        xs = []
        acc = [None] * nout
        for j in reversed(range(len(kidx))):
            k = kf[kidx[j], t, us]
            xs = [xf[xidx[j], t, us]] + xs[:nout - 1]
            for o in reversed(range(len(xs))):
                p = k * xs[o]
                acc[o] = p if acc[o] is None else acc[o] + p
        return [(a[..., 16:24, :] - a[..., 8:16, :], a[..., 16:24, :] + a[..., 0:8, :]) for a in reversed(acc)]

    def cone(c, idx, t, u, pin=None):
        nout = idx[2]
        if nout == 2:
            ri = [((re[0], im[0]), (re[1], im[1])) for re, im in block_conv(idx, t, slice(2 * u, 2 * u + 2))]
        else:
            hs = []
            for h in range(2):
                hs.append(block_conv(idx, t, 2 * u + h))
                tot = [re + im for re, im in hs[h]]
                pin(h, (tot[0] + tot[1]) + (tot[2] + tot[3]))
            ri = list(zip(*hs))
        qs = [(h0[0] + h1[0], h0[1] + h1[1], h0[0] - h1[0], h0[1] - h1[1]) for h0, h1 in ri]
        qv = qbuf.at[pl.ds(c, nout // 2 + 1)]
        qv[nout // 2, t, u] = jnp.concatenate(qs[-1], axis=0)
        prev = qv[0, t, u]
        pv = (prev[0:8], prev[8:16], prev[16:24], prev[24:32])
        res = []
        for cur in qs:
            res.append(jnp.concatenate([cur[0] - pv[1], cur[1] + pv[0]], axis=0))
            res.append(jnp.concatenate([cur[2] - pv[3], cur[3] + pv[2]], axis=0))
            pv = cur
        return res

    def stage_d(yi, t, wfn):
        for b in range(2):
            for par in range(2):
                g = cst_v[2 * C + 64 * par:2 * C + 64 * (par + 1), :]
                y = jnp.dot(g, wfn(2 * b + par), preferred_element_type=F32)
                ybuf[yi, t, pl.ds(b * C + par, 64, stride=2), :] = y

    def ab_all(c):
        for t in range(LT):
            stage_b(c, t, True)
            stage_a(c, t)

    def widen_k(c):
        kk = k_v[c].astype(F32)
        for t in range(LT):
            kbuf[t, pl.ds(_mo(c * M, M) + 32, M), :] = kk[:, _ls(t)]

    def cd_all(c, cmin, cmax):
        idx = lag_idx(c, cmin, cmax, 2)
        for t in range(LT):
            eo = [cone(c, idx, t, u) for u in range(8)]
            stage_d(c, t, lambda n: jnp.concatenate([e[n] for e in eo], axis=0).astype(BF16))

    def norm2_rows(c, r0, yi, x1dst, n1=None):
        rows = slice(r0, r0 + 16)
        x = q_v[c, rows, :].astype(F32).reshape(2, 8, D)
        y = jnp.concatenate([ybuf[yi, t, rows, :] for t in range(LT)], axis=1).reshape(2, 8, D)
        x1 = x + ((_ln(x) if n1 is None else n1) * modv[0][None] + modv[1][None]) * y
        x1dst[rows, :] = x1.reshape(16, D)
        return _ln(x1)

    def mod2(n2):
        return (n2 * modv[2][None] + modv[3][None]).reshape(16, D)

    def store_lhs(dst, r8, top, bot, with_left=True):
        rows = slice(r8, r8 + 8)
        for kt in range(2):
            ss = _asums(top[:, _ls(kt)], top[:, _ls(2 + kt)], bot[:, _ls(kt)], bot[:, _ls(2 + kt)])
            for i in range(7):
                dst[rows, _ls(2 * i + kt)] = _pack(ss[i])
        if with_left:
            dst[rows, _ls(14)] = _pack(top[:, _ls(4)])
            dst[rows, _ls(15)] = _pack(bot[:, _ls(4)])
        return ss[0]

    def mod_cols(c0, c1):
        cf = c_v[...].astype(F32)
        sc = cf * (1.0 / (1.0 + jnp.exp(-cf)))
        lhs = jnp.broadcast_to(sc, (16, D)).astype(BF16)
        return jnp.dot(lhs, wm_v[:, c0:c1], preferred_element_type=F32)[0:8]

    def mod_part(n0, n1):
        mod = mod_cols(n0 * D, n1 * D)
        return [mod[:, n * D:(n + 1) * D] for n in range(n1 - n0)]

    bspec = [((0, 0), (1, 1)), ((0, 0), None), ((0, 1), (1, 1)), ((1, 0), (0, 0)),
             ((1, 1), None), ((0, 0), (0, 1)), ((1, 0), (1, 1))]

    def bsum(quad, i):
        qa, qb = bspec[i]
        if qb is None:
            return pltpu.bitcast(quad(*qa), U32)
        return _pack(quad(*qa).astype(F32) - quad(*qb).astype(F32))

    def prep_gu(col):
        p, mat, i = col // 16, (col // 8) % 2, col % 8
        w = (wg_v, wu_v)[mat]
        if i == 7:
            for cc in range(2):
                wgu[64 * cc:64 * cc + 64, _ls(col)] = pltpu.bitcast(w[512:640, _ls(2 * p + cc)], U32)
        else:
            wgu[0:128, _ls(col)] = bsum(lambda r, c: w[256 * r:256 * r + 256, _ls(2 * p + c)], i)

    def prep_dn(col):
        for p in range(6):
            if col >= 14:
                val = pltpu.bitcast(wd_v[_ls(2 * p + col - 14), _ls(4)], U32)
            else:
                val = bsum(lambda r, c: wd_v[_ls(2 * p + r), _ls(2 * (col // 7) + c)], col % 7)
            wdn[64 * p:64 * p + 64, _ls(col)] = val

    def step(s, mode):
        warm, main, last = mode == "warm", mode == "main", mode == "last"
        nch = 1 if last else 2
        R = 64 * nch
        off = 128 * (s % 2)
        lv = lhsb.at[pl.ds(pl.multiple_of((s - 2) * 64, 64), 2 * R)]
        x1v = x1buf.at[pl.ds(s - 2, 2 * nch)]
        dl_w = dlb.at[pl.ds(pl.multiple_of((s % 2) * 32, 32), R)]
        dl_r = dlb.at[pl.ds(pl.multiple_of(((s + 2) % 2) * 32, 32), R)]

        items = [[] for _ in range(112)]
        if warm:
            c0, nout = s + 1, 2
            idx = lag_idx(c0, W_CMIN, 3, nout)
            items[W_D].append(("d", 0))
            for m, names in W_WAITS.items():
                for name in names:
                    items[m].append(("w", name))
            items[W_AB].append(("ab", 0))
            items[W_MOD].append(("mod", 0))
            c_slots, e_slots, yis = WC_SLOTS, WE_SLOTS, (2, 0)
        elif main:
            c0, nout = s, 4
            idx = lag_idx(c0, 4, 6, nout)
            items[AB_SLOT].append(("ab", 0))
            items[D_SLOT].append(("d", 0))
            c_slots, e_slots, yis = C_SLOTS, E_SLOTS, (0, 1)
        if not last:
            for n, m in enumerate(() if warm else WK_SLOTS):
                items[m].append(("wk", n))
            for p in range(40):
                items[c_slots[p]].append(("c", p))
            for g in range(32):
                items[e_slots[g]].append(("e", g))
        tops, hist, where = {}, {}, {}
        slot = [0]

        def pin_rows(nrows, n):
            return pl.ds(_mo(nrows + off + 8 * n, 8), 8)

        def hook(ref, nrows, col):
            m = slot[0]
            slot[0] += 1
            npin = 0
            todo = [x for x in items[m] if x[0] not in ("c", "e")]
            if warm and not (m < 96 and m % 8 == 7):
                todo.append(("prep", col))
            todo += [x for x in items[m] if x[0] in ("c", "e")]
            for kind, p in todo:
                if kind == "w":
                    wait(p)
                elif kind == "prep":
                    (prep_gu if m < 96 else prep_dn)(p)
                elif kind == "mod":
                    modv[4] = mod_part(5, 6)[0]
                elif kind == "ab":
                    if warm:
                        rw = pl.multiple_of(8 * ((s + (32 + 3 * M) // 8 - 2) % 2048), 8)
                        kk = k_v[c0].astype(F32)
                        for t in range(LT):
                            kbuf[t, pl.ds(rw, M), :] = kk[:, _ls(t)]
                    for ch in range(nout // 2):
                        for t in range(LT):
                            stage_b(c0 + ch, t)
                            stage_a(c0 + ch, t)
                elif kind == "wk":
                    for r in range(WK_SUB):
                        r0 = 8 * (32 * r // WK_SUB)
                        widen_next_k(s, WK_SUB * p + r, hist[m - 1][r0:r0 + 8])
                elif kind == "d":
                    for ch in range(nout // 2):
                        for t in range(LT):
                            def wfn(n):
                                parts = []
                                for u in range(8):
                                    rf, nr, cl = where[8 * t + u]
                                    parts.append(rf[pin_rows(nr, 8 * ch + n), _ls(cl)])
                                return pltpu.bitcast(jnp.concatenate(parts, axis=0), BF16)
                            stage_d(ch, t, wfn)
                    if main:
                        out_copy(s - 4).wait()

                        @pl.when(s == 4)
                        def _():
                            wait("r2")
                elif kind == "c":
                    def pin(h, val):
                        ref[pin_rows(nrows, 15 - 3 * h), _ls(col)] = pltpu.bitcast(val, U32)
                    res = cone(c0, idx, p // 8, p % 8, pin)
                    n0 = (4, 12, 0, 8)[npin // 4] if warm else 0
                    for n in range(2 * nout):
                        ref[pin_rows(nrows, n0 + n % 4 + 8 * (n // 4)), _ls(col)] = _pack(res[n])
                    where[p] = (ref, nrows + 8 * n0, col)
                    npin += 2 * nout
                else:
                    ch, g, half = p // 16, (p % 16) // 2, p % 2
                    h2 = mod2(norm2_rows(s + ch, 16 * g + C * half, yis[ch], x1v.at[2 + ch]))
                    if half == 0:
                        tops[g] = h2
                        val = h2[:, _ls(4)]
                    else:
                        val = store_lhs(lv, R + 64 * ch + 8 * g, tops[g], h2)
                    ref[pin_rows(nrows, npin), _ls(col)] = _pack(val)
                    npin += 1
                assert npin <= (16 if warm and kind == 'c' else 8)

        def dot(a, w):
            r = jnp.dot(pltpu.bitcast(a, BF16), pltpu.bitcast(w, BF16), preferred_element_type=F32)
            hist.setdefault(slot[0] - 1, r)
            return r

        def strassen(lhs, ref, nrows, base, left):
            def m(i):
                hook(ref, nrows, base + i - 1)
                return dot(lhs(i - 1), ref[0:nrows, _ls(base + i - 1)])
            m2 = m(2)
            m4 = m(4)
            c21 = m2 + m4
            m3 = m(3)
            m5 = m(5)
            c12 = m3 + m5
            c11 = m4 + m5
            c22 = m3 + m2
            m1 = m(1)
            m7 = m(7)
            c11 = c11 + m1 + m7
            c22 = c22 - m1
            c22 = c22 - m(6)
            if left is not None:
                hook(ref, nrows, base + 7)
                c22 = c22 + left(1, 1)
                c11 = c11 + left(0, 0)
                c12 = c12 + left(0, 1)
                c21 = c21 + left(1, 0)
            return c11, c12, c21, c22

        for p in range(6):
            res = []
            for mat in range(2):
                base = (2 * p + mat) * 8
                res.append(strassen(
                    lambda i: lv[0:R, 256 * i:256 * i + 256], wgu, 128, base,
                    lambda r, c: accb[r, :, _ls(12 * mat + 2 * p + c)] if warm else
                    dot(lv[0:R, _ls(14 + r)], wgu[64 * c:64 * c + 64, _ls(base + 7)])))
            hq = [res[0][i] * res[1][i] for i in range(4)]
            for i, x in enumerate(_asums(*hq) + [hq[1], hq[2]]):
                if p < 5:
                    dl_w[:, _ls(5 * i + p)] = _pack(x)
                else:
                    dl5[0:R, _ls(i)] = _pack(x)

        def dla(i):
            return dl_r[:, 640 * i:640 * i + 640]

        def dlz(i):
            return dl5[0:R, _ls(i)]

        def dl(i):
            return jnp.concatenate([dla(i), dlz(i)], axis=1)

        def emit(r, n, o):
            rows = slice(r * C, (r + 1) * C)
            for ch in range(nch):
                res = (x1v[ch, rows, _ls(n)].reshape(16, 8, 128)
                       + o[ch * C:(ch + 1) * C].reshape(16, 8, 128) * modv[4, :, _ls(n)][None])
                o_v[s - 2 + ch, rows, _ls(n)] = res.reshape(C, 128).astype(BF16)

        hook(wdn, 384, 14)
        ta = dot(dla(2), wdn[0:320, _ls(14)])
        tb = dot(dla(8), wdn[0:320, _ls(14)])
        ta = ta + dot(dlz(2), wdn[320:384, _ls(14)])
        tb = tb + dot(dlz(8), wdn[320:384, _ls(14)])
        hook(wdn, 384, 15)
        emit(0, 4, ta + dot(dl(7), wdn[0:384, _ls(15)]))
        emit(1, 4, tb + dot(dl(3), wdn[0:384, _ls(15)]))
        if last:
            out_copy(s - 2, *last_parts[0]).start()
        for pp in range(2):
            cs = strassen(dl, wdn, 384, 7 * pp, None)
            for n, i in enumerate((2, 1, 0, 3)):
                emit(i // 2, 2 * pp + i % 2, cs[i])
                if last and pp == 1:
                    out_copy(s - 2, *last_parts[2 + n]).start()
            if last and pp == 0:
                out_copy(s - 2, *last_parts[1]).start()
        if not last:
            out_copy(s - 2).start()

    wait("k0")
    widen_k(0)

    def conv012(c, carry):
        for n in range(3):
            @pl.when(c == n)
            def _():
                wait("c%d" % n)
        with jax.named_scope("ab"):
            ab_all(c)

        for n in range(2):
            @pl.when(c == n)
            def _():
                wait("k%d" % (n + 1))

        @pl.when(c < 2)
        def _():
            widen_k(c + 1)

        for n in range(3):
            @pl.when(c == n)
            def _():
                with jax.named_scope("cd"):
                    cd_all(c, n, n)
        return carry
    lax.fori_loop(0, 3, conv012, 0)
    wait("q01")

    def ln01(c, carry):
        with jax.named_scope("ln1"):
            for g in range(16):
                x = q_v[c, 16 * g:16 * g + 16, :].astype(F32).reshape(2, 8, D)
                wbuf[c, 16 * g:16 * g + 16, :] = _ln(x).reshape(16, D)
        return carry
    lax.fori_loop(0, 2, ln01, 0)

    def passes(i, s):
        @pl.when(i == 0)
        def _():
            wait("wm1")
            with jax.named_scope("mod1"):
                sa, ca, ga = mod_part(0, 3)
                modv[0] = ga * (1.0 + ca)
                modv[1] = ga * sa

                def norm01(c, carry):
                    for g in range(16):
                        rows = slice(16 * g, 16 * g + 16)
                        wbuf[c, rows, :] = norm2_rows(c, 16 * g, c, x1buf.at[c],
                                                      wbuf[c, rows, :].reshape(2, 8, D)).reshape(16, D)
                    return carry
                lax.fori_loop(0, 2, norm01, 0)
            wait("k4")
            with jax.named_scope("k4"):
                modv[3, :, _ls(4)] = mod_cols(4 * D - 128, 4 * D)
                modv[2, :, _ls(4)] = 1.0 + mod_cols(5 * D - 128, 5 * D)
                n2 = jnp.concatenate([wbuf[c, r * C:(r + 1) * C, _ls(4)] for r in range(2) for c in range(2)], axis=0)
                h4 = (n2.reshape(64, 8, 128) * modv[2, :, _ls(4)][None] + modv[3, :, _ls(4)][None])
                h4 = h4.reshape(2 * M, 128).astype(BF16)
                for p in range(6):
                    for mat in range(2):
                        prep_gu((2 * p + mat) * 8 + 7)
                        for cc in range(2):
                            w = pltpu.bitcast(wgu[64 * cc:64 * cc + 64, _ls((2 * p + mat) * 8 + 7)], BF16)
                            r = jnp.dot(h4, w, preferred_element_type=F32)
                            accb[:, :, _ls(12 * mat + 2 * p + cc)] = r.reshape(2, M, 128)
            wait("wm2")
            with jax.named_scope("mod2"):
                modv[3, :, 0:512] = mod_cols(3 * D, 4 * D - 128)
                modv[2, :, 0:512] = 1.0 + mod_cols(4 * D, 5 * D - 128)
                for c in range(2):
                    for g in range(8):
                        top, bot = [mod2(wbuf[c, r:r + 16, :].reshape(2, 8, D)) for r in (16 * g, C + 16 * g)]
                        store_lhs(lhsb, 64 * c + 8 * g, top, bot, False)
            step(s, "warm")
            wait("r1")
            with jax.named_scope("widen45"):
                def widen45(c, carry):
                    widen_k(c)
                    return carry
                lax.fori_loop(4, 6, widen45, 0)

        @pl.when(jnp.logical_and(i > 0, i < 3))
        def _():
            with jax.named_scope("main"):
                step(s, "main")

        @pl.when(i >= 3)
        def _():
            with jax.named_scope("tail"):
                step(s, "last")
        return s + jnp.where(i < 3, 2, 1)
    lax.fori_loop(0, 5, passes, 2)

    with jax.named_scope("wait_out"):
        out_copy(4).wait()
        for c in (6, 7):
            for part in last_parts:
                out_copy(c, *part).wait()


@jax.jit
def pallas_adaLN_cond__ssm_conv_h3__glu_gated_bilinear__prompt_kernel(A_q, A_k, A_v, A_shift_k, A_ssm_k, A_ssm_D, B_x, B_w_gate, B_w_up, B_w_down, c, w_mod):
    cst = jnp.asarray(_dft_consts(), dtype=BF16)
    any_spec = pl.BlockSpec(memory_space=pl.ANY)
    out = pl.pallas_call(
        _kernel,
        grid=(1,),
        in_specs=[any_spec] * 12,
        out_specs=any_spec,
        out_shape=jax.ShapeDtypeStruct((NC, M, D), BF16),
        scratch_shapes=[
            pltpu.VMEM((NC, M, D), BF16), pltpu.VMEM((NC, M, D), BF16), pltpu.VMEM((NC, M, D), BF16),
            pltpu.VMEM((D, S), BF16),
            pltpu.VMEM((D, FF), BF16), pltpu.VMEM((D, FF), BF16), pltpu.VMEM((FF, D), BF16),
            pltpu.VMEM((D, 6 * D), BF16),
            pltpu.VMEM((3 * C, C), BF16),
            pltpu.VMEM((NC, M, D), BF16),
            pltpu.VMEM((LT, 32 + S + 2 * M, 128), F32),
            pltpu.VMEM((NB + 1, LT, 16, 24, 128), F32),
            pltpu.VMEM((NB, LT, 16, 24, 128), F32),
            pltpu.VMEM((NC + 1, LT, 8, 32, 128), F32),
            pltpu.VMEM((3, LT, M, 128), F32),
            pltpu.VMEM((NC + 2, M, D), F32),
            pltpu.VMEM(((NC + 2) * 64, 16 * 128), U32),
            pltpu.VMEM((128 + 128, 96 * 128), U32),
            pltpu.VMEM((384 + 64, 16 * 128), U32),
            pltpu.VMEM((128 + 32, 9 * 640), U32),
            pltpu.VMEM((2 * 64, 9 * 128), U32),
            pltpu.VMEM((2, M, D), F32),
            pltpu.VMEM((2, M, 24 * 128), F32),
            pltpu.VMEM((8, 8, D), F32),
            pltpu.VMEM((4, 8, D), F32),
            pltpu.VMEM((4, D), BF16), pltpu.VMEM((D,), BF16), pltpu.VMEM((1, D), BF16),
            pltpu.VMEM((14, 1, 128), F32),
            pltpu.SemaphoreType.DMA((18,)),
            pltpu.SemaphoreType.DMA(()),
        ],
        compiler_params=pltpu.CompilerParams(vmem_limit_bytes=120 * 1024 * 1024,
                                             disable_bounds_checks=True, disable_semaphore_checks=True),
        name="fused_h3_glu",
    )(A_q.reshape(NC, M, D), A_k.reshape(NC, M, D), A_v.reshape(NC, M, D), A_shift_k.T, A_ssm_k, A_ssm_D,
      B_w_gate, B_w_up, B_w_down, c, w_mod, cst)
    return out.reshape(1, S, D)
```
